```python
import jax
import jax.numpy as jnp

def _softmax(x, axis=-1):
    return jax.nn.softmax(x, axis=axis)
def _gelu(x):
    return jax.nn.gelu(x, approximate=True)
def _silu(x):
    return jax.nn.silu(x)
def _sigmoid(x):
    return jax.nn.sigmoid(x)
def _layernorm(x, axis=-1, eps=1e-5):
    m = jnp.mean(x, axis=axis, keepdims=True)
    v = jnp.var(x, axis=axis, keepdims=True)
    return (x - m) / jnp.sqrt(v + eps)
def _scatter_add(tgt, idx, src, axis=0):
    return tgt.at[idx].add(src)
def _segment_sum(src, seg, n):
    return jax.ops.segment_sum(src, seg, n)
class _Rng:
    def __init__(self, key):
        self._k = key
    def _next(self):
        self._k, sub = jax.random.split(self._k)
        return sub
    def normal(self, shape):
        return jax.random.normal(self._next(), shape, dtype=jnp.bfloat16)
    def randint(self, lo, hi, shape):
        return jax.random.randint(self._next(), shape, lo, hi, dtype=jnp.int32)
    def uniform(self, shape, lo=0.0, hi=1.0):
        return jax.random.uniform(self._next(), shape, jnp.bfloat16, lo, hi)
    def permutation(self, n):
        return jax.random.permutation(self._next(), n)


kernel_name = 'gated_mix__compressed_kv_cla__ssm_conv_s5__prompt'

def setup_inputs():
    _rng = _Rng(jax.random.key(int.from_bytes(__import__("os").urandom(4), "little")))
    _w = (lambda a: (lambda t: t.astype(jnp.bfloat16) if jnp.issubdtype(t.dtype, jnp.floating) else t)(jnp.asarray(a)))
    def _A_setup():
        B, H, Sq, Sk, D, M = 1, 16, 2048, 2048, 256, 448
        Dc = 4 * D
        return {
            "x": _w((lambda *s: _rng.normal(s) * 0.05)(B, Sq, M)),
            "c_kv": _w((lambda *s: _rng.normal(s) * 0.05)(B, Sk, Dc)),
            "w_q": _w((lambda *s: _rng.normal(s) * 0.05)(M, H, D) * (M ** -0.5)),
            "w_uk": _w((lambda *s: _rng.normal(s) * 0.05)(Dc, H, D) * (Dc ** -0.5)),
            "w_uv": _w((lambda *s: _rng.normal(s) * 0.05)(Dc, H, D) * (Dc ** -0.5)),
            "w_o": _w((lambda *s: _rng.normal(s) * 0.05)(H, D, M) * ((H * D) ** -0.5)),
        }
    _A_in = _A_setup()

    def _B_setup():
        B, S, D = 1, 2048, 448
        P = D
        Lambda_re = -0.5 * jnp.exp((lambda *s: _rng.normal(s) * 0.05)(P))
        Lambda_im = (lambda *s: _rng.normal(s) * 0.05)(P) * 1.0
        B_re = (lambda *s: _rng.normal(s) * 0.05)(P, D) * (D ** -0.5)
        B_im = (lambda *s: _rng.normal(s) * 0.05)(P, D) * (D ** -0.5)
        C_re = (lambda *s: _rng.normal(s) * 0.05)(D, P) * (P ** -0.5)
        C_im = (lambda *s: _rng.normal(s) * 0.05)(D, P) * (P ** -0.5)
        log_dt = (lambda *s: _rng.normal(s) * 0.05)(P) * 0.3 - 2.0
        Dskip = (lambda *s: _rng.normal(s) * 0.05)(D)
        return {
            "x": _w((lambda *s: _rng.normal(s) * 0.05)(B, S, D)),
            "Lambda_re": _w(Lambda_re),
            "Lambda_im": _w(Lambda_im),
            "B_re": _w(B_re),
            "B_im": _w(B_im),
            "C_re": _w(C_re),
            "C_im": _w(C_im),
            "log_dt": _w(log_dt),
            "Dskip": _w(Dskip),
        }
    _B_in = _B_setup()

    return {
        "A_x": _A_in["x"],
        "A_c_kv": _A_in["c_kv"],
        "A_w_q": _A_in["w_q"],
        "A_w_uk": _A_in["w_uk"],
        "A_w_uv": _A_in["w_uv"],
        "A_w_o": _A_in["w_o"],
        "B_x": _B_in["x"],
        "B_Lambda_re": _B_in["Lambda_re"],
        "B_Lambda_im": _B_in["Lambda_im"],
        "B_B_re": _B_in["B_re"],
        "B_B_im": _B_in["B_im"],
        "B_C_re": _B_in["C_re"],
        "B_C_im": _B_in["C_im"],
        "B_log_dt": _B_in["log_dt"],
        "B_Dskip": _B_in["Dskip"],
        "gate_w": _w((lambda *s: _rng.normal(s) * 0.05)(448)),
    }

def reference(A_x, A_c_kv, A_w_q, A_w_uk, A_w_uv, A_w_o, B_x, B_Lambda_re, B_Lambda_im, B_B_re, B_B_im, B_C_re, B_C_im, B_log_dt, B_Dskip, gate_w):
    def _A_ref(x, c_kv, w_q, w_uk, w_uv, w_o):
        B, Sq, M = x.shape[0], x.shape[1], x.shape[2]
        Sk = c_kv.shape[1]
        H, D = w_q.shape[1], w_q.shape[2]
        q = jnp.einsum("bqm,mhd->bhqd", x, w_q)
        k = jnp.einsum("bkc,chd->bhkd", c_kv, w_uk)
        v = jnp.einsum("bkc,chd->bhkd", c_kv, w_uv)
        scores = jnp.einsum("bhqd,bhkd->bhqk", q, k) * (D ** -0.5)
        off = Sk - Sq
        qi = jnp.arange(Sq)[:, None]
        kj = jnp.arange(Sk)[None, :]
        cmask = kj <= (qi + off)
        scores = jnp.where(cmask[None, None], scores, -1e9)
        p = _softmax(scores, axis=-1)
        ctx = jnp.einsum("bhqk,bhkd->bhqd", p, v)
        return jnp.einsum("bhqd,hdm->bqm", ctx, w_o)

    def _B_ref(x, Lambda_re, Lambda_im, B_re, B_im, C_re, C_im, log_dt, Dskip):
        Bsz, L, H = x.shape
        Lam = Lambda_re + 1j * Lambda_im
        Bmat = B_re + 1j * B_im
        Cmat = C_re + 1j * C_im
        dt = jnp.exp(log_dt)
        Lam_bar = jnp.exp(dt * Lam)
        B_bar = ((Lam_bar - 1.0) / Lam)[:, None] * Bmat
        Bu = jnp.einsum("bld,pd->blp", x + 0j, B_bar)
        h = jnp.zeros_like(Bu[:, 0, :])
        hs = []
        for t in range(L):
            h = Lam_bar[None, :] * h + Bu[:, t, :]
            hs.append(h)
        hseq = jnp.stack(hs, 1)
        y = 2.0 * jnp.einsum("blp,dp->bld", hseq, Cmat).real + x * Dskip[None, None, :]
        return y

    x = A_x
    g = _sigmoid((x * gate_w).sum(-1, keepdims=True))
    a = _A_ref(x, A_c_kv, A_w_q, A_w_uk, A_w_uv, A_w_o)
    b = _B_ref(x, B_Lambda_re, B_Lambda_im, B_B_re, B_B_im, B_C_re, B_C_im, B_log_dt, B_Dskip)
    return g * a + (1 - g) * b
```

```python
import math

import jax
import jax.numpy as jnp
from jax import lax
import jax.experimental.pallas as pl
import jax.experimental.pallas.tpu as pltpu

S, M, H, D, DC = 2048, 448, 16, 256, 1024
BQ = 256
TC = 256
F32, BF16 = jnp.float32, jnp.bfloat16
NT = (((1,), (1,)), ((), ()))


def _dot(a, b):
    return jnp.dot(a, b, preferred_element_type=F32)


def _dot_nt(a, b):
    return lax.dot_general(a, b, NT, preferred_element_type=F32)


def _head_pair(w_ref, j, rows):
    base = pl.multiple_of((j // 4) * 4, 4)
    cols = []
    for c in range(2):
        r = w_ref.at[c].bitcast(jnp.uint32).at[pl.ds(base, rows * 8 - 4)]
        w = r[pl.ds(0, rows, stride=8), :]
        for b in range(1, 4):
            w = jnp.where(j % 4 == b, r[pl.ds(b, rows, stride=8), :], w)
        cols.append(w)
    w = jnp.concatenate(cols, axis=1)
    lo = lax.bitcast_convert_type(w << 16, F32)
    hi = lax.bitcast_convert_type(w & jnp.uint32(0xFFFF0000), F32)
    return lo, hi


def _cmul(ar, ai, br, bi):
    return ar * br - ai * bi, ar * bi + ai * br


def _row(ref):
    return ref[...].astype(F32).reshape(1, M)


def _kernel(xT_hbm, c_hbm, wq_hbm, wk_hbm, wv_hbm, woT_hbm, lre_ref, lim_ref,
            bre_hbm, bim_hbm, cre_hbm, cim_hbm, ldt_ref, dsk_ref, gw_ref,
            outT_hbm,
            xT_v, c_v, wq_v, wk_v, wv_v, woT_v, b_v, cre_v, cim_v,
            qT_v, ure_v, uim_v, hre_v, him_v, k_v, vT_v, gT_v,
            oT_v, sems, osems):
    halves = lambda r: (r.at[:, :128], r.at[:, 128:])
    srcs = (xT_hbm, bre_hbm, bim_hbm, *halves(wq_hbm), c_hbm, *halves(wk_hbm), *halves(wv_hbm),
            woT_hbm, cre_hbm, cim_hbm)
    dsts = (xT_v, b_v.at[:M], b_v.at[M:2 * M], wq_v.at[0], wq_v.at[1], c_v, wk_v.at[0], wk_v.at[1],
            wv_v.at[0], wv_v.at[1], woT_v, cre_v, cim_v)
    copies = [pltpu.make_async_copy(s, d, sems.at[i]) for i, (s, d) in enumerate(zip(srcs, dsts))]
    for cp in copies:
        cp.start()

    lre, lim = _row(lre_ref), _row(lim_ref)
    dt = jnp.exp(_row(ldt_ref)).astype(BF16).astype(F32)
    mag = jnp.exp(dt * lre)
    a1r, a1i = mag * jnp.cos(dt * lim), mag * jnp.sin(dt * lim)
    den = lre * lre + lim * lim
    cfr, cfi = _cmul(a1r - 1.0, a1i, 2.0 * lre / den, -2.0 * lim / den)
    a2r, a2i = _cmul(a1r, a1i, a1r, a1i)
    a4r, a4i = _cmul(a2r, a2i, a2r, a2i)
    row = lax.broadcasted_iota(jnp.int32, (8, M), 0)
    steps = [(s, jnp.where(row >= s, ar, 0.0), jnp.where(row >= s, ai, 0.0))
             for s, ar, ai in ((1, a1r, a1i), (2, a2r, a2i), (4, a4r, a4i))]
    pwr = jnp.broadcast_to(a1r, (8, M))
    pwi = jnp.broadcast_to(a1i, (8, M))
    for s, ar, ai in ((1, a1r, a1i), (2, a2r, a2i), (4, a4r, a4i)):
        nr, ni = _cmul(pwr, pwi, ar, ai)
        on = (row & s) != 0
        pwr, pwi = jnp.where(on, nr, pwr), jnp.where(on, ni, pwi)
    b_v[2 * M:] = jnp.broadcast_to(_row(gw_ref), (16, M)).astype(BF16)

    copies[0].wait()
    copies[1].wait()
    copies[2].wait()
    for t in range(S // TC):
        ts = pl.ds(t * TC, TC)
        u = _dot(b_v[...], xT_v[:, ts])
        ure_v[ts, :] = u[:M].T
        uim_v[ts, :] = u[M:2 * M].T
        gT_v[:, ts] = jax.nn.sigmoid(u[2 * M:2 * M + 8])

    copies[3].wait()
    copies[4].wait()
    qscale = D ** -0.5 * math.log2(math.e)

    def q_and_scan(j, carry):
        w0, w1 = _head_pair(wq_v, j, M)
        wT = jnp.concatenate([w0.T.astype(BF16), w1.T.astype(BF16)], axis=0)
        qT_v[pl.ds(pl.multiple_of(j * 2 * D, 2 * D), 2 * D), :] = (
            _dot(wT, xT_v[...]) * qscale).astype(BF16)
        hr, hi = carry
        base = pl.multiple_of(j * TC, TC)
        outr, outi = [], []
        for a in range(TC // 8):
            ur = ure_v[pl.ds(base + 8 * a, 8), :]
            ui = uim_v[pl.ds(base + 8 * a, 8), :]
            for s, ar, ai in steps:
                dr, di = _cmul(pltpu.roll(ur, s, 0), pltpu.roll(ui, s, 0), ar, ai)
                ur, ui = ur + dr, ui + di
            dr, di = _cmul(hr, hi, pwr, pwi)
            ur, ui = ur + dr, ui + di
            hr = jnp.broadcast_to(ur[7:8], (8, M))
            hi = jnp.broadcast_to(ui[7:8], (8, M))
            outr.append(ur)
            outi.append(ui)
        yr, yi = _cmul(jnp.concatenate(outr, axis=0), jnp.concatenate(outi, axis=0), cfr, cfi)
        hre_v[pl.ds(base, TC), :] = yr.astype(BF16)
        him_v[pl.ds(base, TC), :] = (-yi).astype(BF16)
        return hr, hi

    zero = jnp.zeros((8, M), F32)
    lax.fori_loop(0, H // 2, q_and_scan, (zero, zero))

    for cp in copies[5:10]:
        cp.wait()
    kk = lax.broadcasted_iota(jnp.int32, (BQ, BQ), 0)
    qq = lax.broadcasted_iota(jnp.int32, (BQ, BQ), 1)
    causal = kk <= qq

    def head_pair(j, _):
        wk = _head_pair(wk_v, j, DC)
        wv = _head_pair(wv_v, j, DC)
        w = jnp.concatenate([t.astype(BF16) for t in (*wk, *wv)], axis=1)
        for t in range(S // 512):
            rows = pl.ds(t * 512, 512)
            kv = _dot(c_v[rows, :], w)
            k_v[rows, :] = kv[:, :2 * D].astype(BF16)
            vT_v[:, rows] = kv[:, 2 * D:].T.astype(BF16)
        for e in range(2):
            cols = pl.ds(e * D, D)
            hd = pl.ds(pl.multiple_of(j * 2 * D + e * D, D), D)
            for i in range(S // BQ):
                n = (i + 1) * BQ
                qs = pl.ds(i * BQ, BQ)
                s = _dot(k_v[:n, cols], qT_v[hd, qs])
                sd = jnp.where(causal, s[n - BQ:], -1e30)
                s = sd if i == 0 else jnp.concatenate([s[:n - BQ], sd], axis=0)
                m = jnp.max(s, axis=0, keepdims=True)
                p = jnp.exp2(s - m)
                l = jnp.sum(p, axis=0, keepdims=True)
                ctx = _dot(vT_v[cols, :n], p.astype(BF16))
                qT_v[hd, qs] = (ctx * (1.0 / l)).astype(BF16)
        return 0

    lax.fori_loop(0, H // 2, head_pair, 0)

    for cp in copies[10:]:
        cp.wait()
    dsk = jnp.broadcast_to(_row(dsk_ref), (TC, M)).T
    outs = []
    for t in range(S // TC):
        ts = pl.ds(t * TC, TC)
        a = _dot(woT_v[0], qT_v[:D, ts])
        for h in range(1, H):
            a += _dot(woT_v[h], qT_v[h * D:(h + 1) * D, ts])
        b = (_dot_nt(cre_v[...], hre_v[ts, :]) + _dot_nt(cim_v[...], him_v[ts, :])
             + xT_v[:, ts].astype(F32) * dsk)
        g = gT_v[:1, ts]
        oT_v[:, ts] = g * a + (1.0 - g) * b
        cp = pltpu.make_async_copy(oT_v.at[:, ts], outT_hbm.at[:, ts], osems.at[t])
        cp.start()
        outs.append(cp)
    for cp in outs:
        cp.wait()


@jax.jit
def pallas_gated_mix__compressed_kv_cla__ssm_conv_s5__prompt_kernel(
    A_x: jax.Array,
    A_c_kv: jax.Array,
    A_w_q: jax.Array,
    A_w_uk: jax.Array,
    A_w_uv: jax.Array,
    A_w_o: jax.Array,
    B_x: jax.Array,
    B_Lambda_re: jax.Array,
    B_Lambda_im: jax.Array,
    B_B_re: jax.Array,
    B_B_im: jax.Array,
    B_C_re: jax.Array,
    B_C_im: jax.Array,
    B_log_dt: jax.Array,
    B_Dskip: jax.Array,
    gate_w: jax.Array,
):
    del B_x
    hbm = pl.BlockSpec(memory_space=pltpu.MemorySpace.HBM)
    vmem = pl.BlockSpec(memory_space=pltpu.MemorySpace.VMEM)
    V = pltpu.VMEM
    outT = pl.pallas_call(
        _kernel,
        in_specs=[hbm] * 6 + [vmem] * 2 + [hbm] * 4 + [vmem] * 3,
        out_specs=hbm,
        out_shape=jax.ShapeDtypeStruct((M, S), F32),
        scratch_shapes=[
            V((M, S), BF16), V((S, DC), BF16), V((2, M * H, 128), BF16), V((2, DC * H, 128), BF16),
            V((2, DC * H, 128), BF16), V((H, M, D), BF16),
            V((2 * M + 16, M), BF16), V((M, M), BF16), V((M, M), BF16),
            V((H * D, S), BF16),
            V((S, M), F32), V((S, M), F32), V((S, M), BF16), V((S, M), BF16),
            V((S, 2 * D), BF16), V((2 * D, S), BF16), V((8, S), F32),
            V((M, S), F32),
            pltpu.SemaphoreType.DMA((13,)), pltpu.SemaphoreType.DMA((S // TC,)),
        ],
        compiler_params=pltpu.CompilerParams(vmem_limit_bytes=120 * 1024 * 1024),
    )(A_x.reshape(S, M).T, A_c_kv.reshape(S, DC), A_w_q.reshape(M * H, D), A_w_uk.reshape(DC * H, D),
      A_w_uv.reshape(DC * H, D), A_w_o.transpose(0, 2, 1), B_Lambda_re, B_Lambda_im,
      B_B_re, B_B_im, B_C_re, B_C_im, B_log_dt, B_Dskip, gate_w)
    return outT.T.reshape(1, S, M)
```

```python
import functools
import math

import jax
import jax.numpy as jnp
from jax import lax
import jax.experimental.pallas as pl
import jax.experimental.pallas.tpu as pltpu

S, M, H, D, DC = 2048, 448, 16, 256, 1024
BQ = 256
TC = 256
CK = 512
CR = 512
F32, BF16 = jnp.float32, jnp.bfloat16
NT = (((1,), (1,)), ((), ()))


def _dot(a, b):
    return jnp.dot(a, b, preferred_element_type=F32)


def _dot_nt(a, b):
    return lax.dot_general(a, b, NT, preferred_element_type=F32)


def _head_pair(w_ref, j, lo, rows, halves=(0, 1)):
    base = pl.multiple_of((j // 4) * 4, 4) + lo * 8
    cols = []
    for c in halves:
        r = w_ref.at[c].bitcast(jnp.uint32).at[pl.ds(base, rows * 8 - 4)]
        w = r[pl.ds(0, rows, stride=8), :]
        for b in range(1, 4):
            w = jnp.where(j % 4 == b, r[pl.ds(b, rows, stride=8), :], w)
        cols.append(w)
    w = jnp.concatenate(cols, axis=1)
    lo = lax.bitcast_convert_type(w << 16, F32)
    hi = lax.bitcast_convert_type(w & jnp.uint32(0xFFFF0000), F32)
    return lo, hi


def _pacer(j):
    zero = jnp.full((8, 128), j >> 4, jnp.int32)

    def after(x, dep):
        bits = lax.bitcast_convert_type(dep, jnp.int32) & zero
        bits = jnp.tile(bits, (x.shape[0] // 8, -(-x.shape[1] // 128)))[:, :x.shape[1]]
        return lax.bitcast_convert_type(lax.bitcast_convert_type(x, jnp.int32) | bits, F32)
    return after


def _pace(work, n, deps, lo, hi):
    next(work)
    for i in range(n):
        work.send(deps[int((lo + (hi - lo) * i / n) * len(deps))])


def _lhs7(a11, a12, a21, a22):
    return a11 + a22, a21 + a22, a11, a22, a11 + a12, a21 - a11, a12 - a22


def _rhs7(b11, b12, b21, b22):
    return b11 + b22, b11, b12 - b22, b21 - b11, b22, b11 + b12, b21 + b22


def _combine7(m):
    return m[0] + m[3] - m[4] + m[6], m[2] + m[4], m[1] + m[3], m[0] - m[1] + m[2] + m[5]


def _cmul(ar, ai, br, bi):
    return ar * br - ai * bi, ar * bi + ai * br


def _row(ref):
    return ref[...].astype(F32).reshape(1, M)


def _kernel(xT_hbm, c_hbm, wq_hbm, wk_hbm, wv_hbm, woT_hbm, lre_ref, lim_ref,
            bre_hbm, bim_hbm, cre_hbm, cim_hbm, ldt_ref, dsk_ref, gw_ref,
            outT_hbm,
            xT_v, c_v, wq_v, wk_v, wv_v, woT_v, b_v, cre_v, cim_v,
            qT_v, ure_v, uim_v, hre_v, him_v, k_v, vT_v, gT_v, w_v, s_v, p_v, wqT_v, ca_v,
            oT_v, sems, osems):
    halves = lambda r: (r.at[:, :128], r.at[:, 128:])
    srcs = (xT_hbm, bre_hbm, bim_hbm, *halves(wq_hbm), c_hbm, *halves(wk_hbm), *halves(wv_hbm),
            woT_hbm, cre_hbm, cim_hbm)
    dsts = (xT_v, b_v.at[:M], b_v.at[M:2 * M], wq_v.at[0], wq_v.at[1], c_v, wk_v.at[0], wk_v.at[1],
            wv_v.at[0], wv_v.at[1], woT_v, cre_v, cim_v)
    copies = [pltpu.make_async_copy(s, d, sems.at[i]) for i, (s, d) in enumerate(zip(srcs, dsts))]
    for cp in copies[:3]:
        cp.start()

    lre, lim = _row(lre_ref), _row(lim_ref)
    dt = jnp.exp(_row(ldt_ref)).astype(BF16).astype(F32)
    mag = jnp.exp(dt * lre)
    a1r, a1i = mag * jnp.cos(dt * lim), mag * jnp.sin(dt * lim)
    den = lre * lre + lim * lim
    cfr, cfi = _cmul(a1r - 1.0, a1i, 2.0 * lre / den, -2.0 * lim / den)
    a2r, a2i = _cmul(a1r, a1i, a1r, a1i)
    a4r, a4i = _cmul(a2r, a2i, a2r, a2i)
    row = lax.broadcasted_iota(jnp.int32, (8, M), 0)
    steps = [(s, jnp.where(row >= s, ar, 0.0), jnp.where(row >= s, ai, 0.0))
             for s, ar, ai in ((1, a1r, a1i), (2, a2r, a2i), (4, a4r, a4i))]
    pwr = jnp.broadcast_to(a1r, (8, M))
    pwi = jnp.broadcast_to(a1i, (8, M))
    for s, ar, ai in ((1, a1r, a1i), (2, a2r, a2i), (4, a4r, a4i)):
        nr, ni = _cmul(pwr, pwi, ar, ai)
        on = (row & s) != 0
        pwr, pwi = jnp.where(on, nr, pwr), jnp.where(on, ni, pwi)
    b_v[2 * M:] = jnp.broadcast_to(_row(gw_ref), (16, M)).astype(BF16)

    copies[0].wait()
    copies[1].wait()
    copies[2].wait()
    copies[3].start()
    copies[4].start()
    for t in range(S // TC):
        ts = pl.ds(t * TC, TC)
        u = _dot(b_v[...], xT_v[:, ts])
        ure_v[ts, :] = u[:M].T
        uim_v[ts, :] = u[M:2 * M].T
        gT_v[:, ts] = jax.nn.sigmoid(u[2 * M:2 * M + 8])

    copies[3].wait()
    copies[4].wait()
    for cp in copies[5:]:
        cp.start()
    qscale = D ** -0.5 * math.log2(math.e)

    def wq_operands(j, slot, after):
        for c in range(2):
            dep = yield
            for e, w in enumerate(_head_pair(wq_v, j, 0, M, (c,))):
                wqT_v[slot, (2 * e + c) * 128:(2 * e + c + 1) * 128, :] = after(w.T, dep).astype(BF16)
        yield

    def c_operands(t, after):
        for lo in range(0, CR // 2, 16):
            dep = yield
            top, bot = (after(c_v[pl.ds(pl.multiple_of(t * CR + o + lo, 16), 16), :].astype(F32), dep)
                        for o in (0, CR // 2))
            dst = pl.ds(pl.multiple_of(t * (CR // 2) + lo, 16), 16)
            for a, x in enumerate(_lhs7(top[:, :DC // 2], top[:, DC // 2:], bot[:, :DC // 2], bot[:, DC // 2:])):
                ca_v[a, dst, :] = x.astype(BF16)
        yield

    def scan(j, carry, after):
        hr, hi = carry
        for a in range(TC // 16):
            ys = []
            for b in range(2):
                dep = yield
                rows = pl.ds(pl.multiple_of(j * TC + 16 * a + 8 * b, 8), 8)
                ur, ui = after(ure_v[rows, :], dep), after(uim_v[rows, :], dep)
                for s, ar, ai in steps:
                    dr, di = _cmul(pltpu.roll(ur, s, 0), pltpu.roll(ui, s, 0), ar, ai)
                    ur, ui = ur + dr, ui + di
                dr, di = _cmul(hr, hi, pwr, pwi)
                ur, ui = ur + dr, ui + di
                hr = jnp.broadcast_to(ur[7:8], (8, M))
                hi = jnp.broadcast_to(ui[7:8], (8, M))
                ys.append(_cmul(ur, ui, cfr, cfi))
            rows = pl.ds(pl.multiple_of(j * TC + 16 * a, 16), 16)
            hre_v[rows, :] = jnp.concatenate([ys[0][0], ys[1][0]], axis=0).astype(BF16)
            him_v[rows, :] = (-jnp.concatenate([ys[0][1], ys[1][1]], axis=0)).astype(BF16)
        carry[:] = hr, hi
        yield

    def q_and_scan(j, carry, with_c):
        after = _pacer(j)
        deps = []
        for t in range(S // 512):
            q = _dot(wqT_v[0], xT_v[:, t * 512:(t + 1) * 512])
            qT_v[pl.ds(pl.multiple_of(j * 2 * D, 2 * D), 2 * D), t * 512:(t + 1) * 512] = (
                q * qscale).astype(BF16)
            deps += [q[r:r + 8, c:c + 128] for c in range(0, 512, 128) for r in range(0, 512, 128)]
        carry = list(carry)
        _pace(scan(j, carry, after), TC // 8, deps, 0.0, 0.85)
        if with_c:
            _pace(c_operands(j - H // 4, after), CR // 32, deps, 0.0, 0.85)
        _pace(wq_operands(jnp.minimum(j + 1, H // 2 - 1), 1, after), 2, deps, 0.2, 0.8)
        wqT_v[0] = wqT_v[1]
        return tuple(carry)

    _pace(wq_operands(0, 0, None or (lambda x, dep: x)), 2, [None], 0.0, 1.0)
    zero = jnp.zeros((8, M), F32)
    carry = lax.fori_loop(0, H // 4, functools.partial(q_and_scan, with_c=False), (zero, zero))
    copies[5].wait()
    lax.fori_loop(H // 4, H // 2, functools.partial(q_and_scan, with_c=True), carry)

    for cp in copies[6:10]:
        cp.wait()
    kk = lax.broadcasted_iota(jnp.int32, (128, BQ), 0)
    qq = lax.broadcasted_iota(jnp.int32, (128, BQ), 1)
    causal = kk <= qq

    def kv_operands(j, after):
        for t, w_ref in enumerate((wk_v, wv_v)):
            for lo in range(0, DC // 2, 32):
                dep = yield
                top, bot = ([after(w, dep) for w in _head_pair(w_ref, j, o + lo, 32)]
                            for o in (0, DC // 2))
                for a, x in enumerate(_rhs7(*top, *bot)):
                    w_v[a, lo:lo + 32, t * D:(t + 1) * D] = x.astype(BF16)
        yield

    _pace(kv_operands(0, lambda x, dep: x), DC // 32, [None], 0.0, 1.0)

    def head_pair(j, _):
        after = _pacer(j)

        def project(t):
            m = [_dot(ca_v[a, t * (CR // 2):(t + 1) * (CR // 2), :], w_v[a]) for a in range(7)]
            deps = [x[r:r + 8, c:c + 128] for x in m for c in range(0, 512, 128)
                    for r in range(0, CR // 2, 128)]
            return m, deps

        def finish(t, m):
            for lo in range(0, CR // 2, 128):
                for col in range(0, 2 * D, 128):
                    dep = yield
                    x = [y[lo:lo + 128, col:col + 128] for y in m]
                    x[0], x[1], x[2] = (after(y, dep) for y in x[:3])
                    for a, y in enumerate(_combine7(x)):
                        rows = pl.ds(t * CR + (a // 2) * (CR // 2) + lo, 128)
                        cols = pl.ds((a % 2) * D + col % D, 128)
                        if col < D:
                            k_v[rows, cols] = y.astype(BF16)
                        else:
                            vT_v[cols, rows] = y.T.astype(BF16)
            yield

        tasks = [(0, i) for i in range(S // BQ)] + [(1, i) for i in reversed(range(S // BQ))]
        st = [dict() for _ in tasks]

        def where(t):
            e, i = tasks[t]
            return (pl.ds(e * D, D), pl.ds(pl.multiple_of(j * 2 * D + e * D, D), D),
                    pl.ds(i * BQ, BQ), i * BQ + 128)

        def chunks(n):
            ends = list(range(0, n - 255, CK))[1:] + [n]
            return zip([0] + ends[:-1], ends)

        def colmax(x):
            return jnp.max(x.reshape(-1, 8, x.shape[1]), axis=0)

        def scores(t):
            cols, hd, qs, n = where(t)
            q = qT_v[hd, qs]
            for lo, hi in chunks(n):
                s = s0 = _dot(k_v[lo:hi, cols], q)
                if hi == n:
                    sd = jnp.where(causal, s[hi - lo - 128:], -1e30)
                    s = sd if hi - lo == 128 else jnp.concatenate([s[:hi - lo - 128], sd], axis=0)
                s_v[t % 2, lo:hi, :] = s
                m = colmax(s) if lo == 0 else jnp.maximum(m, colmax(s))
                for r in range(0, hi - lo, 32):
                    yield s0[r:r + 8, :128]
            s = _dot(k_v[n:n + 128, cols], q[:, 128:])
            yield s[:8]
            yield s[64:72]
            s = jnp.where(causal[:, :128], s, -1e30)
            s_v[t % 2, n:n + 128, 128:] = s
            st[t]["m"] = jnp.concatenate([m[:, :128], jnp.maximum(m[:, 128:], colmax(s))], axis=1)

        def softmax(t):
            n = where(t)[3]
            m = jnp.broadcast_to(jnp.max(st[t]["m"], axis=0, keepdims=True), (8, BQ))
            for rows, c in ([(pl.ds(lo, 32), 0) for lo in range(0, n, 32)]
                            + [(pl.ds(lo, 64), 128) for lo in (n, n + 64)]):
                dep = yield
                p = jnp.exp2(s_v[t % 2, rows, c:].reshape(-1, 8, BQ - c) - after(m[:, c:], dep))
                p_v[t % 2, rows, c:] = p.reshape(-1, BQ - c).astype(BF16)
                p = jnp.sum(p, axis=0)
                if c:
                    l = jnp.concatenate([l[:, :c], l[:, c:] + p], axis=1)
                else:
                    l = p if rows.start == 0 else l + p
            st[t]["l"] = l
            yield

        def context(t):
            cols, hd, qs, n = where(t)
            tail = _dot(vT_v[cols, n:n + 128], p_v[t % 2, n:n + 128, 128:])
            yield tail[:8]
            yield tail[128:136]
            for lo, hi in chunks(n):
                d = _dot(vT_v[cols, lo:hi], p_v[t % 2, lo:hi, :])
                acc = d if lo == 0 else acc + d
                k = (hi - lo) // 32
                for r in range(k):
                    yield d[r * D // k // 8 * 8:][:8, :128]
            acc = jnp.concatenate([acc[:, :128], acc[:, 128:] + tail], axis=1)
            l = jnp.sum(st[t]["l"], axis=0, keepdims=True)
            qT_v[hd, qs] = (acc * (1.0 / l)).astype(BF16)

        m, _ = project(0)
        for t in range(1, S // CR):
            m_next, deps = project(t)
            _pace(finish(t - 1, m), CR // 64, deps, 0.0, 0.8)
            m = m_next
        deps = list(scores(0))
        late = []
        for t in range(len(tasks) + 1):
            deps = list(context(t - 1)) if t > 0 else []
            if t + 1 < len(tasks):
                deps += list(scores(t + 1))
            if t < len(tasks):
                _pace(softmax(t), where(t)[3] // 32 + 2, deps, 0.0, 0.8)
            late += deps
            if t == 3:
                _pace(finish(S // CR - 1, m), CR // 64, late, 0.0, 1.0)
                late = []
        _pace(kv_operands(jnp.minimum(j + 1, H // 2 - 1), after), DC // 32, late, 0.0, 0.8)
        return 0

    lax.fori_loop(0, H // 2, head_pair, 0)

    for cp in copies[10:]:
        cp.wait()
    dsk = jnp.broadcast_to(_row(dsk_ref), (TC, M)).T
    outs = []
    for t in range(S // TC):
        ts = pl.ds(t * TC, TC)
        a = _dot(woT_v[0], qT_v[:D, ts])
        for h in range(1, H):
            a += _dot(woT_v[h], qT_v[h * D:(h + 1) * D, ts])
        b = (_dot_nt(cre_v[...], hre_v[ts, :]) + _dot_nt(cim_v[...], him_v[ts, :])
             + xT_v[:, ts].astype(F32) * dsk)
        g = gT_v[:1, ts]
        oT_v[:, ts] = g * a + (1.0 - g) * b
        cp = pltpu.make_async_copy(oT_v.at[:, ts], outT_hbm.at[:, ts], osems.at[t])
        cp.start()
        outs.append(cp)
    for cp in outs:
        cp.wait()


@jax.jit
def pallas_gated_mix__compressed_kv_cla__ssm_conv_s5__prompt_kernel(
    A_x: jax.Array,
    A_c_kv: jax.Array,
    A_w_q: jax.Array,
    A_w_uk: jax.Array,
    A_w_uv: jax.Array,
    A_w_o: jax.Array,
    B_x: jax.Array,
    B_Lambda_re: jax.Array,
    B_Lambda_im: jax.Array,
    B_B_re: jax.Array,
    B_B_im: jax.Array,
    B_C_re: jax.Array,
    B_C_im: jax.Array,
    B_log_dt: jax.Array,
    B_Dskip: jax.Array,
    gate_w: jax.Array,
):
    del B_x
    hbm = pl.BlockSpec(memory_space=pltpu.MemorySpace.HBM)
    vmem = pl.BlockSpec(memory_space=pltpu.MemorySpace.VMEM)
    V = pltpu.VMEM
    outT = pl.pallas_call(
        _kernel,
        in_specs=[hbm] * 6 + [vmem] * 2 + [hbm] * 4 + [vmem] * 3,
        out_specs=hbm,
        out_shape=jax.ShapeDtypeStruct((M, S), F32),
        scratch_shapes=[
            V((M, S), BF16), V((S, DC), BF16), V((2, M * H, 128), BF16), V((2, DC * H, 128), BF16),
            V((2, DC * H, 128), BF16), V((H, M, D), BF16),
            V((2 * M + 16, M), BF16), V((M, M), BF16), V((M, M), BF16),
            V((H * D, S), BF16),
            V((S, M), F32), V((S, M), F32), V((S, M), BF16), V((S, M), BF16),
            V((S, 2 * D), BF16), V((2 * D, S), BF16), V((8, S), F32), V((7, DC // 2, 2 * D), BF16), V((2, S, BQ), F32), V((2, S, BQ), BF16),
            V((2, 2 * D, M), BF16), V((7, S // 2, DC // 2), BF16),
            V((M, S), F32),
            pltpu.SemaphoreType.DMA((13,)), pltpu.SemaphoreType.DMA((S // TC,)),
        ],
        compiler_params=pltpu.CompilerParams(vmem_limit_bytes=120 * 1024 * 1024),
    )(A_x.reshape(S, M).T, A_c_kv.reshape(S, DC), A_w_q.reshape(M * H, D), A_w_uk.reshape(DC * H, D),
      A_w_uv.reshape(DC * H, D), A_w_o.transpose(0, 2, 1), B_Lambda_re, B_Lambda_im,
      B_B_re, B_B_im, B_C_re, B_C_im, B_log_dt, B_Dskip, gate_w)
    return outT.T.reshape(1, S, M)
```

```python
import functools
import math

import jax
import jax.numpy as jnp
from jax import lax
import jax.experimental.pallas as pl
import jax.experimental.pallas.tpu as pltpu

S, M, H, D, DC = 2048, 448, 16, 256, 1024
BQ = 256
TC = 256
CK = 512
CR = 512
F32, BF16 = jnp.float32, jnp.bfloat16
NT = (((1,), (1,)), ((), ()))


def _dot(a, b):
    return jnp.dot(a, b, preferred_element_type=F32)


def _dot_nt(a, b):
    return lax.dot_general(a, b, NT, preferred_element_type=F32)


def _head_pair(w_ref, j, lo, rows, halves=(0, 1)):
    base = pl.multiple_of((j // 4) * 4, 4) + lo * 8
    cols = []
    for c in halves:
        r = w_ref.at[c].bitcast(jnp.uint32).at[pl.ds(base, rows * 8 - 4)]
        w = r[pl.ds(0, rows, stride=8), :]
        for b in range(1, 4):
            w = jnp.where(j % 4 == b, r[pl.ds(b, rows, stride=8), :], w)
        cols.append(w)
    w = jnp.concatenate(cols, axis=1)
    lo = lax.bitcast_convert_type(w << 16, F32)
    hi = lax.bitcast_convert_type(w & jnp.uint32(0xFFFF0000), F32)
    return lo, hi


def _pacer(j):
    zero = jnp.full((8, 128), j >> 4, jnp.int32)

    def after(x, dep):
        bits = lax.bitcast_convert_type(dep, jnp.int32) & zero
        bits = jnp.tile(bits, (x.shape[0] // 8, -(-x.shape[1] // 128)))[:, :x.shape[1]]
        return lax.bitcast_convert_type(lax.bitcast_convert_type(x, jnp.int32) | bits, F32)
    return after


def _pace(work, n, deps, lo, hi):
    next(work)
    for i in range(n):
        work.send(deps[int((lo + (hi - lo) * i / n) * len(deps))])


def _lhs7(a11, a12, a21, a22):
    return a11 + a22, a21 + a22, a11, a22, a11 + a12, a21 - a11, a12 - a22


def _rhs7(b11, b12, b21, b22):
    return b11 + b22, b11, b12 - b22, b21 - b11, b22, b11 + b12, b21 + b22


def _combine7(m):
    return m[0] + m[3] - m[4] + m[6], m[2] + m[4], m[1] + m[3], m[0] - m[1] + m[2] + m[5]


def _cmul(ar, ai, br, bi):
    return ar * br - ai * bi, ar * bi + ai * br


def _row(ref):
    return ref[...].astype(F32).reshape(1, M)


def _kernel(xT_hbm, c_hbm, wq_hbm, wk_hbm, wv_hbm, woT_hbm, lre_ref, lim_ref,
            bre_hbm, bim_hbm, cre_hbm, cim_hbm, ldt_ref, dsk_ref, gw_ref,
            outT_hbm,
            xT_v, c_v, wq_v, wk_v, wv_v, woT_v, b_v, cre_v, cim_v,
            qT_v, ure_v, uim_v, hre_v, him_v, k_v, v_v, vT_v, gT_v, w_v, s_v, p_v, wqT_v, ca_v,
            oT_v, sems, osems):
    halves = lambda r: (r.at[:, :128], r.at[:, 128:])
    srcs = (xT_hbm, bre_hbm, bim_hbm, *halves(wq_hbm), c_hbm, *halves(wk_hbm), *halves(wv_hbm),
            woT_hbm, cre_hbm, cim_hbm)
    dsts = (xT_v, b_v.at[:M], b_v.at[M:2 * M], wq_v.at[0], wq_v.at[1], c_v, wk_v.at[0], wk_v.at[1],
            wv_v.at[0], wv_v.at[1], woT_v, cre_v, cim_v)
    copies = [pltpu.make_async_copy(s, d, sems.at[i]) for i, (s, d) in enumerate(zip(srcs, dsts))]
    for cp in copies[:3]:
        cp.start()

    lre, lim = _row(lre_ref), _row(lim_ref)
    dt = jnp.exp(_row(ldt_ref)).astype(BF16).astype(F32)
    mag = jnp.exp(dt * lre)
    a1r, a1i = mag * jnp.cos(dt * lim), mag * jnp.sin(dt * lim)
    den = lre * lre + lim * lim
    cfr, cfi = _cmul(a1r - 1.0, a1i, 2.0 * lre / den, -2.0 * lim / den)
    a2r, a2i = _cmul(a1r, a1i, a1r, a1i)
    a4r, a4i = _cmul(a2r, a2i, a2r, a2i)
    row = lax.broadcasted_iota(jnp.int32, (8, M), 0)
    steps = [(s, jnp.where(row >= s, ar, 0.0), jnp.where(row >= s, ai, 0.0))
             for s, ar, ai in ((1, a1r, a1i), (2, a2r, a2i), (4, a4r, a4i))]
    pwr = jnp.broadcast_to(a1r, (8, M))
    pwi = jnp.broadcast_to(a1i, (8, M))
    for s, ar, ai in ((1, a1r, a1i), (2, a2r, a2i), (4, a4r, a4i)):
        nr, ni = _cmul(pwr, pwi, ar, ai)
        on = (row & s) != 0
        pwr, pwi = jnp.where(on, nr, pwr), jnp.where(on, ni, pwi)
    b_v[2 * M:] = jnp.broadcast_to(_row(gw_ref), (16, M)).astype(BF16)

    copies[0].wait()
    copies[1].wait()
    copies[2].wait()
    copies[3].start()
    copies[4].start()
    for t in range(S // TC):
        ts = pl.ds(t * TC, TC)
        u = _dot(b_v[...], xT_v[:, ts])
        ure_v[ts, :] = u[:M].T
        uim_v[ts, :] = u[M:2 * M].T
        gT_v[:, ts] = jax.nn.sigmoid(u[2 * M:2 * M + 8])

    copies[3].wait()
    copies[4].wait()
    for cp in copies[5:]:
        cp.start()
    qscale = D ** -0.5 * math.log2(math.e)

    def wq_operands(j, slot, after):
        for c in range(2):
            dep = yield
            for e, w in enumerate(_head_pair(wq_v, j, 0, M, (c,))):
                wqT_v[slot, (2 * e + c) * 128:(2 * e + c + 1) * 128, :] = after(w.T, dep).astype(BF16)
        yield

    def c_operands(t, after):
        for lo in range(0, CR // 2, 16):
            dep = yield
            top, bot = (after(c_v[pl.ds(pl.multiple_of(t * CR + o + lo, 16), 16), :].astype(F32), dep)
                        for o in (0, CR // 2))
            dst = pl.ds(pl.multiple_of(t * (CR // 2) + lo, 16), 16)
            for a, x in enumerate(_lhs7(top[:, :DC // 2], top[:, DC // 2:], bot[:, :DC // 2], bot[:, DC // 2:])):
                ca_v[a, dst, :] = x.astype(BF16)
        yield

    def scan(j, carry, after):
        hr, hi = carry
        for a in range(TC // 16):
            ys = []
            for b in range(2):
                dep = yield
                rows = pl.ds(pl.multiple_of(j * TC + 16 * a + 8 * b, 8), 8)
                ur, ui = after(ure_v[rows, :], dep), after(uim_v[rows, :], dep)
                for s, ar, ai in steps:
                    dr, di = _cmul(pltpu.roll(ur, s, 0), pltpu.roll(ui, s, 0), ar, ai)
                    ur, ui = ur + dr, ui + di
                dr, di = _cmul(hr, hi, pwr, pwi)
                ur, ui = ur + dr, ui + di
                hr = jnp.broadcast_to(ur[7:8], (8, M))
                hi = jnp.broadcast_to(ui[7:8], (8, M))
                ys.append(_cmul(ur, ui, cfr, cfi))
            rows = pl.ds(pl.multiple_of(j * TC + 16 * a, 16), 16)
            hre_v[rows, :] = jnp.concatenate([ys[0][0], ys[1][0]], axis=0).astype(BF16)
            him_v[rows, :] = (-jnp.concatenate([ys[0][1], ys[1][1]], axis=0)).astype(BF16)
        carry[:] = hr, hi
        yield

    def q_and_scan(j, carry, with_c):
        after = _pacer(j)
        deps = []
        for t in range(S // 512):
            q = _dot(wqT_v[0], xT_v[:, t * 512:(t + 1) * 512])
            qT_v[pl.ds(pl.multiple_of(j * 2 * D, 2 * D), 2 * D), t * 512:(t + 1) * 512] = (
                q * qscale).astype(BF16)
            deps += [q[r:r + 8, c:c + 128] for c in range(0, 512, 128) for r in range(0, 512, 128)]
        carry = list(carry)
        _pace(scan(j, carry, after), TC // 8, deps, 0.0, 0.85)
        if with_c:
            _pace(c_operands(j - H // 4, after), CR // 32, deps, 0.0, 0.85)
        _pace(wq_operands(jnp.minimum(j + 1, H // 2 - 1), 1, after), 2, deps, 0.2, 0.8)
        wqT_v[0] = wqT_v[1]
        return tuple(carry)

    _pace(wq_operands(0, 0, None or (lambda x, dep: x)), 2, [None], 0.0, 1.0)
    zero = jnp.zeros((8, M), F32)
    carry = lax.fori_loop(0, H // 4, functools.partial(q_and_scan, with_c=False), (zero, zero))
    copies[5].wait()
    lax.fori_loop(H // 4, H // 2, functools.partial(q_and_scan, with_c=True), carry)

    for cp in copies[6:]:
        cp.wait()
    kk = lax.broadcasted_iota(jnp.int32, (128, BQ), 0)
    qq = lax.broadcasted_iota(jnp.int32, (128, BQ), 1)
    causal = kk <= qq

    def kv_operands(j, after):
        for t, w_ref in enumerate((wk_v, wv_v)):
            for lo in range(0, DC // 2, 32):
                dep = yield
                top, bot = ([after(w, dep) for w in _head_pair(w_ref, j, o + lo, 32)]
                            for o in (0, DC // 2))
                for a, x in enumerate(_rhs7(*top, *bot)):
                    w_v[a, lo:lo + 32, t * D:(t + 1) * D] = x.astype(BF16)
        yield

    _pace(kv_operands(0, lambda x, dep: x), DC // 32, [None], 0.0, 1.0)

    def head_pair(j, _):
        after = _pacer(j)

        def project(t):
            m = [_dot(ca_v[a, t * (CR // 2):(t + 1) * (CR // 2), :], w_v[a]) for a in range(7)]
            deps = [x[r:r + 8, c:c + 128] for x in m for c in range(0, 512, 128)
                    for r in range(0, CR // 2, 128)]
            return m, deps

        def finish(t, m):
            for col in range(0, 2 * D, 128):
                for lo in range(0, CR // 2, 32):
                    dep = yield
                    x = [y[lo:lo + 32, col:col + 128] for y in m]
                    x[0], x[1], x[2] = (after(y, dep) for y in x[:3])
                    for a, y in enumerate(_combine7(x)):
                        rows = pl.ds(t * CR + (a // 2) * (CR // 2) + lo, 32)
                        (k_v if col < D else v_v)[rows, pl.ds((a % 2) * D + col % D, 128)] = y.astype(BF16)
            yield

        def transpose_v(blocks):
            for e, r in blocks:
                for col in range(e * D, (e + 1) * D, 128):
                    dep = yield
                    y = after(v_v[r:r + 128, col:col + 128].astype(F32), dep)
                    vT_v[col:col + 128, r:r + 128] = y.T.astype(BF16)
            yield

        def out_proj(lo, hi):
            for t in range(lo, hi):
                ts = pl.ds(t * TC, TC)
                d = _dot(jnp.concatenate([woT_v[2 * j], woT_v[2 * j + 1]], axis=1),
                         qT_v[pl.ds(pl.multiple_of(j * 2 * D, 2 * D), 2 * D), ts])
                oT_v[:, ts] += d

        tasks = [(0, i) for i in range(S // BQ)] + [(1, i) for i in reversed(range(S // BQ))]
        st = [dict() for _ in tasks]

        def where(t):
            e, i = tasks[t]
            return (pl.ds(e * D, D), pl.ds(pl.multiple_of(j * 2 * D + e * D, D), D),
                    pl.ds(i * BQ, BQ), i * BQ + 128)

        def chunks(n):
            ends = list(range(0, n - 255, CK))[1:] + [n]
            return zip([0] + ends[:-1], ends)

        def colmax(x):
            return jnp.max(x.reshape(-1, 8, x.shape[1]), axis=0)

        def scores(t):
            cols, hd, qs, n = where(t)
            q = qT_v[hd, qs]
            for lo, hi in chunks(n):
                s = s0 = _dot(k_v[lo:hi, cols], q)
                if hi == n:
                    sd = jnp.where(causal, s[hi - lo - 128:], -1e30)
                    s = sd if hi - lo == 128 else jnp.concatenate([s[:hi - lo - 128], sd], axis=0)
                s_v[t % 2, lo:hi, :] = s
                m = colmax(s) if lo == 0 else jnp.maximum(m, colmax(s))
                for r in range(0, hi - lo, 32):
                    yield s0[r:r + 8, :128]
            s = _dot(k_v[n:n + 128, cols], q[:, 128:])
            yield s[:8]
            yield s[64:72]
            s = jnp.where(causal[:, :128], s, -1e30)
            s_v[t % 2, n:n + 128, 128:] = s
            st[t]["m"] = jnp.concatenate([m[:, :128], jnp.maximum(m[:, 128:], colmax(s))], axis=1)

        def softmax(t):
            n = where(t)[3]
            m = jnp.broadcast_to(jnp.max(st[t]["m"], axis=0, keepdims=True), (8, BQ))
            for rows, c in ([(pl.ds(lo, 32), 0) for lo in range(0, n, 32)]
                            + [(pl.ds(lo, 64), 128) for lo in (n, n + 64)]):
                dep = yield
                p = jnp.exp2(s_v[t % 2, rows, c:].reshape(-1, 8, BQ - c) - after(m[:, c:], dep))
                p_v[t % 2, rows, c:] = p.reshape(-1, BQ - c).astype(BF16)
                p = jnp.sum(p, axis=0)
                if c:
                    l = jnp.concatenate([l[:, :c], l[:, c:] + p], axis=1)
                else:
                    l = p if rows.start == 0 else l + p
            st[t]["l"] = l
            yield

        def context(t):
            cols, hd, qs, n = where(t)
            tail = _dot(vT_v[cols, n:n + 128], p_v[t % 2, n:n + 128, 128:])
            yield tail[:8]
            yield tail[128:136]
            for lo, hi in chunks(n):
                d = _dot(vT_v[cols, lo:hi], p_v[t % 2, lo:hi, :])
                acc = d if lo == 0 else acc + d
                k = (hi - lo) // 32
                for r in range(k):
                    yield d[r * D // k // 8 * 8:][:8, :128]
            acc = jnp.concatenate([acc[:, :128], acc[:, 128:] + tail], axis=1)
            l = jnp.sum(st[t]["l"], axis=0, keepdims=True)
            qT_v[hd, qs] = (acc * (1.0 / l)).astype(BF16)

        m, _ = project(0)
        for t in range(1, S // CR):
            m_next, deps = project(t)
            _pace(finish(t - 1, m), CR // 16, deps, 0.0, 0.9)
            if t > 1:
                _pace(transpose_v([(0, r) for r in range((t - 2) * CR, (t - 1) * CR, 128)]),
                      CR // 64, deps, 0.0, 0.9)
            m = m_next
        deps = list(scores(0))
        late = []
        for t in range(len(tasks) + 1):
            deps = list(context(t - 1)) if t > 0 else []
            if t + 1 < len(tasks):
                deps += list(scores(t + 1))
            if t < len(tasks):
                _pace(softmax(t), where(t)[3] // 32 + 2, deps, 0.0, 0.8)
            late += deps
            if t == 2:
                _pace(finish(S // CR - 1, m), CR // 16, late, 0.0, 1.0)
            if t == 3:
                _pace(transpose_v([(0, r) for r in range(S // 2, S, 128)]), 16, deps, 0.0, 0.9)
            if t == 4:
                late = []
            if t == 7:
                _pace(transpose_v([(1, r) for r in range(0, S, 128)]), 32, late, 0.0, 0.9)
                late = []
            if t == len(tasks) - 1:
                out_proj(4, S // TC)
        out_proj(0, 4)
        _pace(kv_operands(jnp.minimum(j + 1, H // 2 - 1), after), DC // 32, late, 0.0, 0.9)
        return 0

    oT_v[...] = jnp.zeros_like(oT_v)
    lax.fori_loop(0, H // 2, head_pair, 0)

    dsk = jnp.broadcast_to(_row(dsk_ref), (TC, M)).T
    outs = []
    for t in range(S // TC):
        ts = pl.ds(t * TC, TC)
        b = (_dot_nt(cre_v[...], hre_v[ts, :]) + _dot_nt(cim_v[...], him_v[ts, :])
             + xT_v[:, ts].astype(F32) * dsk)
        g = gT_v[:1, ts]
        oT_v[:, ts] = g * oT_v[:, ts] + (1.0 - g) * b
        cp = pltpu.make_async_copy(oT_v.at[:, ts], outT_hbm.at[:, ts], osems.at[t])
        cp.start()
        outs.append(cp)
    for cp in outs:
        cp.wait()


@jax.jit
def pallas_gated_mix__compressed_kv_cla__ssm_conv_s5__prompt_kernel(
    A_x: jax.Array,
    A_c_kv: jax.Array,
    A_w_q: jax.Array,
    A_w_uk: jax.Array,
    A_w_uv: jax.Array,
    A_w_o: jax.Array,
    B_x: jax.Array,
    B_Lambda_re: jax.Array,
    B_Lambda_im: jax.Array,
    B_B_re: jax.Array,
    B_B_im: jax.Array,
    B_C_re: jax.Array,
    B_C_im: jax.Array,
    B_log_dt: jax.Array,
    B_Dskip: jax.Array,
    gate_w: jax.Array,
):
    del B_x
    hbm = pl.BlockSpec(memory_space=pltpu.MemorySpace.HBM)
    vmem = pl.BlockSpec(memory_space=pltpu.MemorySpace.VMEM)
    V = pltpu.VMEM
    outT = pl.pallas_call(
        _kernel,
        in_specs=[hbm] * 6 + [vmem] * 2 + [hbm] * 4 + [vmem] * 3,
        out_specs=hbm,
        out_shape=jax.ShapeDtypeStruct((M, S), F32),
        scratch_shapes=[
            V((M, S), BF16), V((S, DC), BF16), V((2, M * H, 128), BF16), V((2, DC * H, 128), BF16),
            V((2, DC * H, 128), BF16), V((H, M, D), BF16),
            V((2 * M + 16, M), BF16), V((M, M), BF16), V((M, M), BF16),
            V((H * D, S), BF16),
            V((S, M), F32), V((S, M), F32), V((S, M), BF16), V((S, M), BF16),
            V((S, 2 * D), BF16), V((S, 2 * D), BF16), V((2 * D, S), BF16), V((8, S), F32), V((7, DC // 2, 2 * D), BF16), V((2, S, BQ), F32), V((2, S, BQ), BF16),
            V((2, 2 * D, M), BF16), V((7, S // 2, DC // 2), BF16),
            V((M, S), F32),
            pltpu.SemaphoreType.DMA((13,)), pltpu.SemaphoreType.DMA((S // TC,)),
        ],
        compiler_params=pltpu.CompilerParams(vmem_limit_bytes=120 * 1024 * 1024),
    )(A_x.reshape(S, M).T, A_c_kv.reshape(S, DC), A_w_q.reshape(M * H, D), A_w_uk.reshape(DC * H, D),
      A_w_uv.reshape(DC * H, D), A_w_o.transpose(0, 2, 1), B_Lambda_re, B_Lambda_im,
      B_B_re, B_B_im, B_C_re, B_C_im, B_log_dt, B_Dskip, gate_w)
    return outT.T.reshape(1, S, M)
```

```python
import functools
import math

import jax
import jax.numpy as jnp
from jax import lax
import jax.experimental.pallas as pl
import jax.experimental.pallas.tpu as pltpu

S, M, H, D, DC = 2048, 448, 16, 256, 1024
BQ = 256
TC = 256
QC = 512
CS, CP = 1024, 1024
QSCALE = D ** -0.5 * math.log2(math.e)
V = pltpu.VMEM
PLAN = dict(p2=[2, 2, 2, 1, 0, 0, 0, 0, 0, 0, 0, 0, 0, 0, 0, 0, 0],
            p3=[0, 0, 0, 0, 1, 1, 2, 2, 1, 0, 0, 0, 0, 0, 0, 0, 0],
            out=[0, 0, 0, 0, 0, 0, 0, 0, 0, 0, 1, 2, 3, 4, 5, 6, 7, 8],
            fin=[0, 4, 9])
CR = 512
F32, BF16 = jnp.float32, jnp.bfloat16
NT = (((1,), (1,)), ((), ()))


def _dot(a, b):
    return jnp.dot(a, b, preferred_element_type=F32)


def _dot_nt(a, b):
    return lax.dot_general(a, b, NT, preferred_element_type=F32)


def _head_pair(w_ref, j, lo, rows, halves=(0, 1)):
    cols = []
    for c in halves:
        r = w_ref.at[c].bitcast(jnp.uint32)
        if isinstance(j, int):
            w = r[pl.ds(lo * 8 + j, rows, stride=8), :]
        else:
            r = r.at[pl.ds(pl.multiple_of((j // 4) * 4, 4) + lo * 8, rows * 8 - 4)]
            w = r[pl.ds(0, rows, stride=8), :]
            for b in range(1, 4):
                w = jnp.where(j % 4 == b, r[pl.ds(b, rows, stride=8), :], w)
        cols.append(w)
    return jnp.concatenate(cols, axis=1)


def _unpair(w):
    lo = lax.bitcast_convert_type(w << 16, F32)
    hi = lax.bitcast_convert_type(w & jnp.uint32(0xFFFF0000), F32)
    return lo, hi


def _pacer(zero):
    def after(x, dep):
        bits = lax.bitcast_convert_type(dep, jnp.int32) & zero
        bits = jnp.tile(bits, (x.shape[0] // 8, -(-x.shape[1] // 128)))[:, :x.shape[1]]
        return lax.bitcast_convert_type(lax.bitcast_convert_type(x, jnp.int32) | bits, x.dtype)
    return after


def _pace(work, n, deps, lo, hi):
    next(work)
    for i in range(n):
        work.send(deps[int((lo + (hi - lo) * i / n) * len(deps))])


def _marks(x):
    y, k = x
    tiles = [(r, c) for c in range(0, y.shape[1], 128) for r in range(0, y.shape[0], 8)]
    n = len(tiles) * (k // 128) // 16
    return [y[r:r + 8, c:c + 128] for r, c in (tiles[i * len(tiles) // n] for i in range(n))]


def _lhs7(a11, a12, a21, a22):
    return a11 + a22, a21 + a22, a11, a22, a11 + a12, a21 - a11, a12 - a22


def _lhs9(a11, a12, a21, a22):
    return (*_lhs7(a11, a12, a21, a22), a12, a21)


Q11, Q12, Q21, Q22 = 2, 7, 8, 3


def _rhs7(b11, b12, b21, b22):
    return b11 + b22, b11, b12 - b22, b21 - b11, b22, b11 + b12, b21 + b22


def _combine7(m):
    return m[0] + m[3] - m[4] + m[6], m[2] + m[4], m[1] + m[3], m[0] - m[1] + m[2] + m[5]


def _cmul(ar, ai, br, bi):
    return ar * br - ai * bi, ar * bi + ai * br


def _row(ref):
    return ref[...].astype(F32).reshape(1, M)


def _kernel(xT_hbm, c_hbm, wq_hbm, wk_hbm, wv_hbm, woT_hbm, lre_ref, lim_ref,
            bre_hbm, bim_hbm, cre_hbm, cim_hbm, ldt_ref, dsk_ref, gw_ref,
            outT_hbm,
            xT_v, c_v, wq_v, wk_v, wv_v, woT_v, b_v, cre_v, cim_v,
            qT_v, hre_v, him_v, gT_v, wg_v, w_v, ca_v, oT_v, sems, osems):
    halves = lambda r: (r.at[:, :128], r.at[:, 128:])
    srcs = (xT_hbm, bre_hbm, bim_hbm, *halves(wq_hbm), c_hbm, *halves(wk_hbm), *halves(wv_hbm),
            woT_hbm, cre_hbm, cim_hbm)
    dsts = (xT_v, b_v.at[:M], b_v.at[M:2 * M], wq_v.at[0], wq_v.at[1], c_v, wk_v.at[0], wk_v.at[1],
            wv_v.at[0], wv_v.at[1], woT_v, cre_v, cim_v)
    copies = [pltpu.make_async_copy(s, d, sems.at[i]) for i, (s, d) in enumerate(zip(srcs, dsts))]
    for cp in copies[:3]:
        cp.start()

    lre, lim = _row(lre_ref), _row(lim_ref)
    dt = jnp.exp(_row(ldt_ref)).astype(BF16).astype(F32)
    mag = jnp.exp(dt * lre)
    a1r, a1i = mag * jnp.cos(dt * lim), mag * jnp.sin(dt * lim)
    den = lre * lre + lim * lim
    cfr, cfi = _cmul(a1r - 1.0, a1i, 2.0 * lre / den, -2.0 * lim / den)
    a2r, a2i = _cmul(a1r, a1i, a1r, a1i)
    a4r, a4i = _cmul(a2r, a2i, a2r, a2i)
    row = lax.broadcasted_iota(jnp.int32, (8, M), 0)
    steps = [(s, jnp.where(row >= s, ar, 0.0), jnp.where(row >= s, ai, 0.0))
             for s, ar, ai in ((1, a1r, a1i), (2, a2r, a2i), (4, a4r, a4i))]
    pwr = jnp.broadcast_to(a1r, (8, M))
    pwi = jnp.broadcast_to(a1i, (8, M))
    for s, ar, ai in ((1, a1r, a1i), (2, a2r, a2i), (4, a4r, a4i)):
        nr, ni = _cmul(pwr, pwi, ar, ai)
        on = (row & s) != 0
        pwr, pwi = jnp.where(on, nr, pwr), jnp.where(on, ni, pwi)
    b_v[2 * M:] = jnp.broadcast_to(_row(gw_ref), (16, M)).astype(BF16)

    def kv_gather(j, after):
        for t, w_ref in enumerate((wk_v, wv_v)):
            for lo in range(0, DC, 8):
                dep = yield
                wg_v[t, lo:lo + 8, :] = after(_head_pair(w_ref, j, lo, 8), dep)
        yield

    def kv_operands(read, after):
        for t in range(2):
            for lo in range(0, DC // 2, 16):
                for c in range(2):
                    dep = yield
                    top, bot = (_unpair(after(read(t, o + lo, c), dep)) for o in (0, DC // 2))
                    for a, x in enumerate(_rhs7(*top, *bot)):
                        w_v[a, lo:lo + 16, pl.ds(t * D + c * 128, 128)] = x.astype(BF16)
        yield

    def first_phase(ure_v, uim_v, xa_v, wa_v, waT_v):
        after = _pacer(lax.bitcast_convert_type(jnp.broadcast_to(mag[:, :128], (8, 128)), jnp.int32) >> 31)
        HM = M // 2

        def x_operands():
            for lo in range(0, HM, 16):
                for col in range(0, S // 2, QC // 2):
                    dep = yield
                    x = [after(xT_v[pl.ds(r + lo, 16), pl.ds(2 * col + o, QC // 2)].astype(F32), dep)
                         for r in (0, HM) for o in (0, QC // 2)]
                    for a, y in enumerate(_rhs7(*x)):
                        xa_v[a, lo:lo + 16, pl.ds(col, QC // 2)] = y.astype(BF16)
            yield

        def wq_operands(j):
            for lo in range(0, HM, 16):
                dep = yield
                (a11, a21), (a12, a22) = ([after(w, dep) for w in _unpair(_head_pair(wq_v, j, o + lo, 16))]
                                          for o in (0, HM))
                for a, x in enumerate(_lhs7(a11, a12, a21, a22)):
                    wa_v[a, lo:lo + 16, :] = x.astype(BF16)
            for a in range(7):
                for c in (0, 128):
                    dep = yield
                    y = after(wa_v[a, :, c:c + 128].astype(F32), dep)
                    waT_v[j % 2, a, c:c + 128, :] = y.T.astype(BF16)
            yield

        def q_finish(j, t, m):
            for lo in range(0, D, 16):
                dep = yield
                x = [y[lo:lo + 16] for y in m]
                x[:3] = (after(y, dep) for y in x[:3])
                for a, y in enumerate(_combine7(x)):
                    qT_v[pl.ds((2 * j + a // 2) * D + lo, 16),
                         pl.ds(t * QC + (a % 2) * (QC // 2), QC // 2)] = (y * QSCALE).astype(BF16)
            yield

        def c_operands():
            for t in range(S // CR):
                for lo in range(0, CR // 2, 16):
                    for col in range(0, DC // 2, 256):
                        dep = yield
                        x = [after(c_v[pl.ds(t * CR + r + lo, 16), pl.ds(col + o, 256)].astype(F32), dep)
                             for r in (0, CR // 2) for o in (0, DC // 2)]
                        for a, y in enumerate(_lhs7(*x)):
                            ca_v[a, pl.ds(t * (CR // 2) + lo, 16), col:col + 256] = y.astype(BF16)
            yield

        def scan():
            tiles = [slice(c, min(c + 128, M)) for c in range(0, M, 128)]
            h = [None] * len(tiles)
            for lo in range(0, S, 16):
                for n, c in enumerate(tiles):
                    ys = []
                    for r in (lo, lo + 8):
                        dep = yield
                        ur, ui = after(ure_v[r:r + 8, c], dep), after(uim_v[r:r + 8, c], dep)
                        for s, ar, ai in steps:
                            dr, di = _cmul(pltpu.roll(ur, s, 0), pltpu.roll(ui, s, 0), ar[:, c], ai[:, c])
                            ur, ui = ur + dr, ui + di
                        if r:
                            dr, di = _cmul(*h[n], pwr[:, c], pwi[:, c])
                            ur, ui = ur + dr, ui + di
                        h[n] = ur[7:8], ui[7:8]
                        ys.append(_cmul(ur, ui, cfr[:, c], cfi[:, c]))
                    hre_v[lo:lo + 16, c] = jnp.concatenate([ys[0][0], ys[1][0]], axis=0).astype(BF16)
                    him_v[lo:lo + 16, c] = (-jnp.concatenate([ys[0][1], ys[1][1]], axis=0)).astype(BF16)
            yield

        def clear_out():
            for r in range(0, M, 8):
                dep = yield
                oT_v[r:r + 8, :] = after(jnp.zeros((8, S), F32), dep)
            yield

        def project_q(pairs, pending):
            seen = []
            for j in pairs:
                for t in range(S // QC):
                    m = [_dot(waT_v[j % 2, a], xa_v[a, :, t * (QC // 2):(t + 1) * (QC // 2)])
                         for a in range(7)]
                    deps = [x[r:r + 8, :128] for x in m for r in range(0, D, 32)]
                    if pending:
                        _pace(q_finish(*pending), D // 16, deps, 0.0, 0.95)
                    pending = j, t, m
                    seen += deps
                if j + 1 < H // 2:
                    _pace(wq_operands(j + 1), HM // 16 + 14, seen[-len(deps) * (S // QC):], 0.0, 0.8)
            return pending, seen

        for cp in copies[:3]:
            cp.wait()
        for cp in copies[3:5]:
            cp.start()
        for t in range(S // TC):
            if t == S // TC - 2:
                _pace(x_operands(), HM // 16 * (S // QC), deps, 0.0, 1.0)
                for cp in copies[3:5]:
                    cp.wait()
                for cp in copies[5:]:
                    cp.start()
            if t in (0, S // TC - 2):
                deps = []
            ts = pl.ds(t * TC, TC)
            u = _dot(b_v[...], xT_v[:, ts])
            ure_v[ts, :] = u[:M].T
            uim_v[ts, :] = u[M:2 * M].T
            gT_v[:, ts] = jax.nn.sigmoid(u[2 * M:2 * M + 8])
            deps += [u[r:r + 8, c:c + 128] for c in (0, 128) for r in range(0, 2 * M, 64)]
        _pace(wq_operands(0), HM // 16 + 14, deps, 0.0, 0.8)
        pending, deps = project_q(range(6), None)
        _pace(scan(), S // 8 * 4, deps, 0.0, 0.98)
        for cp in copies[5:]:
            cp.wait()
        pending, deps = project_q(range(6, H // 2), pending)
        _pace(c_operands(), S // 32 * 2, deps, 0.0, 0.95)
        _pace(kv_operands(lambda t, r, c: _head_pair((wk_v, wv_v)[t], 0, r, 16, (c,)), after), DC // 8, deps, 0.0, 0.95)
        _pace(clear_out(), M // 8, deps, 0.0, 0.95)
        _pace(q_finish(*pending), D // 16, deps, 0.99, 0.999)

    pl.run_scoped(first_phase, V((S, M), F32), V((S, M), F32), V((7, M // 2, S // 2), BF16),
                  V((7, M // 2, D), BF16), V((2, 7, D, M // 2), BF16))

    def head_pair(j, k_v, v_v, vT_v, s_v, p_v, pd_v, o_v):
        after = _pacer(jnp.full((8, 128), j >> 4, jnp.int32))
        causal = (lax.broadcasted_iota(jnp.int32, (128, 128), 0)
                  <= lax.broadcasted_iota(jnp.int32, (128, 128), 1))

        log = []

        def dot(a, b):
            y = _dot(a, b)
            log.extend(_marks((y, a.shape[1])))
            return y

        def project(t, m, n):
            for a in range(len(m), len(m) + n):
                m.append(dot(ca_v[a, t * (CR // 2):(t + 1) * (CR // 2), :], w_v[a]))

        def finish(t, m):
            for col in (0, D):
                for lo in range(0, CR // 2, 16):
                    dep = yield
                    x = [z[lo:lo + 16, col:col + D] for z in m]
                    x[:3] = (after(z, dep) for z in x[:3])
                    for a, z in enumerate(_combine7(x)):
                        ref = v_v if col else k_v
                        ref[a % 2, pl.ds(t * CR + (a // 2) * (CR // 2) + lo, 16), :] = z.astype(ref.dtype)
            yield

        def v_operands(blocks):
            for e, b in blocks:
                tiles = [(e, pl.ds(b * 256 + r, 128), pl.ds(c, 128)) for c in (0, 128) for r in (0, 128)]
                for tile in tiles:
                    dep = yield
                    v_v[tile] = after(v_v[tile], dep).T
                for lo in range(0, 128, 16):
                    dep = yield
                    x = [after(v_v[e, pl.ds(r.start + lo, 16), c], dep) for _, r, c in tiles]
                    for n, z in enumerate(_lhs9(*x)):
                        vT_v[e, n, lo:lo + 16, b * 128:(b + 1) * 128] = z.astype(BF16)
            yield

        def out_proj(lo, hi):
            for t in range(lo, hi):
                ts = pl.ds(t * TC, TC)
                d = dot(jnp.concatenate([woT_v[2 * j], woT_v[2 * j + 1]], axis=1), o_v[:, ts])
                oT_v[:, ts] += d

        tasks = [(e, i) for i in range(S // BQ) for e in range(2)]
        st = [dict() for _ in tasks]
        chunks = lambda n, size: [(lo, min(lo + size, n)) for lo in range(0, n, size)]
        r8 = lambda x: x.reshape(-1, 8, 128)
        head = lambda e: pl.ds(pl.multiple_of(j * 2 * D + e * D, D), D)

        def scores(t):
            e, i = tasks[t]
            h = i * 128
            q = qT_v[head(e), pl.ds(i * BQ, BQ)]
            s22 = dot(k_v[e, 2 * h + 128:2 * h + 256, :], q[:, 128:])
            s22 = jnp.where(causal, s22, -1e30)
            s_v[t % 2, 3, h:h + 128, :] = s22
            m = [None, jnp.max(r8(s22), axis=0)]
            starts = list(range(0, 2 * h, CS)) or [0]
            for lo, hi in zip(starts, starts[1:] + [2 * h + 128]):
                s = dot(k_v[e, lo:hi, :], q)
                for r in range(lo, hi, 128):
                    for c in range(2):
                        x = s[r - lo:r - lo + 128, c * 128:(c + 1) * 128]
                        if r == 2 * h and c == 0:
                            x = jnp.where(causal, x, -1e30)
                        s_v[t % 2, r // 128 % 2 * 2 + c, pl.ds(r // 256 * 128, 128), :] = x
                        x = jnp.max(r8(x), axis=0)
                        m[c] = x if m[c] is None else jnp.maximum(m[c], x)
            st[t]["m"] = m

        def softmax(t):
            h = tasks[t][1] * 128
            m = [jnp.broadcast_to(jnp.max(x, axis=0, keepdims=True), (8, 128)) for x in st[t]["m"]]
            l = [0.0, 0.0]
            for lo in range(0, h + 128, 16):
                dep = yield
                mm = [after(x, dep) for x in m]
                p = {}
                for a in ((0, 1, 2, 3) if lo < h else (0, 1, 3)):
                    p[a] = jnp.exp2(r8(s_v[t % 2, a, lo:lo + 16, :]) - mm[a % 2])
                    l[a % 2] = l[a % 2] + jnp.sum(p[a], axis=0)
                if lo < h:
                    for a, x in enumerate(_rhs7(p[0], p[1], p[2], p[3])):
                        p_v[t % 2, a, lo:lo + 16, :] = x.reshape(16, 128).astype(BF16)
                else:
                    for a, x in p.items():
                        pd_v[t % 2, a // 2, pl.ds(lo - h, 16), pl.ds((a % 2) * 128, 128)] = (
                            x.reshape(16, 128).astype(BF16))
            st[t]["l"] = l
            yield

        def context(t):
            e, i = tasks[t]
            h = i * 128
            acc = None
            for lo, hi in chunks(h, CP):
                m = [dot(vT_v[e, a, :, lo:hi], p_v[t % 2, a, lo:hi, :]) for a in range(7)]
                acc = m if acc is None else [x + y for x, y in zip(acc, m)]
            d1 = dot(jnp.concatenate([vT_v[e, n, :, h:h + 128] for n in (Q11, Q21)], axis=0), pd_v[t % 2, 0])
            d2 = dot(jnp.concatenate([vT_v[e, n, :, h:h + 128] for n in (Q12, Q22)], axis=0),
                      pd_v[t % 2, 1, :, 128:])
            c = [d1[:, :128], d1[:, 128:] + d2]
            if acc:
                y = _combine7(acc)
                c = [c[a] + jnp.concatenate([y[a], y[a + 2]], axis=0) for a in range(2)]
            for a in range(2):
                l = jnp.sum(st[t]["l"][a], axis=0, keepdims=True)
                o_v[e * D:(e + 1) * D, pl.ds(i * BQ + a * 128, 128)] = (c[a] * (1.0 / l)).astype(BF16)

        m = [[] for _ in range(S // CR)]
        both = lambda *bs: [(e, b) for b in bs for e in range(2)]
        project(0, m[0], 7)
        at = len(log)
        _pace(kv_gather(jnp.minimum(j + 1, H // 2 - 1), after), DC // 4, log, 0.0, 1.0)
        project(1, m[1], 7)
        _pace(finish(0, m[0]), 32, log[at:], 0.0, 0.6)
        _pace(v_operands(both(0)), 24, log[at:], 0.6, 0.95)
        scores(0)
        start = []
        for t in range(len(tasks) + 1):
            start.append(len(log))
            if t > 0:
                context(t - 1)
            for n in range(PLAN["p2"][t]):
                project(2, m[2], 1)
            for n in range(PLAN["p3"][t]):
                project(3, m[3], 1)
            out_proj(*PLAN["out"][t:t + 2])
            if t in (3, 7, 11):
                _pace(finish(t // 4 + 1, m[t // 4 + 1]), 32, log[start[PLAN["fin"][t // 4]]:], 0.0, 0.95)
            if t + 1 < len(tasks):
                scores(t + 1)
            if t % 2 == 0 and 0 < t < len(tasks):
                _pace(v_operands(both(t // 2)), 24, log[start[t - (t % 4 == 2) - 1]:], 0.0, 0.95)
            if t < len(tasks):
                _pace(softmax(t), (tasks[t][1] + 1) * 8, log[start[t]:], 0.0, 0.9)
        _pace(kv_operands(lambda t, r, c: wg_v[t, r:r + 16, c * 128:(c + 1) * 128], after), DC // 8,
              log[start[9]:], 0.0, 0.97)

    @functools.partial(
        pl.run_scoped, k_v=V((2, S, D), BF16), v_v=V((2, S, D), F32),
        vT_v=V((2, 9, 128, S // 2), BF16), s_v=V((2, 4, S // 2, 128), F32),
        p_v=V((2, 7, S // 2, 128), BF16), pd_v=V((2, 2, 128, BQ), BF16), o_v=V((2 * D, S), BF16))
    def _(**refs):
        lax.fori_loop(0, H // 2, lambda j, c: head_pair(j, **refs), None)

    dsk = jnp.broadcast_to(_row(dsk_ref), (TC, M)).T
    outs = []
    for t in range(S // TC):
        ts = pl.ds(t * TC, TC)
        b = (_dot_nt(cre_v[...], hre_v[ts, :]) + _dot_nt(cim_v[...], him_v[ts, :])
             + xT_v[:, ts].astype(F32) * dsk)
        g = gT_v[:1, ts]
        oT_v[:, ts] = g * oT_v[:, ts] + (1.0 - g) * b
        cp = pltpu.make_async_copy(oT_v.at[:, ts], outT_hbm.at[:, ts], osems.at[t])
        cp.start()
        outs.append(cp)
    for cp in outs:
        cp.wait()


@jax.jit
def pallas_gated_mix__compressed_kv_cla__ssm_conv_s5__prompt_kernel(
    A_x: jax.Array,
    A_c_kv: jax.Array,
    A_w_q: jax.Array,
    A_w_uk: jax.Array,
    A_w_uv: jax.Array,
    A_w_o: jax.Array,
    B_x: jax.Array,
    B_Lambda_re: jax.Array,
    B_Lambda_im: jax.Array,
    B_B_re: jax.Array,
    B_B_im: jax.Array,
    B_C_re: jax.Array,
    B_C_im: jax.Array,
    B_log_dt: jax.Array,
    B_Dskip: jax.Array,
    gate_w: jax.Array,
):
    del B_x
    hbm = pl.BlockSpec(memory_space=pltpu.MemorySpace.HBM)
    vmem = pl.BlockSpec(memory_space=pltpu.MemorySpace.VMEM)
    outT = pl.pallas_call(
        _kernel,
        in_specs=[hbm] * 6 + [vmem] * 2 + [hbm] * 4 + [vmem] * 3,
        out_specs=hbm,
        out_shape=jax.ShapeDtypeStruct((M, S), F32),
        scratch_shapes=[
            V((M, S), BF16), V((S, DC), BF16), V((2, M * H, 128), BF16), V((2, DC * H, 128), BF16),
            V((2, DC * H, 128), BF16), V((H, M, D), BF16),
            V((2 * M + 16, M), BF16), V((M, M), BF16), V((M, M), BF16),
            V((H * D, S), BF16), V((S, M), BF16), V((S, M), BF16), V((8, S), F32),
            V((2, DC, D), jnp.uint32),
            V((7, DC // 2, 2 * D), BF16), V((7, S // 2, DC // 2), BF16), V((M, S), F32),
            pltpu.SemaphoreType.DMA((13,)), pltpu.SemaphoreType.DMA((S // TC,)),
        ],
        compiler_params=pltpu.CompilerParams(vmem_limit_bytes=120 * 1024 * 1024),
    )(A_x.reshape(S, M).T, A_c_kv.reshape(S, DC), A_w_q.reshape(M * H, D), A_w_uk.reshape(DC * H, D),
      A_w_uv.reshape(DC * H, D), A_w_o.transpose(0, 2, 1), B_Lambda_re, B_Lambda_im,
      B_B_re, B_B_im, B_C_re, B_C_im, B_log_dt, B_Dskip, gate_w)
    return outT.T.reshape(1, S, M)
```

```python
import functools
import math

import jax
import jax.numpy as jnp
from jax import lax
import jax.experimental.pallas as pl
import jax.experimental.pallas.tpu as pltpu

S, M, H, D, DC = 2048, 448, 16, 256, 1024
BQ = 256
TC = 256
QC = 512
CS, CP = 1024, 1024
QSCALE = D ** -0.5 * math.log2(math.e)
V = pltpu.VMEM
PLAN = dict(p2=[3, 2, 2, 0, 0, 0, 0, 0, 0, 0, 0, 0, 0, 0, 0, 0, 0],
            p3=[0, 0, 0, 2, 2, 2, 1, 0, 0, 0, 0, 0, 0, 0, 0, 0, 0],
            out=[0, 0, 0, 0, 0, 0, 0, 0, 1, 2, 3, 4, 4, 5, 5, 6, 7, 8],
            fin=[0, 3, 7])
CR = 512
F32, BF16 = jnp.float32, jnp.bfloat16
NT = (((1,), (1,)), ((), ()))


def _tiled(*shape):
    return V((*shape[:-2], shape[-1] // 128, shape[-2], 128), BF16)


class _Tiled:
    def __init__(self, ref):
        self.ref = ref

    def _split(self, idx):
        *lead, rows, cols = idx
        if isinstance(cols, slice):
            lo, hi, _ = cols.indices(self.ref.shape[-3] * 128)
        else:
            lo, hi = cols.start, cols.start + cols.size
        return [(*lead, c, rows, slice(None)) for c in range(lo // 128, hi // 128)]

    def __getitem__(self, idx):
        return jnp.concatenate([self.ref[i] for i in self._split(idx)], axis=1)

    def __setitem__(self, idx, value):
        for n, i in enumerate(self._split(idx)):
            self.ref[i] = value[:, n * 128:(n + 1) * 128]


def _dot(a, b):
    return jnp.dot(a, b, preferred_element_type=F32)


def _dot_nt(a, b):
    return lax.dot_general(a, b, NT, preferred_element_type=F32)


def _head_pair(w_ref, j, lo, rows, halves=(0, 1)):
    cols = []
    for c in halves:
        r = w_ref.at[c].bitcast(jnp.uint32)
        if isinstance(j, int):
            w = r[pl.ds(lo * 8 + j, rows, stride=8), :]
        else:
            i, odd = j
            r = r.at[pl.ds(pl.multiple_of((i // 2) * 4, 4) + lo * 8, rows * 8 - 4)]
            w = jnp.where(i % 2 == 0, r[pl.ds(odd, rows, stride=8), :],
                          r[pl.ds(odd + 2, rows, stride=8), :])
        cols.append(w)
    return jnp.concatenate(cols, axis=1)


def _unpair(w):
    lo = lax.bitcast_convert_type(w << 16, F32)
    hi = lax.bitcast_convert_type(w & jnp.uint32(0xFFFF0000), F32)
    return lo, hi


def _pacer(zero):
    def after(x, dep):
        bits = lax.bitcast_convert_type(dep, jnp.int32) & zero
        bits = jnp.tile(bits, (x.shape[0] // 8, -(-x.shape[1] // 128)))[:, :x.shape[1]]
        return lax.bitcast_convert_type(lax.bitcast_convert_type(x, jnp.int32) | bits, x.dtype)
    return after


def _pace(work, n, deps, lo, hi, started=False):
    if not started:
        next(work)
    for i in range(n):
        work.send(deps[int((lo + (hi - lo) * i / n) * len(deps))])


def _marks(x):
    y, k = x
    tiles = [(r, c) for c in range(0, y.shape[1], 128) for r in range(0, y.shape[0], 8)]
    n = len(tiles) * (k // 128) // 16
    return [y[r:r + 8, c:c + 128] for r, c in (tiles[i * len(tiles) // n] for i in range(n))]


def _lhs7(a11, a12, a21, a22):
    return a11 + a22, a21 + a22, a11, a22, a11 + a12, a21 - a11, a12 - a22


def _lhs9(a11, a12, a21, a22):
    return (*_lhs7(a11, a12, a21, a22), a12, a21)


Q11, Q12, Q21, Q22 = 2, 7, 8, 3


def _rhs7(b11, b12, b21, b22):
    return b11 + b22, b11, b12 - b22, b21 - b11, b22, b11 + b12, b21 + b22


def _combine7(m):
    return m[0] + m[3] - m[4] + m[6], m[2] + m[4], m[1] + m[3], m[0] - m[1] + m[2] + m[5]


def _cmul(ar, ai, br, bi):
    return ar * br - ai * bi, ar * bi + ai * br


def _row(ref):
    return ref[...].astype(F32).reshape(1, M)


def _kernel(xT_hbm, c_hbm, wq_hbm, wk_hbm, wv_hbm, woT_hbm, lre_ref, lim_ref,
            bre_hbm, bim_hbm, cre_hbm, cim_hbm, ldt_ref, dsk_ref, gw_ref,
            outT_hbm,
            xT_v, c_v, wq_v, wk_v, wv_v, woT_v, b_v, cre_v, cim_v,
            qT_v, hre_v, him_v, gT_v, wg_v, wk7_v, wv49_v, ca_v, oT_v, sems, osems):
    halves = lambda r: (r.at[:, :128], r.at[:, 128:])
    srcs = (xT_hbm, bre_hbm, bim_hbm, *halves(wq_hbm), c_hbm, *halves(wk_hbm), *halves(wv_hbm),
            woT_hbm.at[:, :, :128], woT_hbm.at[:, :, 128:], cre_hbm, cim_hbm)
    dsts = (xT_v, b_v.at[:M], b_v.at[M:2 * M], wq_v.at[0], wq_v.at[1], c_v, wk_v.at[0], wk_v.at[1],
            wv_v.at[0], wv_v.at[1], woT_v.at[:, 0], woT_v.at[:, 1], cre_v, cim_v)
    copies = [pltpu.make_async_copy(s, d, sems.at[i]) for i, (s, d) in enumerate(zip(srcs, dsts))]
    for cp in copies:
        cp.start()
    woT_v, qT_v, wk7_v, ca_v = map(_Tiled, (woT_v, qT_v, wk7_v, ca_v))

    lre, lim = _row(lre_ref), _row(lim_ref)
    dt = jnp.exp(_row(ldt_ref)).astype(BF16).astype(F32)
    mag = jnp.exp(dt * lre)
    a1r, a1i = mag * jnp.cos(dt * lim), mag * jnp.sin(dt * lim)
    den = lre * lre + lim * lim
    cfr, cfi = _cmul(a1r - 1.0, a1i, 2.0 * lre / den, -2.0 * lim / den)
    a2r, a2i = _cmul(a1r, a1i, a1r, a1i)
    a4r, a4i = _cmul(a2r, a2i, a2r, a2i)
    row = lax.broadcasted_iota(jnp.int32, (8, M), 0)
    steps = [(s, jnp.where(row >= s, ar, 0.0), jnp.where(row >= s, ai, 0.0))
             for s, ar, ai in ((1, a1r, a1i), (2, a2r, a2i), (4, a4r, a4i))]
    pwr = jnp.broadcast_to(a1r, (8, M))
    pwi = jnp.broadcast_to(a1i, (8, M))
    for s, ar, ai in ((1, a1r, a1i), (2, a2r, a2i), (4, a4r, a4i)):
        nr, ni = _cmul(pwr, pwi, ar, ai)
        on = (row & s) != 0
        pwr, pwi = jnp.where(on, nr, pwr), jnp.where(on, ni, pwi)
    b_v[2 * M:] = jnp.broadcast_to(_row(gw_ref), (16, M)).astype(BF16)

    def kv_gather(j, after):
        for t, w_ref in enumerate((wk_v, wv_v)):
            for lo in range(0, DC, 8):
                dep = yield
                wg_v[t, lo:lo + 8, :] = after(_head_pair(w_ref, j, lo, 8), dep)
        yield

    def kv_operands(read, after):
        for lo in range(0, DC // 2, 16):
            for c in range(2):
                dep = yield
                top, bot = (_unpair(after(read(0, o + lo, c), dep)) for o in (0, DC // 2))
                for a, x in enumerate(_rhs7(*top, *bot)):
                    wk7_v[a, lo:lo + 16, pl.ds(c * 128, 128)] = x.astype(BF16)
        for lo in range(0, DC // 4, 16):
            dep = yield
            x = [_rhs7(*(w for o in (0, DC // 2) for w in _unpair(after(read(1, o + r + lo, c), dep))))
                 for r in (0, DC // 4) for c in range(2)]
            for a in range(7):
                dep = yield
                y = [z[a] for z in x]
                for b, z in enumerate(_rhs7(after(y[0], dep), y[1], y[2], after(y[3], dep))):
                    wv49_v[a, b, lo:lo + 16, :] = z.astype(BF16)
        yield

    def first_phase(ure_v, uim_v, xa_v, wa_v, waT_v):
        after = _pacer(lax.bitcast_convert_type(jnp.broadcast_to(mag[:, :128], (8, 128)), jnp.int32) >> 31)
        HM = M // 2
        xa_v = _Tiled(xa_v)

        def x_operands():
            for lo in range(0, HM, 16):
                for col in range(0, S // 2, QC // 2):
                    dep = yield
                    x = [after(xT_v[pl.ds(r + lo, 16), pl.ds(2 * col + o, QC // 2)].astype(F32), dep)
                         for r in (0, HM) for o in (0, QC // 2)]
                    for a, y in enumerate(_rhs7(*x)):
                        xa_v[a, lo:lo + 16, pl.ds(col, QC // 2)] = y.astype(BF16)
            yield

        def wq_operands(j):
            for lo in range(0, HM, 16):
                dep = yield
                (a11, a21), (a12, a22) = ([after(w, dep) for w in _unpair(_head_pair(wq_v, j, o + lo, 16))]
                                          for o in (0, HM))
                for a, x in enumerate(_lhs7(a11, a12, a21, a22)):
                    wa_v[a, lo:lo + 16, :] = x.astype(BF16)
            for a in range(7):
                for c in (0, 128):
                    dep = yield
                    y = after(wa_v[a, :, c:c + 128].astype(F32), dep)
                    waT_v[j % 2, a, c:c + 128, :] = y.T.astype(BF16)
            yield

        def q_finish(j, t, m):
            for lo in range(0, D, 16):
                dep = yield
                x = [y[lo:lo + 16] for y in m]
                x[:3] = (after(y, dep) for y in x[:3])
                for a, y in enumerate(_combine7(x)):
                    qT_v[pl.ds((2 * j + a // 2) * D + lo, 16),
                         pl.ds(t * QC + (a % 2) * (QC // 2), QC // 2)] = (y * QSCALE).astype(BF16)
            yield

        def c_operands():
            for t in range(S // CR):
                for lo in range(0, CR // 4, 16):
                    for col in range(0, DC // 4, 128):
                        dep = yield
                        x = [_lhs7(*(after(c_v[pl.ds(t * CR + r1 + r2 + lo, 16),
                                               pl.ds(c1 + c2 + col, 128)].astype(F32), dep)
                                     for r1 in (0, CR // 2) for c1 in (0, DC // 2)))
                             for r2 in (0, CR // 4) for c2 in (0, DC // 4)]
                        for a in range(7):
                            dep = yield
                            y = [z[a] for z in x]
                            for b, z in enumerate(_lhs9(after(y[0], dep), y[1], y[2], after(y[3], dep))):
                                ca_v[a, b, pl.ds(t * (CR // 4) + lo, 16), col:col + 128] = z.astype(BF16)
            yield

        def scan():
            tiles = [slice(c, min(c + 128, M)) for c in range(0, M, 128)]
            h = [None] * len(tiles)
            for lo in range(0, S, 16):
                for n, c in enumerate(tiles):
                    ys = []
                    for r in (lo, lo + 8):
                        dep = yield
                        ur, ui = after(ure_v[r:r + 8, c], dep), after(uim_v[r:r + 8, c], dep)
                        for s, ar, ai in steps:
                            dr, di = _cmul(pltpu.roll(ur, s, 0), pltpu.roll(ui, s, 0), ar[:, c], ai[:, c])
                            ur, ui = ur + dr, ui + di
                        if r:
                            dr, di = _cmul(*h[n], pwr[:, c], pwi[:, c])
                            ur, ui = ur + dr, ui + di
                        h[n] = ur[7:8], ui[7:8]
                        ys.append(_cmul(ur, ui, cfr[:, c], cfi[:, c]))
                    hre_v[lo:lo + 16, c] = jnp.concatenate([ys[0][0], ys[1][0]], axis=0).astype(BF16)
                    him_v[lo:lo + 16, c] = (-jnp.concatenate([ys[0][1], ys[1][1]], axis=0)).astype(BF16)
            yield

        def clear_out():
            for r in range(0, M, 8):
                dep = yield
                oT_v[r:r + 8, :] = after(jnp.zeros((8, S), F32), dep)
            yield

        def project_q(pairs, pending):
            seen = []
            for j in pairs:
                for t in range(S // QC):
                    m = [_dot(waT_v[j % 2, a], xa_v[a, :, t * (QC // 2):(t + 1) * (QC // 2)])
                         for a in range(7)]
                    deps = [x[r:r + 8, :128] for x in m for r in range(0, D, 32)]
                    if pending:
                        _pace(q_finish(*pending), D // 16, deps, 0.0, 0.95)
                    pending = j, t, m
                    seen += deps
                if j + 1 < H // 2:
                    _pace(wq_operands(j + 1), HM // 16 + 14, seen[-len(deps) * (S // QC):], 0.0, 0.8)
            return pending, seen

        for cp in copies[:3]:
            cp.wait()
        for t in range(S // TC):
            if t == S // TC - 2:
                _pace(x_operands(), HM // 16 * (S // QC), deps, 0.0, 1.0)
                for cp in copies[3:5]:
                    cp.wait()
            if t in (0, S // TC - 2):
                deps = []
            ts = pl.ds(t * TC, TC)
            u = _dot(b_v[...], xT_v[:, ts])
            ure_v[ts, :] = u[:M].T
            uim_v[ts, :] = u[M:2 * M].T
            gT_v[:, ts] = jax.nn.sigmoid(u[2 * M:2 * M + 8])
            deps += [u[r:r + 8, c:c + 128] for c in (0, 128) for r in range(0, 2 * M, 64)]
        _pace(wq_operands(0), HM // 16 + 14, deps, 0.0, 0.8)
        pending, deps = project_q(range(1), None)
        _pace(clear_out(), M // 8, deps, 0.0, 0.95)
        work = scan()
        _pace(work, S // 16, deps, 0.0, 0.98)
        copies[5].wait()
        pending, deps = project_q(range(1, 7), pending)
        _pace(work, S // 16 * 6, deps, 0.0, 0.99, True)
        _pace(c_operands(), S // 64 * 16, deps, 0.0, 0.99)
        for cp in copies[6:10]:
            cp.wait()
        pending, deps = project_q(range(7, H // 2), pending)
        _pace(work, S // 16, deps, 0.0, 0.95, True)
        _pace(kv_operands(lambda t, r, c: _head_pair((wk_v, wv_v)[t], 0, r, 16, (c,)), after),
              DC // 16 + DC // 8, deps, 0.0, 0.95)
        _pace(q_finish(*pending), D // 16, deps, 0.99, 0.999)

    pl.run_scoped(first_phase, V((S, M), F32), V((S, M), F32), _tiled(7, M // 2, S // 2),
                  V((7, M // 2, D), BF16), V((2, 7, D, M // 2), BF16))

    for cp in copies[10:]:
        cp.wait()

    def head_pair(j, j_next, k_v, v_v, vT_v, s_v, p_v, pd_v, o_v):
        after = _pacer(jnp.full((8, 128), j >> 4, jnp.int32))
        k_v, vT_v, pd_v, o_v = map(_Tiled, (k_v, vT_v, pd_v, o_v))
        causal = (lax.broadcasted_iota(jnp.int32, (128, 128), 0)
                  <= lax.broadcasted_iota(jnp.int32, (128, 128), 1))

        log = []

        def dot(a, b):
            y = _dot(a, b)
            log.extend(_marks((y, a.shape[1])))
            return y

        def project(t, m, n):
            for a in range(len(m), len(m) + n):
                c = [ca_v[a, b, t * (CR // 4):(t + 1) * (CR // 4), :] for b in range(9)]
                full = jnp.concatenate([jnp.concatenate([c[Q11], c[Q12]], axis=1),
                                        jnp.concatenate([c[Q21], c[Q22]], axis=1)], axis=0)
                m.append((dot(full, wk7_v[a, :, :]), [dot(c[b], wv49_v[a, b]) for b in range(7)]))

        def finish(t, m):
            for lo in range(0, CR // 2, 16):
                dep = yield
                x = [z[lo:lo + 16] for z, _ in m]
                x[:3] = (after(z, dep) for z in x[:3])
                for a, z in enumerate(_combine7(x)):
                    k_v[a % 2, pl.ds(t * CR + (a // 2) * (CR // 2) + lo, 16), :] = z.astype(BF16)
            for lo in range(0, CR // 4, 8):
                dep = yield
                y = []
                for _, z in m:
                    x = [u[lo:lo + 8] for u in z]
                    x[:3] = (after(u, dep) for u in x[:3])
                    y.append(_combine7(x))
                for b in range(4):
                    for a, z in enumerate(_combine7([u[b] for u in y])):
                        v_v[a % 2, pl.ds(t * CR + (a // 2) * (CR // 2) + (b // 2) * (CR // 4) + lo, 8),
                            pl.ds((b % 2) * 128, 128)] = z
            yield

        def v_operands(blocks):
            for e, b in blocks:
                tiles = [(e, pl.ds(b * 256 + r, 128), pl.ds(c, 128)) for c in (0, 128) for r in (0, 128)]
                for tile in tiles:
                    dep = yield
                    v_v[tile] = after(v_v[tile], dep).T
                for lo in range(0, 128, 16):
                    dep = yield
                    x = [after(v_v[e, pl.ds(r.start + lo, 16), c], dep) for _, r, c in tiles]
                    for n, z in enumerate(_lhs9(*x)):
                        vT_v[e, n, lo:lo + 16, b * 128:(b + 1) * 128] = z.astype(BF16)
            yield

        def out_proj(lo, hi):
            for t in range(lo, hi):
                ts = pl.ds(t * TC, TC)
                d = dot(jnp.concatenate([woT_v[2 * j + e, :, :] for e in range(2)], axis=1), o_v[:, ts])
                oT_v[:, ts] += d

        tasks = [(e, i) for i in range(S // BQ) for e in range(2)]
        st = [dict() for _ in tasks]
        chunks = lambda n, size: [(lo, min(lo + size, n)) for lo in range(0, n, size)]
        r8 = lambda x: x.reshape(-1, 8, 128)
        head = lambda e: pl.ds(pl.multiple_of(j * 2 * D + e * D, D), D)

        def scores(t):
            e, i = tasks[t]
            h = i * 128
            q = qT_v[head(e), pl.ds(i * BQ, BQ)]
            s22 = dot(k_v[e, 2 * h + 128:2 * h + 256, :], q[:, 128:])
            s22 = jnp.where(causal, s22, -1e30)
            s_v[t % 2, 3, h:h + 128, :] = s22
            m = [None, jnp.max(r8(s22), axis=0)]
            starts = list(range(0, 2 * h, CS)) or [0]
            for lo, hi in zip(starts, starts[1:] + [2 * h + 128]):
                s = dot(k_v[e, lo:hi, :], q)
                for r in range(lo, hi, 128):
                    for c in range(2):
                        x = s[r - lo:r - lo + 128, c * 128:(c + 1) * 128]
                        if r == 2 * h and c == 0:
                            x = jnp.where(causal, x, -1e30)
                        s_v[t % 2, r // 128 % 2 * 2 + c, pl.ds(r // 256 * 128, 128), :] = x
                        x = jnp.max(r8(x), axis=0)
                        m[c] = x if m[c] is None else jnp.maximum(m[c], x)
            st[t]["m"] = m

        def softmax(t):
            h = tasks[t][1] * 128
            m = [jnp.broadcast_to(jnp.max(x, axis=0, keepdims=True), (8, 128)) for x in st[t]["m"]]
            l = [0.0, 0.0]
            for lo in range(0, h + 128, 16):
                dep = yield
                mm = [after(x, dep) for x in m]
                p = {}
                for a in ((0, 1, 2, 3) if lo < h else (0, 1, 3)):
                    p[a] = jnp.exp2(r8(s_v[t % 2, a, lo:lo + 16, :]) - mm[a % 2])
                    l[a % 2] = l[a % 2] + jnp.sum(p[a], axis=0)
                if lo < h:
                    for a, x in enumerate(_rhs7(p[0], p[1], p[2], p[3])):
                        p_v[t % 2, a, lo:lo + 16, :] = x.reshape(16, 128).astype(BF16)
                else:
                    for a, x in p.items():
                        pd_v[t % 2, a // 2, pl.ds(lo - h, 16), pl.ds((a % 2) * 128, 128)] = (
                            x.reshape(16, 128).astype(BF16))
            st[t]["l"] = l
            yield

        def context(t):
            e, i = tasks[t]
            h = i * 128
            acc = None
            for lo, hi in chunks(h, CP):
                m = [dot(vT_v[e, a, :, lo:hi], p_v[t % 2, a, lo:hi, :]) for a in range(7)]
                acc = m if acc is None else [x + y for x, y in zip(acc, m)]
            d1 = dot(jnp.concatenate([vT_v[e, n, :, h:h + 128] for n in (Q11, Q21)], axis=0), pd_v[t % 2, 0, :, :])
            d2 = dot(jnp.concatenate([vT_v[e, n, :, h:h + 128] for n in (Q12, Q22)], axis=0),
                      pd_v[t % 2, 1, :, 128:])
            c = [d1[:, :128], d1[:, 128:] + d2]
            if acc:
                y = _combine7(acc)
                c = [c[a] + jnp.concatenate([y[a], y[a + 2]], axis=0) for a in range(2)]
            for a in range(2):
                l = jnp.sum(st[t]["l"][a], axis=0, keepdims=True)
                o_v[e * D:(e + 1) * D, pl.ds(i * BQ + a * 128, 128)] = (c[a] * (1.0 / l)).astype(BF16)

        m = [[] for _ in range(S // CR)]
        both = lambda *bs: [(e, b) for b in bs for e in range(2)]
        project(0, m[0], 7)
        at = len(log)
        _pace(kv_gather(j_next, after), DC // 4, log, 0.0, 1.0)
        project(1, m[1], 7)
        _pace(finish(0, m[0]), 32, log[at:], 0.0, 0.6)
        _pace(v_operands(both(0)), 24, log[at:], 0.6, 0.95)
        scores(0)
        start = []
        for t in range(len(tasks) + 1):
            start.append(len(log))
            if t > 0:
                context(t - 1)
            for n in range(PLAN["p2"][t]):
                project(2, m[2], 1)
            for n in range(PLAN["p3"][t]):
                project(3, m[3], 1)
            out_proj(*PLAN["out"][t:t + 2])
            if t in (3, 7, 11):
                _pace(finish(t // 4 + 1, m[t // 4 + 1]), 32, log[start[PLAN["fin"][t // 4]]:], 0.0, 0.95)
            if t + 1 < len(tasks):
                scores(t + 1)
            if t % 2 == 0 and 0 < t < len(tasks):
                _pace(v_operands(both(t // 2)), 24, log[start[t - (t % 4 == 2) - 1]:], 0.0, 0.95)
            if t < len(tasks):
                _pace(softmax(t), (tasks[t][1] + 1) * 8, log[start[t]:], 0.0, 0.9)
        _pace(kv_operands(lambda t, r, c: wg_v[t, r:r + 16, c * 128:(c + 1) * 128], after),
              DC // 16 + DC // 8,              log[start[PLAN["fin"][2]]:], 0.0, 0.97)

    @functools.partial(
        pl.run_scoped, k_v=_tiled(2, S, D), v_v=V((2, S, D), F32),
        vT_v=_tiled(2, 9, 128, S // 2), s_v=V((2, 4, S // 2, 128), F32),
        p_v=V((2, 7, S // 2, 128), BF16), pd_v=_tiled(2, 2, 128, BQ), o_v=_tiled(2 * D, S))
    def _(**refs):
        def two_pairs(i, _):
            head_pair(2 * i, (i, 1), **refs)
            head_pair(2 * i + 1, (jnp.minimum(i + 1, H // 4 - 1), 0), **refs)

        lax.fori_loop(0, H // 4, two_pairs, None)

    dsk = jnp.broadcast_to(_row(dsk_ref), (TC, M)).T
    outs = []
    for t in range(S // TC):
        ts = pl.ds(t * TC, TC)
        b = (_dot_nt(cre_v[...], hre_v[ts, :]) + _dot_nt(cim_v[...], him_v[ts, :])
             + xT_v[:, ts].astype(F32) * dsk)
        g = gT_v[:1, ts]
        oT_v[:, ts] = g * oT_v[:, ts] + (1.0 - g) * b
        cp = pltpu.make_async_copy(oT_v.at[:, ts], outT_hbm.at[:, ts], osems.at[t])
        cp.start()
        outs.append(cp)
    for cp in outs:
        cp.wait()


@jax.jit
def pallas_gated_mix__compressed_kv_cla__ssm_conv_s5__prompt_kernel(
    A_x: jax.Array,
    A_c_kv: jax.Array,
    A_w_q: jax.Array,
    A_w_uk: jax.Array,
    A_w_uv: jax.Array,
    A_w_o: jax.Array,
    B_x: jax.Array,
    B_Lambda_re: jax.Array,
    B_Lambda_im: jax.Array,
    B_B_re: jax.Array,
    B_B_im: jax.Array,
    B_C_re: jax.Array,
    B_C_im: jax.Array,
    B_log_dt: jax.Array,
    B_Dskip: jax.Array,
    gate_w: jax.Array,
):
    del B_x
    hbm = pl.BlockSpec(memory_space=pltpu.MemorySpace.HBM)
    vmem = pl.BlockSpec(memory_space=pltpu.MemorySpace.VMEM)
    outT = pl.pallas_call(
        _kernel,
        in_specs=[hbm] * 6 + [vmem] * 2 + [hbm] * 4 + [vmem] * 3,
        out_specs=hbm,
        out_shape=jax.ShapeDtypeStruct((M, S), F32),
        scratch_shapes=[
            V((M, S), BF16), V((S, DC), BF16), V((2, M * H, 128), BF16), V((2, DC * H, 128), BF16),
            V((2, DC * H, 128), BF16), _tiled(H, M, D),
            V((2 * M + 16, M), BF16), V((M, M), BF16), V((M, M), BF16),
            _tiled(H * D, S), V((S, M), BF16), V((S, M), BF16), V((8, S), F32),
            V((2, DC, D), jnp.uint32),
            _tiled(7, DC // 2, D), V((7, 7, DC // 4, D // 2), BF16),
            _tiled(7, 9, S // 4, DC // 4), V((M, S), F32),
            pltpu.SemaphoreType.DMA((14,)), pltpu.SemaphoreType.DMA((S // TC,)),
        ],
        compiler_params=pltpu.CompilerParams(vmem_limit_bytes=126 * 1024 * 1024),
    )(A_x.reshape(S, M).T, A_c_kv.reshape(S, DC), A_w_q.reshape(M * H, D), A_w_uk.reshape(DC * H, D),
      A_w_uv.reshape(DC * H, D), A_w_o.transpose(0, 2, 1), B_Lambda_re, B_Lambda_im,
      B_B_re, B_B_im, B_C_re, B_C_im, B_log_dt, B_Dskip, gate_w)
    return outT.T.reshape(1, S, M)
```

```python
import functools
import math

import jax
import jax.numpy as jnp
from jax import lax
import jax.experimental.pallas as pl
import jax.experimental.pallas.tpu as pltpu

S, M, H, D, DC = 2048, 448, 16, 256, 1024
BQ = 256
TC = 256
QC = 512
CS, CP = 1024, 1024
QSCALE = D ** -0.5 * math.log2(math.e)
V = pltpu.VMEM
PLAN = dict(p2=[3, 2, 2, 0, 0, 0, 0, 0, 0, 0, 0, 0, 0, 0, 0, 0, 0],
            p3=[0, 0, 0, 2, 2, 2, 1, 0, 0, 0, 0, 0, 0, 0, 0, 0, 0],
            out=[0, 0, 0, 0, 0, 0, 0, 0, 1, 2, 3, 4, 4, 5, 5, 6, 7, 8],
            fin=[0, 3, 7])
CR = 512
F32, BF16 = jnp.float32, jnp.bfloat16
NT = (((1,), (1,)), ((), ()))


def _tiled(*shape):
    return V((*shape[:-2], shape[-1] // 128, shape[-2], 128), BF16)


class _Tiled:
    def __init__(self, ref):
        self.ref = ref

    def _split(self, idx):
        *lead, rows, cols = idx
        if isinstance(cols, slice):
            lo, hi, _ = cols.indices(self.ref.shape[-3] * 128)
        else:
            lo, hi = cols.start, cols.start + cols.size
        return [(*lead, c, rows, slice(None)) for c in range(lo // 128, hi // 128)]

    def __getitem__(self, idx):
        return jnp.concatenate([self.ref[i] for i in self._split(idx)], axis=1)

    def __setitem__(self, idx, value):
        for n, i in enumerate(self._split(idx)):
            self.ref[i] = value[:, n * 128:(n + 1) * 128]


def _dot(a, b):
    return jnp.dot(a, b, preferred_element_type=F32)


def _dot_nt(a, b):
    return lax.dot_general(a, b, NT, preferred_element_type=F32)


def _head_pair(w_ref, j, lo, rows, halves=(0, 1)):
    cols = []
    for c in halves:
        r = w_ref.at[c].bitcast(jnp.uint32)
        if isinstance(j, int):
            w = r[pl.ds(lo * 8 + j, rows, stride=8), :]
        else:
            i, odd = j
            r = r.at[pl.ds(pl.multiple_of((i // 2) * 4, 4) + lo * 8, rows * 8 - 4)]
            w = jnp.where(i % 2 == 0, r[pl.ds(odd, rows, stride=8), :],
                          r[pl.ds(odd + 2, rows, stride=8), :])
        cols.append(w)
    return jnp.concatenate(cols, axis=1)


def _unpair(w):
    lo = lax.bitcast_convert_type(w << 16, F32)
    hi = lax.bitcast_convert_type(w & jnp.uint32(0xFFFF0000), F32)
    return lo, hi


def _pacer(zero):
    def after(x, dep):
        bits = lax.bitcast_convert_type(dep, jnp.int32) & zero
        bits = jnp.tile(bits, (x.shape[0] // 8, -(-x.shape[1] // 128)))[:, :x.shape[1]]
        return lax.bitcast_convert_type(lax.bitcast_convert_type(x, jnp.int32) | bits, x.dtype)
    return after


def _pace(work, n, deps, lo, hi, started=False):
    if not started:
        next(work)
    for i in range(n):
        work.send(deps[int((lo + (hi - lo) * i / n) * len(deps))])


def _marks(x):
    y, k = x
    tiles = [(r, c) for c in range(0, y.shape[1], 128) for r in range(0, y.shape[0], 8)]
    n = len(tiles) * (k // 128) // 16
    return [y[r:r + 8, c:c + 128] for r, c in (tiles[i * len(tiles) // n] for i in range(n))]


def _lhs7(a11, a12, a21, a22):
    return a11 + a22, a21 + a22, a11, a22, a11 + a12, a21 - a11, a12 - a22


def _lhs9(a11, a12, a21, a22):
    return (*_lhs7(a11, a12, a21, a22), a12, a21)


Q11, Q12, Q21, Q22 = 2, 7, 8, 3


def _rhs7(b11, b12, b21, b22):
    return b11 + b22, b11, b12 - b22, b21 - b11, b22, b11 + b12, b21 + b22


def _combine7(m):
    return m[0] + m[3] - m[4] + m[6], m[2] + m[4], m[1] + m[3], m[0] - m[1] + m[2] + m[5]


def _cmul(ar, ai, br, bi):
    return ar * br - ai * bi, ar * bi + ai * br


def _row(ref):
    return ref[...].astype(F32).reshape(1, M)


def _kernel(xT_hbm, c_hbm, wq_hbm, wk_hbm, wv_hbm, woT_hbm, lre_hbm, lim_hbm,
            bre_hbm, bim_hbm, cre_hbm, cim_hbm, ldt_hbm, dsk_hbm, gw_hbm,
            outT_hbm,
            xT_v, c_v, wq_v, wk_v, wv_v, woT_v, b_v, cre_v, cim_v,
            lre_ref, lim_ref, ldt_ref, dsk_ref, gw_ref,
            qT_v, hre_v, him_v, gT_v, wg_v, wk7_v, wv49_v, ca_v, oT_v, sems, osems):
    halves = lambda src, dst: [(src.at[:, :128], dst.at[0]), (src.at[:, 128:], dst.at[1])]
    x_part = lambda lo, hi: [(xT_hbm.at[:, lo * TC:hi * TC], xT_v.at[:, lo * TC:hi * TC])]
    loads = dict(
        vectors=[(lre_hbm, lre_ref), (lim_hbm, lim_ref), (ldt_hbm, ldt_ref), (dsk_hbm, dsk_ref),
                 (gw_hbm, gw_ref)],
        x0=x_part(0, 1) + [(bre_hbm, b_v.at[:M]), (bim_hbm, b_v.at[M:2 * M])],
        x1=x_part(1, 3), x3=x_part(3, S // TC),
        wq=halves(wq_hbm, wq_v),
        c=[(cre_hbm, cre_v), (cim_hbm, cim_v), (c_hbm, c_v)],
        wkv=halves(wk_hbm, wk_v) + halves(wv_hbm, wv_v),
        wo=[(woT_hbm.at[:, :, :128], woT_v.at[:, 0]), (woT_hbm.at[:, :, 128:], woT_v.at[:, 1])])
    n = 0
    for name, pairs in loads.items():
        loads[name] = [pltpu.make_async_copy(*p, sems.at[n + i]) for i, p in enumerate(pairs)]
        n += len(pairs)
        for cp in loads[name]:
            cp.start()

    def wait(name):
        for cp in loads.get(name, ()):
            cp.wait()

    wait("vectors")
    woT_v, qT_v, wk7_v, ca_v = map(_Tiled, (woT_v, qT_v, wk7_v, ca_v))

    lre, lim = _row(lre_ref), _row(lim_ref)
    dt = jnp.exp(_row(ldt_ref)).astype(BF16).astype(F32)
    mag = jnp.exp(dt * lre)
    a1r, a1i = mag * jnp.cos(dt * lim), mag * jnp.sin(dt * lim)
    den = lre * lre + lim * lim
    cfr, cfi = _cmul(a1r - 1.0, a1i, 2.0 * lre / den, -2.0 * lim / den)
    a2r, a2i = _cmul(a1r, a1i, a1r, a1i)
    a4r, a4i = _cmul(a2r, a2i, a2r, a2i)
    row = lax.broadcasted_iota(jnp.int32, (8, M), 0)
    steps = [(s, jnp.where(row >= s, ar, 0.0), jnp.where(row >= s, ai, 0.0))
             for s, ar, ai in ((1, a1r, a1i), (2, a2r, a2i), (4, a4r, a4i))]
    pwr = jnp.broadcast_to(a1r, (8, M))
    pwi = jnp.broadcast_to(a1i, (8, M))
    for s, ar, ai in ((1, a1r, a1i), (2, a2r, a2i), (4, a4r, a4i)):
        nr, ni = _cmul(pwr, pwi, ar, ai)
        on = (row & s) != 0
        pwr, pwi = jnp.where(on, nr, pwr), jnp.where(on, ni, pwi)
    b_v[2 * M:] = jnp.broadcast_to(_row(gw_ref), (16, M)).astype(BF16)

    def kv_gather(j, after):
        for t, w_ref in enumerate((wk_v, wv_v)):
            for lo in range(0, DC, 8):
                dep = yield
                wg_v[t, lo:lo + 8, :] = after(_head_pair(w_ref, j, lo, 8), dep)
        yield

    def kv_operands(read, after):
        for lo in range(0, DC // 2, 16):
            for c in range(2):
                dep = yield
                top, bot = (_unpair(after(read(0, o + lo, c), dep)) for o in (0, DC // 2))
                for a, x in enumerate(_rhs7(*top, *bot)):
                    wk7_v[a, lo:lo + 16, pl.ds(c * 128, 128)] = x.astype(BF16)
        for lo in range(0, DC // 4, 16):
            dep = yield
            x = [_rhs7(*(w for o in (0, DC // 2) for w in _unpair(after(read(1, o + r + lo, c), dep))))
                 for r in (0, DC // 4) for c in range(2)]
            for a in range(7):
                dep = yield
                y = [z[a] for z in x]
                for b, z in enumerate(_rhs7(after(y[0], dep), y[1], y[2], after(y[3], dep))):
                    wv49_v[a, b, lo:lo + 16, :] = z.astype(BF16)
        yield

    def first_phase(ure_v, uim_v, xa_v, wa_v, waT_v):
        after = _pacer(lax.bitcast_convert_type(jnp.broadcast_to(mag[:, :128], (8, 128)), jnp.int32) >> 31)
        HM = M // 2
        xa_v = _Tiled(xa_v)

        def x_operands():
            for lo in range(0, HM, 16):
                for col in range(0, S // 2, QC // 2):
                    dep = yield
                    x = [after(xT_v[pl.ds(r + lo, 16), pl.ds(2 * col + o, QC // 2)].astype(F32), dep)
                         for r in (0, HM) for o in (0, QC // 2)]
                    for a, y in enumerate(_rhs7(*x)):
                        xa_v[a, lo:lo + 16, pl.ds(col, QC // 2)] = y.astype(BF16)
            yield

        def wq_operands(j):
            for lo in range(0, HM, 16):
                dep = yield
                (a11, a21), (a12, a22) = ([after(w, dep) for w in _unpair(_head_pair(wq_v, j, o + lo, 16))]
                                          for o in (0, HM))
                for a, x in enumerate(_lhs7(a11, a12, a21, a22)):
                    wa_v[a, lo:lo + 16, :] = x.astype(BF16)
            for a in range(7):
                for c in (0, 128):
                    dep = yield
                    y = after(wa_v[a, :, c:c + 128].astype(F32), dep)
                    waT_v[j % 2, a, c:c + 128, :] = y.T.astype(BF16)
            yield

        def q_finish(j, t, m):
            for lo in range(0, D, 16):
                dep = yield
                x = [y[lo:lo + 16] for y in m]
                x[:3] = (after(y, dep) for y in x[:3])
                for a, y in enumerate(_combine7(x)):
                    qT_v[pl.ds((2 * j + a // 2) * D + lo, 16),
                         pl.ds(t * QC + (a % 2) * (QC // 2), QC // 2)] = (y * QSCALE).astype(BF16)
            yield

        def c_operands():
            for t in range(S // CR):
                for lo in range(0, CR // 4, 16):
                    for col in range(0, DC // 4, 128):
                        dep = yield
                        x = [_lhs7(*(after(c_v[pl.ds(t * CR + r1 + r2 + lo, 16),
                                               pl.ds(c1 + c2 + col, 128)].astype(F32), dep)
                                     for r1 in (0, CR // 2) for c1 in (0, DC // 2)))
                             for r2 in (0, CR // 4) for c2 in (0, DC // 4)]
                        for a in range(7):
                            dep = yield
                            y = [z[a] for z in x]
                            for b, z in enumerate(_lhs9(after(y[0], dep), y[1], y[2], after(y[3], dep))):
                                ca_v[a, b, pl.ds(t * (CR // 4) + lo, 16), col:col + 128] = z.astype(BF16)
            yield

        def scan():
            tiles = [slice(c, min(c + 128, M)) for c in range(0, M, 128)]
            h = [None] * len(tiles)
            for lo in range(0, S, 16):
                for n, c in enumerate(tiles):
                    ys = []
                    for r in (lo, lo + 8):
                        dep = yield
                        ur, ui = after(ure_v[r:r + 8, c], dep), after(uim_v[r:r + 8, c], dep)
                        for s, ar, ai in steps:
                            dr, di = _cmul(pltpu.roll(ur, s, 0), pltpu.roll(ui, s, 0), ar[:, c], ai[:, c])
                            ur, ui = ur + dr, ui + di
                        if r:
                            dr, di = _cmul(*h[n], pwr[:, c], pwi[:, c])
                            ur, ui = ur + dr, ui + di
                        h[n] = ur[7:8], ui[7:8]
                        ys.append((ur, ui))
                    hre_v[lo:lo + 16, c] = jnp.concatenate([ys[0][0], ys[1][0]], axis=0).astype(BF16)
                    him_v[lo:lo + 16, c] = jnp.concatenate([ys[0][1], ys[1][1]], axis=0).astype(BF16)
            yield

        def clear_out():
            for r in range(0, M, 8):
                dep = yield
                oT_v[r:r + 8, :] = after(jnp.zeros((8, S), F32), dep)
            yield

        def project_q(pairs, pending):
            seen = []
            for j in pairs:
                for t in range(S // QC):
                    m = [_dot(waT_v[j % 2, a], xa_v[a, :, t * (QC // 2):(t + 1) * (QC // 2)])
                         for a in range(7)]
                    deps = [x[r:r + 8, :128] for x in m for r in range(0, D, 32)]
                    if pending:
                        _pace(q_finish(*pending), D // 16, deps, 0.0, 0.95)
                    pending = j, t, m
                    seen += deps
                if j + 1 < H // 2:
                    _pace(wq_operands(j + 1), HM // 16 + 14, seen[-len(deps) * (S // QC):], 0.0, 0.8)
            return pending, seen

        def scale_c():
            for lo in range(0, M, 16):
                dep = yield
                yr, yi = _cmul(after(cre_v[lo:lo + 16].astype(F32), dep), cim_v[lo:lo + 16].astype(F32),
                               cfr, cfi)
                cre_v[lo:lo + 16] = yr.astype(BF16)
                cim_v[lo:lo + 16] = (-yi).astype(BF16)
            yield

        work = scan()
        next(work)
        seen = []
        for t in range(S // TC):
            if t == S // TC - 2:
                _pace(x_operands(), HM // 16 * (S // QC), seen, 0.0, 1.0)
                wait("wq")
            if t in (3, S // TC - 2):
                seen = []
            wait(f"x{t}")
            ts = pl.ds(t * TC, TC)
            u = _dot(b_v[...], xT_v[:, ts])
            ure_v[ts, :] = u[:M].T
            uim_v[ts, :] = u[M:2 * M].T
            gT_v[:, ts] = jax.nn.sigmoid(u[2 * M:2 * M + 8])
            deps = _marks((u, 512))
            if t:
                _pace(work, 40, deps, 0.0, 0.95, True)
            seen += deps
        _pace(wq_operands(0), HM // 16 + 14, seen, 0.0, 0.8)
        pending, deps = project_q(range(1), None)
        _pace(clear_out(), M // 8, deps, 0.0, 0.95)
        _pace(work, 124, deps, 0.0, 0.98, True)
        wait("c")
        pending, deps = project_q(range(1, 7), pending)
        _pace(work, S // 2 - 7 * 40 - 124, deps, 0.0, 0.99, True)
        _pace(c_operands(), S // 64 * 16, deps, 0.0, 0.99)
        wait("wkv")
        pending, deps = project_q(range(7, H // 2), pending)
        _pace(scale_c(), M // 16, deps, 0.0, 0.95)
        _pace(kv_operands(lambda t, r, c: _head_pair((wk_v, wv_v)[t], 0, r, 16, (c,)), after),
              DC // 16 + DC // 8, deps, 0.0, 0.95)
        _pace(q_finish(*pending), D // 16, deps, 0.99, 0.999)

    pl.run_scoped(first_phase, V((S, M), F32), V((S, M), F32), _tiled(7, M // 2, S // 2),
                  V((7, M // 2, D), BF16), V((2, 7, D, M // 2), BF16))

    wait("wo")

    def head_pair(j, j_next, k_v, v_v, vT_v, s_v, p_v, pd_v, o_v):
        after = _pacer(jnp.full((8, 128), j >> 4, jnp.int32))
        k_v, vT_v, pd_v, o_v = map(_Tiled, (k_v, vT_v, pd_v, o_v))
        causal = (lax.broadcasted_iota(jnp.int32, (128, 128), 0)
                  <= lax.broadcasted_iota(jnp.int32, (128, 128), 1))

        log = []

        def dot(a, b):
            y = _dot(a, b)
            log.extend(_marks((y, a.shape[1])))
            return y

        def project(t, m, n):
            for a in range(len(m), len(m) + n):
                c = [ca_v[a, b, t * (CR // 4):(t + 1) * (CR // 4), :] for b in range(9)]
                full = jnp.concatenate([jnp.concatenate([c[Q11], c[Q12]], axis=1),
                                        jnp.concatenate([c[Q21], c[Q22]], axis=1)], axis=0)
                m.append((dot(full, wk7_v[a, :, :]), [dot(c[b], wv49_v[a, b]) for b in range(7)]))

        def finish(t, m):
            for lo in range(0, CR // 2, 16):
                dep = yield
                x = [z[lo:lo + 16] for z, _ in m]
                x[:3] = (after(z, dep) for z in x[:3])
                for a, z in enumerate(_combine7(x)):
                    k_v[a % 2, pl.ds(t * CR + (a // 2) * (CR // 2) + lo, 16), :] = z.astype(BF16)
            for lo in range(0, CR // 4, 8):
                dep = yield
                y = []
                for _, z in m:
                    x = [u[lo:lo + 8] for u in z]
                    x[:3] = (after(u, dep) for u in x[:3])
                    y.append(_combine7(x))
                for b in range(4):
                    for a, z in enumerate(_combine7([u[b] for u in y])):
                        v_v[a % 2, pl.ds(t * CR + (a // 2) * (CR // 2) + (b // 2) * (CR // 4) + lo, 8),
                            pl.ds((b % 2) * 128, 128)] = z
            yield

        def v_operands(blocks):
            for e, b in blocks:
                tiles = [(e, pl.ds(b * 256 + r, 128), pl.ds(c, 128)) for c in (0, 128) for r in (0, 128)]
                for tile in tiles:
                    dep = yield
                    v_v[tile] = after(v_v[tile], dep).T
                for lo in range(0, 128, 16):
                    dep = yield
                    x = [after(v_v[e, pl.ds(r.start + lo, 16), c], dep) for _, r, c in tiles]
                    for n, z in enumerate(_lhs9(*x)):
                        vT_v[e, n, lo:lo + 16, b * 128:(b + 1) * 128] = z.astype(BF16)
            yield

        def out_proj(lo, hi):
            for t in range(lo, hi):
                ts = pl.ds(t * TC, TC)
                d = dot(jnp.concatenate([woT_v[2 * j + e, :, :] for e in range(2)], axis=1), o_v[:, ts])
                oT_v[:, ts] += d

        tasks = [(e, i) for i in range(S // BQ) for e in range(2)]
        st = [dict() for _ in tasks]
        chunks = lambda n, size: [(lo, min(lo + size, n)) for lo in range(0, n, size)]
        r8 = lambda x: x.reshape(-1, 8, 128)
        head = lambda e: pl.ds(pl.multiple_of(j * 2 * D + e * D, D), D)

        def scores(t):
            e, i = tasks[t]
            h = i * 128
            q = qT_v[head(e), pl.ds(i * BQ, BQ)]
            s22 = dot(k_v[e, 2 * h + 128:2 * h + 256, :], q[:, 128:])
            s22 = jnp.where(causal, s22, -1e30)
            s_v[t % 2, 3, h:h + 128, :] = s22
            m = [None, jnp.max(r8(s22), axis=0)]
            starts = list(range(0, 2 * h, CS)) or [0]
            for lo, hi in zip(starts, starts[1:] + [2 * h + 128]):
                s = dot(k_v[e, lo:hi, :], q)
                for r in range(lo, hi, 128):
                    for c in range(2):
                        x = s[r - lo:r - lo + 128, c * 128:(c + 1) * 128]
                        if r == 2 * h and c == 0:
                            x = jnp.where(causal, x, -1e30)
                        s_v[t % 2, r // 128 % 2 * 2 + c, pl.ds(r // 256 * 128, 128), :] = x
                        x = jnp.max(r8(x), axis=0)
                        m[c] = x if m[c] is None else jnp.maximum(m[c], x)
            st[t]["m"] = m

        def softmax(t):
            h = tasks[t][1] * 128
            m = [jnp.broadcast_to(jnp.max(x, axis=0, keepdims=True), (8, 128)) for x in st[t]["m"]]
            l = [0.0, 0.0]
            for lo in range(0, h + 128, 16):
                dep = yield
                mm = [after(x, dep) for x in m]
                p = {}
                for a in ((0, 1, 2, 3) if lo < h else (0, 1, 3)):
                    p[a] = jnp.exp2(r8(s_v[t % 2, a, lo:lo + 16, :]) - mm[a % 2])
                    l[a % 2] = l[a % 2] + jnp.sum(p[a], axis=0)
                if lo < h:
                    for a, x in enumerate(_rhs7(p[0], p[1], p[2], p[3])):
                        p_v[t % 2, a, lo:lo + 16, :] = x.reshape(16, 128).astype(BF16)
                else:
                    for a, x in p.items():
                        pd_v[t % 2, a // 2, pl.ds(lo - h, 16), pl.ds((a % 2) * 128, 128)] = (
                            x.reshape(16, 128).astype(BF16))
            st[t]["l"] = l
            yield

        def context(t):
            e, i = tasks[t]
            h = i * 128
            acc = None
            for lo, hi in chunks(h, CP):
                m = [dot(vT_v[e, a, :, lo:hi], p_v[t % 2, a, lo:hi, :]) for a in range(7)]
                acc = m if acc is None else [x + y for x, y in zip(acc, m)]
            d1 = dot(jnp.concatenate([vT_v[e, n, :, h:h + 128] for n in (Q11, Q21)], axis=0), pd_v[t % 2, 0, :, :])
            d2 = dot(jnp.concatenate([vT_v[e, n, :, h:h + 128] for n in (Q12, Q22)], axis=0),
                      pd_v[t % 2, 1, :, 128:])
            c = [d1[:, :128], d1[:, 128:] + d2]
            if acc:
                y = _combine7(acc)
                c = [c[a] + jnp.concatenate([y[a], y[a + 2]], axis=0) for a in range(2)]
            for a in range(2):
                l = jnp.sum(st[t]["l"][a], axis=0, keepdims=True)
                o_v[e * D:(e + 1) * D, pl.ds(i * BQ + a * 128, 128)] = (c[a] * (1.0 / l)).astype(BF16)

        m = [[] for _ in range(S // CR)]
        both = lambda *bs: [(e, b) for b in bs for e in range(2)]
        project(0, m[0], 7)
        at = len(log)
        _pace(kv_gather(j_next, after), DC // 4, log, 0.0, 1.0)
        project(1, m[1], 7)
        _pace(finish(0, m[0]), 32, log[at:], 0.0, 0.6)
        _pace(v_operands(both(0)), 24, log[at:], 0.6, 0.95)
        scores(0)
        start = []
        for t in range(len(tasks) + 1):
            start.append(len(log))
            if t > 0:
                context(t - 1)
            for n in range(PLAN["p2"][t]):
                project(2, m[2], 1)
            for n in range(PLAN["p3"][t]):
                project(3, m[3], 1)
            out_proj(*PLAN["out"][t:t + 2])
            if t in (3, 7, 11):
                _pace(finish(t // 4 + 1, m[t // 4 + 1]), 32, log[start[PLAN["fin"][t // 4]]:], 0.0, 0.95)
            if t + 1 < len(tasks):
                scores(t + 1)
            if t % 2 == 0 and 0 < t < len(tasks):
                _pace(v_operands(both(t // 2)), 24, log[start[t - (t % 4 == 2) - 1]:], 0.0, 0.95)
            if t < len(tasks):
                _pace(softmax(t), (tasks[t][1] + 1) * 8, log[start[t]:], 0.0, 0.9)
        _pace(kv_operands(lambda t, r, c: wg_v[t, r:r + 16, c * 128:(c + 1) * 128], after),
              DC // 16 + DC // 8,              log[start[PLAN["fin"][2]]:], 0.0, 0.97)

    @functools.partial(
        pl.run_scoped, k_v=_tiled(2, S, D), v_v=V((2, S, D), F32),
        vT_v=_tiled(2, 9, 128, S // 2), s_v=V((2, 4, S // 2, 128), F32),
        p_v=V((2, 7, S // 2, 128), BF16), pd_v=_tiled(2, 2, 128, BQ), o_v=_tiled(2 * D, S))
    def _(**refs):
        def two_pairs(i, _):
            head_pair(2 * i, (i, 1), **refs)
            head_pair(2 * i + 1, (jnp.minimum(i + 1, H // 4 - 1), 0), **refs)

        lax.fori_loop(0, H // 4, two_pairs, None)

    dsk = jnp.broadcast_to(_row(dsk_ref), (TC, M)).T
    outs = []
    for t in range(S // TC):
        ts = pl.ds(t * TC, TC)
        b = (_dot_nt(cre_v[...], hre_v[ts, :]) + _dot_nt(cim_v[...], him_v[ts, :])
             + xT_v[:, ts].astype(F32) * dsk)
        g = gT_v[:1, ts]
        oT_v[:, ts] = g * oT_v[:, ts] + (1.0 - g) * b
        cp = pltpu.make_async_copy(oT_v.at[:, ts], outT_hbm.at[:, ts], osems.at[t])
        cp.start()
        outs.append(cp)
    for cp in outs:
        cp.wait()


@jax.jit
def pallas_gated_mix__compressed_kv_cla__ssm_conv_s5__prompt_kernel(
    A_x: jax.Array,
    A_c_kv: jax.Array,
    A_w_q: jax.Array,
    A_w_uk: jax.Array,
    A_w_uv: jax.Array,
    A_w_o: jax.Array,
    B_x: jax.Array,
    B_Lambda_re: jax.Array,
    B_Lambda_im: jax.Array,
    B_B_re: jax.Array,
    B_B_im: jax.Array,
    B_C_re: jax.Array,
    B_C_im: jax.Array,
    B_log_dt: jax.Array,
    B_Dskip: jax.Array,
    gate_w: jax.Array,
):
    del B_x
    hbm = pl.BlockSpec(memory_space=pltpu.MemorySpace.HBM)
    outT = pl.pallas_call(
        _kernel,
        in_specs=[hbm] * 15,
        out_specs=hbm,
        out_shape=jax.ShapeDtypeStruct((M, S), F32),
        scratch_shapes=[
            V((M, S), BF16), V((S, DC), BF16), V((2, M * H, 128), BF16), V((2, DC * H, 128), BF16),
            V((2, DC * H, 128), BF16), _tiled(H, M, D),
            V((2 * M + 16, M), BF16), V((M, M), BF16), V((M, M), BF16), *[V((M,), BF16)] * 5,
            _tiled(H * D, S), V((S, M), BF16), V((S, M), BF16), V((8, S), F32),
            V((2, DC, D), jnp.uint32),
            _tiled(7, DC // 2, D), V((7, 7, DC // 4, D // 2), BF16),
            _tiled(7, 9, S // 4, DC // 4), V((M, S), F32),
            pltpu.SemaphoreType.DMA((21,)), pltpu.SemaphoreType.DMA((S // TC,)),
        ],
        compiler_params=pltpu.CompilerParams(vmem_limit_bytes=126 * 1024 * 1024),
    )(A_x.reshape(S, M).T, A_c_kv.reshape(S, DC), A_w_q.reshape(M * H, D), A_w_uk.reshape(DC * H, D),
      A_w_uv.reshape(DC * H, D), A_w_o.transpose(0, 2, 1), B_Lambda_re, B_Lambda_im,
      B_B_re, B_B_im, B_C_re, B_C_im, B_log_dt, B_Dskip, gate_w)
    return outT.T.reshape(1, S, M)
```

```python
import functools
import math

import jax
import jax.numpy as jnp
from jax import lax
import jax.experimental.pallas as pl
import jax.experimental.pallas.tpu as pltpu

S, M, H, D, DC = 2048, 448, 16, 256, 1024
BQ = 256
TC = 256
QC = 512
CS, CP = 1024, 1024
QSCALE = D ** -0.5 * math.log2(math.e)
V = pltpu.VMEM
PLAN = dict(p2=[3, 2, 2, 0, 0, 0, 0, 0, 0, 0, 0, 0, 0, 0, 0, 0, 0],
            p3=[0, 0, 0, 2, 2, 2, 1, 0, 0, 0, 0, 0, 0, 0, 0, 0, 0],
            out=[0, 0, 0, 0, 0, 0, 0, 0, 1, 2, 3, 4, 4, 5, 5, 6, 7, 8],
            fin=[0, 3, 7])
CR = 512
F32, BF16 = jnp.float32, jnp.bfloat16
NT = (((1,), (1,)), ((), ()))


def _tiled(*shape):
    return V((*shape[:-2], shape[-1] // 128, shape[-2], 128), BF16)


class _Tiled:
    def __init__(self, ref):
        self.ref = ref

    def _split(self, idx):
        *lead, rows, cols = idx
        if isinstance(cols, slice):
            lo, hi, _ = cols.indices(self.ref.shape[-3] * 128)
        else:
            lo, hi = cols.start, cols.start + cols.size
        return [(*lead, c, rows, slice(None)) for c in range(lo // 128, hi // 128)]

    def __getitem__(self, idx):
        return jnp.concatenate([self.ref[i] for i in self._split(idx)], axis=1)

    def __setitem__(self, idx, value):
        for n, i in enumerate(self._split(idx)):
            self.ref[i] = value[:, n * 128:(n + 1) * 128]


def _dot(a, b):
    return jnp.dot(a, b, preferred_element_type=F32)


def _dot_nt(a, b):
    return lax.dot_general(a, b, NT, preferred_element_type=F32)


def _head_pair(w_ref, j, lo, rows, halves=(0, 1)):
    cols = []
    for c in halves:
        r = w_ref.at[c].bitcast(jnp.uint32)
        if isinstance(j, int):
            w = r[pl.ds(lo * 8 + j, rows, stride=8), :]
        else:
            i, odd = j
            r = r.at[pl.ds(pl.multiple_of((i // 2) * 4, 4) + lo * 8, rows * 8 - 4)]
            w = jnp.where(i % 2 == 0, r[pl.ds(odd, rows, stride=8), :],
                          r[pl.ds(odd + 2, rows, stride=8), :])
        cols.append(w)
    return jnp.concatenate(cols, axis=1)


def _unpair(w):
    lo = lax.bitcast_convert_type(w << 16, F32)
    hi = lax.bitcast_convert_type(w & jnp.uint32(0xFFFF0000), F32)
    return lo, hi


def _pacer(zero):
    def after(x, dep):
        bits = lax.bitcast_convert_type(dep, jnp.int32) & zero
        bits = jnp.tile(bits, (x.shape[0] // 8, -(-x.shape[1] // 128)))[:, :x.shape[1]]
        return lax.bitcast_convert_type(lax.bitcast_convert_type(x, jnp.int32) | bits, x.dtype)
    return after


def _pace(work, n, deps, lo, hi, started=False):
    if not started:
        next(work)
    for i in range(n):
        work.send(deps[int((lo + (hi - lo) * i / n) * len(deps))])


def _marks(x):
    y, k = x
    tiles = [(r, c) for c in range(0, y.shape[1], 128) for r in range(0, y.shape[0], 8)]
    n = len(tiles) * (k // 128) // 16
    return [y[r:r + 8, c:c + 128] for r, c in (tiles[i * len(tiles) // n] for i in range(n))]


def _lhs7(a11, a12, a21, a22):
    return a11 + a22, a21 + a22, a11, a22, a11 + a12, a21 - a11, a12 - a22


def _lhs9(a11, a12, a21, a22):
    return (*_lhs7(a11, a12, a21, a22), a12, a21)


Q11, Q12, Q21, Q22 = 2, 7, 8, 3


def _rhs7(b11, b12, b21, b22):
    return b11 + b22, b11, b12 - b22, b21 - b11, b22, b11 + b12, b21 + b22


def _combine7(m):
    return m[0] + m[3] - m[4] + m[6], m[2] + m[4], m[1] + m[3], m[0] - m[1] + m[2] + m[5]


def _cmul(ar, ai, br, bi):
    return ar * br - ai * bi, ar * bi + ai * br


def _row(ref):
    return ref[...].astype(F32).reshape(1, M)


def _kernel(xT_hbm, c_hbm, wq_hbm, wk_hbm, wv_hbm, woT_hbm, lre_hbm, lim_hbm,
            bre_hbm, bim_hbm, cre_hbm, cim_hbm, ldt_hbm, dsk_hbm, gw_hbm,
            outT_hbm,
            xT_v, c_v, wq_v, wk_v, wv_v, woT_v, b_v, cre_v, cim_v,
            lre_ref, lim_ref, ldt_ref, dsk_ref, gw_ref,
            qT_v, h_v, cc_v, gT_v, wg_v, wk7_v, wv49_v, ca_v, oT_v, sems, osems):
    halves = lambda src, dst: [(src.at[:, :128], dst.at[0]), (src.at[:, 128:], dst.at[1])]
    x_part = lambda lo, hi: [(xT_hbm.at[:, lo * TC:hi * TC], xT_v.at[:, lo * TC:hi * TC])]
    loads = dict(
        vectors=[(lre_hbm, lre_ref), (lim_hbm, lim_ref), (ldt_hbm, ldt_ref), (dsk_hbm, dsk_ref),
                 (gw_hbm, gw_ref)],
        x0=x_part(0, 1) + [(bre_hbm, b_v.at[:M]), (bim_hbm, b_v.at[M:2 * M])],
        x1=x_part(1, 3), x3=x_part(3, S // TC),
        wq=halves(wq_hbm, wq_v),
        c=[(cre_hbm, cre_v), (cim_hbm, cim_v), (c_hbm, c_v)],
        wkv=halves(wk_hbm, wk_v) + halves(wv_hbm, wv_v),
        wo=[(woT_hbm.at[:, :, :128], woT_v.at[:, 0]), (woT_hbm.at[:, :, 128:], woT_v.at[:, 1])])
    n = 0
    for name, pairs in loads.items():
        loads[name] = [pltpu.make_async_copy(*p, sems.at[n + i]) for i, p in enumerate(pairs)]
        n += len(pairs)
        for cp in loads[name]:
            cp.start()

    def wait(name):
        for cp in loads.get(name, ()):
            cp.wait()

    wait("vectors")
    woT_v, qT_v, wk7_v, ca_v = map(_Tiled, (woT_v, qT_v, wk7_v, ca_v))

    lre, lim = _row(lre_ref), _row(lim_ref)
    dt = jnp.exp(_row(ldt_ref)).astype(BF16).astype(F32)
    mag = jnp.exp(dt * lre)
    a1r, a1i = mag * jnp.cos(dt * lim), mag * jnp.sin(dt * lim)
    den = lre * lre + lim * lim
    cfr, cfi = _cmul(a1r - 1.0, a1i, 2.0 * lre / den, -2.0 * lim / den)
    a2r, a2i = _cmul(a1r, a1i, a1r, a1i)
    a4r, a4i = _cmul(a2r, a2i, a2r, a2i)
    row = lax.broadcasted_iota(jnp.int32, (8, M), 0)
    steps = [(s, jnp.where(row >= s, ar, 0.0), jnp.where(row >= s, ai, 0.0))
             for s, ar, ai in ((1, a1r, a1i), (2, a2r, a2i), (4, a4r, a4i))]
    pwr = jnp.broadcast_to(a1r, (8, M))
    pwi = jnp.broadcast_to(a1i, (8, M))
    for s, ar, ai in ((1, a1r, a1i), (2, a2r, a2i), (4, a4r, a4i)):
        nr, ni = _cmul(pwr, pwi, ar, ai)
        on = (row & s) != 0
        pwr, pwi = jnp.where(on, nr, pwr), jnp.where(on, ni, pwi)
    b_v[2 * M:] = jnp.broadcast_to(_row(gw_ref), (16, M)).astype(BF16)

    def kv_gather(j, after):
        for t, w_ref in enumerate((wk_v, wv_v)):
            for lo in range(0, DC, 8):
                dep = yield
                wg_v[t, lo:lo + 8, :] = after(_head_pair(w_ref, j, lo, 8), dep)
        yield

    def kv_operands(read, after):
        for lo in range(0, DC // 2, 16):
            for c in range(2):
                dep = yield
                top, bot = (_unpair(after(read(0, o + lo, c), dep)) for o in (0, DC // 2))
                for a, x in enumerate(_rhs7(*top, *bot)):
                    wk7_v[a, lo:lo + 16, pl.ds(c * 128, 128)] = x.astype(BF16)
        for lo in range(0, DC // 4, 16):
            dep = yield
            x = [_rhs7(*(w for o in (0, DC // 2) for w in _unpair(after(read(1, o + r + lo, c), dep))))
                 for r in (0, DC // 4) for c in range(2)]
            for a in range(7):
                dep = yield
                y = [z[a] for z in x]
                for b, z in enumerate(_rhs7(after(y[0], dep), y[1], y[2], after(y[3], dep))):
                    wv49_v[a, b, lo:lo + 16, :] = z.astype(BF16)
        yield

    def first_phase(ure_v, uim_v, xa_v, wa_v, waT_v):
        after = _pacer(lax.bitcast_convert_type(jnp.broadcast_to(mag[:, :128], (8, 128)), jnp.int32) >> 31)
        HM = M // 2
        tiles = [slice(c, min(c + 128, M)) for c in range(0, M, 128)]
        xa_v = _Tiled(xa_v)

        def x_operands():
            for lo in range(0, HM, 16):
                for col in range(0, S // 2, QC // 2):
                    dep = yield
                    x = [after(xT_v[pl.ds(r + lo, 16), pl.ds(2 * col + o, QC // 2)].astype(F32), dep)
                         for r in (0, HM) for o in (0, QC // 2)]
                    for a, y in enumerate(_rhs7(*x)):
                        xa_v[a, lo:lo + 16, pl.ds(col, QC // 2)] = y.astype(BF16)
            yield

        def wq_operands(j):
            for lo in range(0, HM, 16):
                dep = yield
                (a11, a21), (a12, a22) = ([after(w, dep) for w in _unpair(_head_pair(wq_v, j, o + lo, 16))]
                                          for o in (0, HM))
                for a, x in enumerate(_lhs7(a11, a12, a21, a22)):
                    wa_v[a, lo:lo + 16, :] = x.astype(BF16)
            for a in range(7):
                for c in (0, 128):
                    dep = yield
                    y = after(wa_v[a, :, c:c + 128].astype(F32), dep)
                    waT_v[j % 2, a, c:c + 128, :] = y.T.astype(BF16)
            yield

        def q_finish(j, t, m):
            for lo in range(0, D, 16):
                dep = yield
                x = [y[lo:lo + 16] for y in m]
                x[:3] = (after(y, dep) for y in x[:3])
                for a, y in enumerate(_combine7(x)):
                    qT_v[pl.ds((2 * j + a // 2) * D + lo, 16),
                         pl.ds(t * QC + (a % 2) * (QC // 2), QC // 2)] = (y * QSCALE).astype(BF16)
            yield

        def c_operands():
            for t in range(S // CR):
                for lo in range(0, CR // 4, 16):
                    for col in range(0, DC // 4, 128):
                        dep = yield
                        x = [_lhs7(*(after(c_v[pl.ds(t * CR + r1 + r2 + lo, 16),
                                               pl.ds(c1 + c2 + col, 128)].astype(F32), dep)
                                     for r1 in (0, CR // 2) for c1 in (0, DC // 2)))
                             for r2 in (0, CR // 4) for c2 in (0, DC // 4)]
                        for a in range(7):
                            dep = yield
                            y = [z[a] for z in x]
                            for b, z in enumerate(_lhs9(after(y[0], dep), y[1], y[2], after(y[3], dep))):
                                ca_v[a, b, pl.ds(t * (CR // 4) + lo, 16), col:col + 128] = z.astype(BF16)
            yield

        def scan():
            h = [None] * len(tiles)
            for lo in range(0, S, 16):
                for n, c in enumerate(tiles):
                    ys = []
                    for r in (lo, lo + 8):
                        dep = yield
                        ur, ui = after(ure_v[r:r + 8, c], dep), after(uim_v[r:r + 8, c], dep)
                        for s, ar, ai in steps:
                            dr, di = _cmul(pltpu.roll(ur, s, 0), pltpu.roll(ui, s, 0), ar[:, c], ai[:, c])
                            ur, ui = ur + dr, ui + di
                        if r:
                            dr, di = _cmul(*h[n], pwr[:, c], pwi[:, c])
                            ur, ui = ur + dr, ui + di
                        h[n] = ur[7:8], ui[7:8]
                        ys.append((ur, ui))
                    h_v[lo:lo + 16, 2 * c.start:2 * c.stop] = jnp.concatenate(
                        [jnp.concatenate(y, axis=1) for y in ys], axis=0).astype(BF16)
            yield

        def clear_out():
            for r in range(0, M, 8):
                dep = yield
                oT_v[r:r + 8, :] = after(jnp.zeros((8, S), F32), dep)
            yield

        def project_q(pairs, pending):
            seen = []
            for j in pairs:
                for t in range(S // QC):
                    m = [_dot(waT_v[j % 2, a], xa_v[a, :, t * (QC // 2):(t + 1) * (QC // 2)])
                         for a in range(7)]
                    deps = [x[r:r + 8, :128] for x in m for r in range(0, D, 32)]
                    if pending:
                        _pace(q_finish(*pending), D // 16, deps, 0.0, 0.95)
                    pending = j, t, m
                    seen += deps
                if j + 1 < H // 2:
                    _pace(wq_operands(j + 1), HM // 16 + 14, seen[-len(deps) * (S // QC):], 0.0, 0.8)
            return pending, seen

        def scale_c():
            for lo in range(0, M, 16):
                dep = yield
                yr, yi = _cmul(after(cre_v[lo:lo + 16].astype(F32), dep), cim_v[lo:lo + 16].astype(F32),
                               cfr, cfi)
                for c in tiles:
                    cc_v[lo:lo + 16, 2 * c.start:2 * c.stop] = jnp.concatenate(
                        [yr[:, c], -yi[:, c]], axis=1).astype(BF16)
            yield

        work = scan()
        next(work)
        seen = []
        for t in range(S // TC):
            if t == S // TC - 2:
                _pace(x_operands(), HM // 16 * (S // QC), seen, 0.0, 1.0)
                wait("wq")
            if t in (3, S // TC - 2):
                seen = []
            wait(f"x{t}")
            ts = pl.ds(t * TC, TC)
            u = _dot(b_v[...], xT_v[:, ts])
            ure_v[ts, :] = u[:M].T
            uim_v[ts, :] = u[M:2 * M].T
            gT_v[:, ts] = jax.nn.sigmoid(u[2 * M:2 * M + 8])
            deps = _marks((u, 512))
            if t:
                _pace(work, 40, deps, 0.0, 0.95, True)
            seen += deps
        _pace(wq_operands(0), HM // 16 + 14, seen, 0.0, 0.8)
        pending, deps = project_q(range(1), None)
        _pace(clear_out(), M // 8, deps, 0.0, 0.95)
        _pace(work, 124, deps, 0.0, 0.98, True)
        wait("c")
        pending, deps = project_q(range(1, 7), pending)
        _pace(work, S // 2 - 7 * 40 - 124, deps, 0.0, 0.99, True)
        _pace(c_operands(), S // 64 * 16, deps, 0.0, 0.99)
        wait("wkv")
        pending, deps = project_q(range(7, H // 2), pending)
        _pace(scale_c(), M // 16, deps, 0.0, 0.95)
        _pace(kv_operands(lambda t, r, c: _head_pair((wk_v, wv_v)[t], 0, r, 16, (c,)), after),
              DC // 16 + DC // 8, deps, 0.0, 0.95)
        _pace(q_finish(*pending), D // 16, deps, 0.99, 0.999)

    pl.run_scoped(first_phase, V((S, M), F32), V((S, M), F32), _tiled(7, M // 2, S // 2),
                  V((7, M // 2, D), BF16), V((2, 7, D, M // 2), BF16))

    wait("wo")

    def head_pair(j, j_next, k_v, v_v, vT_v, s_v, p_v, pd_v, o_v):
        after = _pacer(jnp.full((8, 128), j >> 4, jnp.int32))
        k_v, vT_v, pd_v, o_v = map(_Tiled, (k_v, vT_v, pd_v, o_v))
        causal = (lax.broadcasted_iota(jnp.int32, (128, 128), 0)
                  <= lax.broadcasted_iota(jnp.int32, (128, 128), 1))

        log = []

        def dot(a, b):
            y = _dot(a, b)
            log.extend(_marks((y, a.shape[1])))
            return y

        def project(t, m, n):
            for a in range(len(m), len(m) + n):
                c = [ca_v[a, b, t * (CR // 4):(t + 1) * (CR // 4), :] for b in range(9)]
                full = jnp.concatenate([jnp.concatenate([c[Q11], c[Q12]], axis=1),
                                        jnp.concatenate([c[Q21], c[Q22]], axis=1)], axis=0)
                m.append((dot(full, wk7_v[a, :, :]), [dot(c[b], wv49_v[a, b]) for b in range(7)]))

        def finish(t, m):
            for lo in range(0, CR // 2, 16):
                dep = yield
                x = [z[lo:lo + 16] for z, _ in m]
                x[:3] = (after(z, dep) for z in x[:3])
                for a, z in enumerate(_combine7(x)):
                    k_v[a % 2, pl.ds(t * CR + (a // 2) * (CR // 2) + lo, 16), :] = z.astype(BF16)
            for lo in range(0, CR // 4, 8):
                dep = yield
                y = []
                for _, z in m:
                    x = [u[lo:lo + 8] for u in z]
                    x[:3] = (after(u, dep) for u in x[:3])
                    y.append(_combine7(x))
                for b in range(4):
                    for a, z in enumerate(_combine7([u[b] for u in y])):
                        v_v[a % 2, pl.ds(t * CR + (a // 2) * (CR // 2) + (b // 2) * (CR // 4) + lo, 8),
                            pl.ds((b % 2) * 128, 128)] = z
            yield

        def v_operands(blocks):
            for e, b in blocks:
                tiles = [(e, pl.ds(b * 256 + r, 128), pl.ds(c, 128)) for c in (0, 128) for r in (0, 128)]
                for tile in tiles:
                    dep = yield
                    v_v[tile] = after(v_v[tile], dep).T
                for lo in range(0, 128, 16):
                    dep = yield
                    x = [after(v_v[e, pl.ds(r.start + lo, 16), c], dep) for _, r, c in tiles]
                    for n, z in enumerate(_lhs9(*x)):
                        vT_v[e, n, lo:lo + 16, b * 128:(b + 1) * 128] = z.astype(BF16)
            yield

        def out_proj(lo, hi):
            for t in range(lo, hi):
                ts = pl.ds(t * TC, TC)
                d = dot(jnp.concatenate([woT_v[2 * j + e, :, :] for e in range(2)], axis=1), o_v[:, ts])
                oT_v[:, ts] += d

        tasks = [(e, i) for i in range(S // BQ) for e in range(2)]
        st = [dict() for _ in tasks]
        chunks = lambda n, size: [(lo, min(lo + size, n)) for lo in range(0, n, size)]
        r8 = lambda x: x.reshape(-1, 8, 128)
        head = lambda e: pl.ds(pl.multiple_of(j * 2 * D + e * D, D), D)

        def scores(t):
            e, i = tasks[t]
            h = i * 128
            q = qT_v[head(e), pl.ds(i * BQ, BQ)]
            s22 = dot(k_v[e, 2 * h + 128:2 * h + 256, :], q[:, 128:])
            s22 = jnp.where(causal, s22, -1e30)
            s_v[t % 2, 3, h:h + 128, :] = s22
            m = [None, jnp.max(r8(s22), axis=0)]
            starts = list(range(0, 2 * h, CS)) or [0]
            for lo, hi in zip(starts, starts[1:] + [2 * h + 128]):
                s = dot(k_v[e, lo:hi, :], q)
                for r in range(lo, hi, 128):
                    for c in range(2):
                        x = s[r - lo:r - lo + 128, c * 128:(c + 1) * 128]
                        if r == 2 * h and c == 0:
                            x = jnp.where(causal, x, -1e30)
                        s_v[t % 2, r // 128 % 2 * 2 + c, pl.ds(r // 256 * 128, 128), :] = x
                        x = jnp.max(r8(x), axis=0)
                        m[c] = x if m[c] is None else jnp.maximum(m[c], x)
            st[t]["m"] = m

        def softmax(t):
            h = tasks[t][1] * 128
            m = [jnp.broadcast_to(jnp.max(x, axis=0, keepdims=True), (8, 128)) for x in st[t]["m"]]
            l = [0.0, 0.0]
            for lo in range(0, h + 128, 16):
                dep = yield
                mm = [after(x, dep) for x in m]
                p = {}
                for a in ((0, 1, 2, 3) if lo < h else (0, 1, 3)):
                    p[a] = jnp.exp2(r8(s_v[t % 2, a, lo:lo + 16, :]) - mm[a % 2])
                    l[a % 2] = l[a % 2] + jnp.sum(p[a], axis=0)
                if lo < h:
                    for a, x in enumerate(_rhs7(p[0], p[1], p[2], p[3])):
                        p_v[t % 2, a, lo:lo + 16, :] = x.reshape(16, 128).astype(BF16)
                else:
                    for a, x in p.items():
                        pd_v[t % 2, a // 2, pl.ds(lo - h, 16), pl.ds((a % 2) * 128, 128)] = (
                            x.reshape(16, 128).astype(BF16))
            st[t]["l"] = l
            yield

        def context(t):
            e, i = tasks[t]
            h = i * 128
            acc = None
            for lo, hi in chunks(h, CP):
                m = [dot(vT_v[e, a, :, lo:hi], p_v[t % 2, a, lo:hi, :]) for a in range(7)]
                acc = m if acc is None else [x + y for x, y in zip(acc, m)]
            d1 = dot(jnp.concatenate([vT_v[e, n, :, h:h + 128] for n in (Q11, Q21)], axis=0), pd_v[t % 2, 0, :, :])
            d2 = dot(jnp.concatenate([vT_v[e, n, :, h:h + 128] for n in (Q12, Q22)], axis=0),
                      pd_v[t % 2, 1, :, 128:])
            c = [d1[:, :128], d1[:, 128:] + d2]
            if acc:
                y = _combine7(acc)
                c = [c[a] + jnp.concatenate([y[a], y[a + 2]], axis=0) for a in range(2)]
            for a in range(2):
                l = jnp.sum(st[t]["l"][a], axis=0, keepdims=True)
                o_v[e * D:(e + 1) * D, pl.ds(i * BQ + a * 128, 128)] = (c[a] * (1.0 / l)).astype(BF16)

        m = [[] for _ in range(S // CR)]
        both = lambda *bs: [(e, b) for b in bs for e in range(2)]
        project(0, m[0], 7)
        at = len(log)
        _pace(kv_gather(j_next, after), DC // 4, log, 0.0, 1.0)
        project(1, m[1], 7)
        _pace(finish(0, m[0]), 32, log[at:], 0.0, 0.6)
        _pace(v_operands(both(0)), 24, log[at:], 0.6, 0.95)
        scores(0)
        start = []
        for t in range(len(tasks) + 1):
            start.append(len(log))
            if t > 0:
                context(t - 1)
            for n in range(PLAN["p2"][t]):
                project(2, m[2], 1)
            for n in range(PLAN["p3"][t]):
                project(3, m[3], 1)
            out_proj(*PLAN["out"][t:t + 2])
            if t in (3, 7, 11):
                _pace(finish(t // 4 + 1, m[t // 4 + 1]), 32, log[start[PLAN["fin"][t // 4]]:], 0.0, 0.95)
            if t + 1 < len(tasks):
                scores(t + 1)
            if t % 2 == 0 and 0 < t < len(tasks):
                _pace(v_operands(both(t // 2)), 24, log[start[t - (t % 4 == 2) - 1]:], 0.0, 0.95)
            if t < len(tasks):
                _pace(softmax(t), (tasks[t][1] + 1) * 8, log[start[t]:], 0.0, 0.9)
        _pace(kv_operands(lambda t, r, c: wg_v[t, r:r + 16, c * 128:(c + 1) * 128], after),
              DC // 16 + DC // 8,              log[start[PLAN["fin"][2]]:], 0.0, 0.97)

    @functools.partial(
        pl.run_scoped, k_v=_tiled(2, S, D), v_v=V((2, S, D), F32),
        vT_v=_tiled(2, 9, 128, S // 2), s_v=V((2, 4, S // 2, 128), F32),
        p_v=V((2, 7, S // 2, 128), BF16), pd_v=_tiled(2, 2, 128, BQ), o_v=_tiled(2 * D, S))
    def _(**refs):
        def two_pairs(i, _):
            head_pair(2 * i, (i, 1), **refs)
            head_pair(2 * i + 1, (jnp.minimum(i + 1, H // 4 - 1), 0), **refs)

        lax.fori_loop(0, H // 4, two_pairs, None)

    dsk = jnp.broadcast_to(_row(dsk_ref), (TC, M)).T
    outs = []
    for t in range(S // TC):
        ts = pl.ds(t * TC, TC)
        b = _dot_nt(cc_v[...], h_v[ts, :]) + xT_v[:, ts].astype(F32) * dsk
        g = gT_v[:1, ts]
        oT_v[:, ts] = g * oT_v[:, ts] + (1.0 - g) * b
        cp = pltpu.make_async_copy(oT_v.at[:, ts], outT_hbm.at[:, ts], osems.at[t])
        cp.start()
        outs.append(cp)
    for cp in outs:
        cp.wait()


@jax.jit
def pallas_gated_mix__compressed_kv_cla__ssm_conv_s5__prompt_kernel(
    A_x: jax.Array,
    A_c_kv: jax.Array,
    A_w_q: jax.Array,
    A_w_uk: jax.Array,
    A_w_uv: jax.Array,
    A_w_o: jax.Array,
    B_x: jax.Array,
    B_Lambda_re: jax.Array,
    B_Lambda_im: jax.Array,
    B_B_re: jax.Array,
    B_B_im: jax.Array,
    B_C_re: jax.Array,
    B_C_im: jax.Array,
    B_log_dt: jax.Array,
    B_Dskip: jax.Array,
    gate_w: jax.Array,
):
    del B_x
    hbm = pl.BlockSpec(memory_space=pltpu.MemorySpace.HBM)
    outT = pl.pallas_call(
        _kernel,
        in_specs=[hbm] * 15,
        out_specs=hbm,
        out_shape=jax.ShapeDtypeStruct((M, S), F32),
        scratch_shapes=[
            V((M, S), BF16), V((S, DC), BF16), V((2, M * H, 128), BF16), V((2, DC * H, 128), BF16),
            V((2, DC * H, 128), BF16), _tiled(H, M, D),
            V((2 * M + 16, M), BF16), V((M, M), BF16), V((M, M), BF16), *[V((M,), BF16)] * 5,
            _tiled(H * D, S), V((S, 2 * M), BF16), V((M, 2 * M), BF16), V((8, S), F32),
            V((2, DC, D), jnp.uint32),
            _tiled(7, DC // 2, D), V((7, 7, DC // 4, D // 2), BF16),
            _tiled(7, 9, S // 4, DC // 4), V((M, S), F32),
            pltpu.SemaphoreType.DMA((21,)), pltpu.SemaphoreType.DMA((S // TC,)),
        ],
        compiler_params=pltpu.CompilerParams(vmem_limit_bytes=126 * 1024 * 1024),
    )(A_x.reshape(S, M).T, A_c_kv.reshape(S, DC), A_w_q.reshape(M * H, D), A_w_uk.reshape(DC * H, D),
      A_w_uv.reshape(DC * H, D), A_w_o.transpose(0, 2, 1), B_Lambda_re, B_Lambda_im,
      B_B_re, B_B_im, B_C_re, B_C_im, B_log_dt, B_Dskip, gate_w)
    return outT.T.reshape(1, S, M)
```

```python
import functools
import math

import jax
import jax.numpy as jnp
from jax import lax
import jax.experimental.pallas as pl
import jax.experimental.pallas.tpu as pltpu

S, M, H, D, DC = 2048, 448, 16, 256, 1024
BQ = 256
TC = 256
CR = 512
CK = 1024
SK = 32
QSCALE = D ** -0.5 * math.log2(math.e)
KV_BEFORE = [4, 6, 7, 8, 9, 10, 11, 12, 13, 14, 15, 16, 16, 16, 16, 16, 16, 16]
OUT_BEFORE = [0, 0, 0, 0, 0, 0, 0, 0, 0, 0, 0, 0, 1, 2, 3, 4, 5, 8]
F32, BF16 = jnp.float32, jnp.bfloat16
V = pltpu.VMEM


def _dot(a, b):
    return jnp.dot(a, b, preferred_element_type=F32)


def _dot_nt(a, b):
    return lax.dot_general(a, b, (((1,), (1,)), ((), ())), preferred_element_type=F32)


def _head_pair(w_ref, j, half, lo, rows):
    return w_ref.at[half].bitcast(jnp.uint32)[pl.ds(lo * 8 + j, rows, stride=8), :]


def _unpair(w):
    return [lax.bitcast_convert_type(x, F32).astype(BF16) for x in (w << 16, w & jnp.uint32(0xFFFF0000))]


def _pacer(zero):
    def after(x, dep):
        bits = lax.bitcast_convert_type(dep, jnp.int32) & zero
        bits = jnp.tile(bits, (x.shape[0] // 8, -(-x.shape[1] // 128)))[:, :x.shape[1]]
        return lax.bitcast_convert_type(lax.bitcast_convert_type(x, jnp.int32) | bits, x.dtype)
    return after


def _pace(work, n, deps, until=0.95):
    for i in range(n):
        work.send(deps[int(until * i / n * len(deps))])


def _start(work):
    next(work)
    return work


def _logged_dot(log, a, b):
    y = _dot(a, b)
    tiles = [(r, c) for c in range(0, y.shape[1], 128) for r in range(0, y.shape[0], 8)]
    n = len(tiles) * -(-a.shape[1] // 128) // 16
    log += [y[r:r + 8, c:c + 128] for r, c in (tiles[i * len(tiles) // n] for i in range(n))]
    return y


def _cmul(ar, ai, br, bi):
    return ar * br - ai * bi, ar * bi + ai * br


def _row(ref):
    return ref[...].astype(F32).reshape(1, M)


def _kernel(xT_hbm, c_hbm, wq_hbm, wk_hbm, wv_hbm, woT_hbm, lre_hbm, lim_hbm,
            bre_hbm, bim_hbm, cre_hbm, cim_hbm, ldt_hbm, dsk_hbm, gw_hbm,
            outT_hbm,
            xT_v, c_v, wq_v, wk_v, wv_v, woT_v, b_v, cre_v, cim_v,
            lre_ref, lim_ref, ldt_ref, dsk_ref, gw_ref,
            qT_v, h_v, cc_v, gT_v, w_v, oT_v, sems, osems):
    halves = lambda src, dst: [(src.at[:, :128], dst.at[0]), (src.at[:, 128:], dst.at[1])]
    x_part = lambda lo, hi: [(xT_hbm.at[:, lo * TC:hi * TC], xT_v.at[:, lo * TC:hi * TC])]
    loads = dict(
        vectors=[(lre_hbm, lre_ref), (lim_hbm, lim_ref), (ldt_hbm, ldt_ref), (dsk_hbm, dsk_ref),
                 (gw_hbm, gw_ref)],
        x0=x_part(0, 1) + [(bre_hbm, b_v.at[:M]), (bim_hbm, b_v.at[M:2 * M])],
        x1=x_part(1, 3), x3=x_part(3, S // TC),
        wq=halves(wq_hbm, wq_v),
        wkv=[(cre_hbm, cre_v), (cim_hbm, cim_v)] + halves(wk_hbm, wk_v) + halves(wv_hbm, wv_v),
        c=[(c_hbm, c_v), (woT_hbm, woT_v)])
    n = 0
    for name, pairs in loads.items():
        loads[name] = [pltpu.make_async_copy(*p, sems.at[n + i]) for i, p in enumerate(pairs)]
        n += len(pairs)
        for cp in loads[name]:
            cp.start()

    def wait(name):
        for cp in loads.get(name, ()):
            cp.wait()

    wait("vectors")
    lre, lim = _row(lre_ref), _row(lim_ref)
    dt = jnp.exp(_row(ldt_ref)).astype(BF16).astype(F32)
    mag = jnp.exp(dt * lre)
    a1r, a1i = mag * jnp.cos(dt * lim), mag * jnp.sin(dt * lim)
    big = jnp.maximum(jnp.abs(lre), jnp.abs(lim))
    nre, nim = lre / big, lim / big
    den = nre * nre + nim * nim
    cfr, cfi = _cmul((a1r - 1.0) / big, a1i / big, 2.0 * nre / den, -2.0 * nim / den)
    a2r, a2i = _cmul(a1r, a1i, a1r, a1i)
    a4r, a4i = _cmul(a2r, a2i, a2r, a2i)
    row = lax.broadcasted_iota(jnp.int32, (8, M), 0)
    powers = (1, a1r, a1i), (2, a2r, a2i), (4, a4r, a4i)
    steps = [(s, jnp.where(row >= s, ar, 0.0), jnp.where(row >= s, ai, 0.0)) for s, ar, ai in powers]
    pwr, pwi = jnp.broadcast_to(a1r, (8, M)), jnp.broadcast_to(a1i, (8, M))
    for s, ar, ai in powers:
        nr, ni = _cmul(pwr, pwi, ar, ai)
        pwr, pwi = jnp.where((row & s) != 0, nr, pwr), jnp.where((row & s) != 0, ni, pwi)
    b_v[2 * M:] = jnp.broadcast_to(_row(gw_ref), (16, M)).astype(BF16)

    @functools.partial(pl.run_scoped, ure_v=V((S, M), F32), uim_v=V((S, M), F32),
                       wqT_v=V((2, 2 * D, M), BF16))
    def _(ure_v, uim_v, wqT_v):
        after = _pacer(lax.bitcast_convert_type(jnp.broadcast_to(mag[:, :128], (8, 128)), jnp.int32) >> 31)
        tiles = [slice(c, min(c + 128, M)) for c in range(0, M, 128)]

        def unpack_wq(j):
            for m in tiles:
                for half in range(2):
                    dep = yield
                    w = after(_head_pair(wq_v, j, half, m.start, m.stop - m.start), dep).T
                    for e, x in enumerate(_unpair(w)):
                        wqT_v[j % 2, pl.ds(e * D + half * 128, 128), m] = x
            yield

        def unpack_wkv():
            for j in range(H // 2):
                for t, w_ref in enumerate((wk_v, wv_v)):
                    for lo in range(0, DC, 32):
                        dep = yield
                        w = jnp.concatenate([_head_pair(w_ref, j, c, lo, 32) for c in range(2)], axis=1)
                        for e, x in enumerate(_unpair(after(w, dep))):
                            w_v[j, 2 * t + e, lo:lo + 32, :] = x
            yield

        def scan():
            h = [None] * len(tiles)
            for lo in range(0, S, 16):
                for n, c in enumerate(tiles):
                    ys = []
                    for r in (lo, lo + 8):
                        dep = yield
                        ur, ui = after(ure_v[r:r + 8, c], dep), after(uim_v[r:r + 8, c], dep)
                        for s, ar, ai in steps:
                            dr, di = _cmul(pltpu.roll(ur, s, 0), pltpu.roll(ui, s, 0), ar[:, c], ai[:, c])
                            ur, ui = ur + dr, ui + di
                        if r:
                            dr, di = _cmul(*h[n], pwr[:, c], pwi[:, c])
                            ur, ui = ur + dr, ui + di
                        h[n] = ur[7:8], ui[7:8]
                        ys.append(jnp.concatenate([ur, ui], axis=1))
                    h_v[lo:lo + 16, 2 * c.start:2 * c.stop] = jnp.concatenate(ys, axis=0).astype(BF16)
            yield

        def scale_c():
            for lo in range(0, M, 16):
                dep = yield
                yr, yi = _cmul(after(cre_v[lo:lo + 16].astype(F32), dep), cim_v[lo:lo + 16].astype(F32),
                               cfr, cfi)
                for c in tiles:
                    cc_v[lo:lo + 16, 2 * c.start:2 * c.stop] = jnp.concatenate(
                        [yr[:, c], -yi[:, c]], axis=1).astype(BF16)
            yield

        def clear_out():
            for r in range(0, M, 8):
                dep = yield
                oT_v[r:r + 8, :] = after(jnp.zeros((8, S), F32), dep)
            yield

        def project_q(pairs):
            log = []
            for j in pairs:
                at = len(log)
                for t in range(0, S, CR):
                    q = _logged_dot(log, wqT_v[j % 2], xT_v[:, t:t + CR])
                    qT_v[j, :, t:t + CR] = (q * QSCALE).astype(BF16)
                if j + 1 < H // 2:
                    _pace(_start(unpack_wq(j + 1)), 8, log[at:], 0.8)
            return log

        log = []
        for t in range(S // TC):
            wait("wq" if t == S // TC - 2 else f"x{t}")
            ts = pl.ds(t * TC, TC)
            u = _logged_dot(log, b_v[...], xT_v[:, ts])
            ure_v[ts, :] = u[:M].T
            uim_v[ts, :] = u[M:2 * M].T
            gT_v[:, ts] = jax.nn.sigmoid(u[2 * M:2 * M + 8])
        _pace(_start(unpack_wq(0)), 8, log[len(log) * 3 // 4:], 0.8)
        log = project_q(range(H // 4))
        _pace(_start(scan()), S // 2, log)
        _pace(_start(clear_out()), M // 8, log)
        wait("wkv")
        log = project_q(range(H // 4, H // 2))
        _pace(_start(unpack_wkv()), H * DC // 32, log)
        _pace(_start(scale_c()), M // 16, log)

    wait("c")

    def head_pair(j, k_v, vT_v, s_v, p_v, o_v):
        after = _pacer(jnp.full((8, 128), j >> 4, jnp.int32))
        log = []
        dot = functools.partial(_logged_dot, log)
        causal = (lax.broadcasted_iota(jnp.int32, (128, BQ), 0)
                  <= lax.broadcasted_iota(jnp.int32, (128, BQ), 1))
        tasks = [(e, i) for i in range(S // BQ) for e in range(2)]
        stats = [dict() for _ in tasks]
        r8 = lambda x: x.reshape(-1, 8, x.shape[1])

        def project_kv(lo, hi):
            for n in range(lo, hi):
                rows = pl.ds(n // 4 * CR, CR)
                y = dot(c_v[rows, :], w_v[j, n % 4])
                if n % 4 < 2:
                    k_v[n % 2, rows, :] = y.astype(BF16)
                else:
                    vT_v[n % 2, :, rows] = y.T.astype(BF16)

        def project_out(lo, hi):
            for t in range(lo, hi):
                ts = pl.ds(t * TC, TC)
                oT_v[:, ts] += dot(jnp.concatenate([woT_v[2 * j], woT_v[2 * j + 1]], axis=1), o_v[:, ts])

        def keys(t):
            n = tasks[t][1] * BQ + 128
            starts = list(range(0, n - 128, CK)) or [0]
            return n, zip(starts, starts[1:] + [n])

        def scores(t):
            e, i = tasks[t]
            n, chunks = keys(t)
            q = qT_v[j, e * D:(e + 1) * D, i * BQ:(i + 1) * BQ]
            s = jnp.where(causal[:, :128], dot(k_v[e, n:n + 128, :], q[:, 128:]), -jnp.inf)
            s_v[t % 2, n:n + 128, 128:] = s
            m_tail = jnp.max(r8(s), axis=0)
            for lo, hi in chunks:
                s = dot(k_v[e, lo:hi, :], q)
                if hi == n:
                    last = jnp.where(causal, s[-128:], -jnp.inf)
                    s = jnp.concatenate([s[:-128], last], axis=0) if hi - lo > 128 else last
                s_v[t % 2, lo:hi, :] = s
                x = jnp.max(r8(s), axis=0)
                m = x if lo == 0 else jnp.maximum(m, x)
            stats[t]["m"] = jnp.concatenate([m[:, :128], jnp.maximum(m[:, 128:], m_tail)], axis=1)

        def softmax(t):
            n = keys(t)[0]
            m = jnp.broadcast_to(jnp.max(stats[t]["m"], axis=0, keepdims=True), (8, BQ))
            l = jnp.zeros((8, BQ), F32)
            for rows, c in ([(pl.ds(n, 64), 128), (pl.ds(n + 64, 64), 128)]
                            + [(pl.ds(lo, SK), 0) for lo in range(0, n, SK)]):
                dep = yield
                p = jnp.exp2(r8(s_v[t % 2, rows, c:]) - after(m[:, c:], dep))
                p_v[t % 2, rows, c:] = p.reshape(-1, BQ - c).astype(BF16)
                p = jnp.sum(p, axis=0)
                l = jnp.concatenate([l[:, :c], l[:, c:] + p], axis=1) if c else l + p
            stats[t]["l"] = l
            yield

        def context(t):
            e, i = tasks[t]
            n, chunks = keys(t)
            tail = dot(vT_v[e, :, n:n + 128], p_v[t % 2, n:n + 128, 128:])
            for lo, hi in chunks:
                d = dot(vT_v[e, :, lo:hi], p_v[t % 2, lo:hi, :])
                acc = d if lo == 0 else acc + d
            acc = jnp.concatenate([acc[:, :128], acc[:, 128:] + tail], axis=1)
            l = jnp.sum(stats[t]["l"], axis=0, keepdims=True)
            o_v[e * D:(e + 1) * D, i * BQ:(i + 1) * BQ] = (acc * (1.0 / l)).astype(BF16)

        project_kv(0, 2)
        scores(0)
        project_kv(2, KV_BEFORE[0])
        for t in range(len(tasks) + 1):
            at = len(log)
            if t == len(tasks):
                project_out(OUT_BEFORE[t], OUT_BEFORE[t] + 1)
                context(t - 1)
                project_out(OUT_BEFORE[t] + 1, OUT_BEFORE[t + 1])
                break
            if t > 0:
                context(t - 1)
            project_kv(*KV_BEFORE[t:t + 2])
            project_out(*OUT_BEFORE[t:t + 2])
            if t + 1 < len(tasks):
                scores(t + 1)
            _pace(_start(softmax(t)), keys(t)[0] // SK + 2, log[at:], 0.9)

    @functools.partial(pl.run_scoped, k_v=V((2, S, D), BF16), vT_v=V((2, D, S), BF16),
                       s_v=V((2, S, BQ), F32), p_v=V((2, S, BQ), BF16), o_v=V((2 * D, S), BF16))
    def _(**refs):
        lax.fori_loop(0, H // 2, lambda j, _: head_pair(j, **refs), None)

    dsk = jnp.broadcast_to(_row(dsk_ref), (TC, M)).T
    stores = []
    for t in range(S // TC):
        ts = pl.ds(t * TC, TC)
        b = _dot_nt(cc_v[...], h_v[ts, :]) + xT_v[:, ts].astype(F32) * dsk
        g = gT_v[:1, ts]
        oT_v[:, ts] = g * oT_v[:, ts] + (1.0 - g) * b
        stores.append(pltpu.make_async_copy(oT_v.at[:, ts], outT_hbm.at[:, ts], osems.at[t]))
        stores[-1].start()
    for cp in stores:
        cp.wait()


@jax.jit
def pallas_gated_mix__compressed_kv_cla__ssm_conv_s5__prompt_kernel(
    A_x: jax.Array,
    A_c_kv: jax.Array,
    A_w_q: jax.Array,
    A_w_uk: jax.Array,
    A_w_uv: jax.Array,
    A_w_o: jax.Array,
    B_x: jax.Array,
    B_Lambda_re: jax.Array,
    B_Lambda_im: jax.Array,
    B_B_re: jax.Array,
    B_B_im: jax.Array,
    B_C_re: jax.Array,
    B_C_im: jax.Array,
    B_log_dt: jax.Array,
    B_Dskip: jax.Array,
    gate_w: jax.Array,
):
    del B_x
    hbm = pl.BlockSpec(memory_space=pltpu.MemorySpace.HBM)
    outT = pl.pallas_call(
        _kernel,
        in_specs=[hbm] * 15,
        out_specs=hbm,
        out_shape=jax.ShapeDtypeStruct((M, S), F32),
        scratch_shapes=[
            V((M, S), BF16), V((S, DC), BF16), V((2, M * H, 128), BF16), V((2, DC * H, 128), BF16),
            V((2, DC * H, 128), BF16), V((H, M, D), BF16),
            V((2 * M + 16, M), BF16), V((M, M), BF16), V((M, M), BF16), *[V((M,), BF16)] * 5,
            V((H // 2, 2 * D, S), BF16), V((S, 2 * M), BF16), V((M, 2 * M), BF16), V((8, S), F32),
            V((H // 2, 4, DC, D), BF16), V((M, S), F32),
            pltpu.SemaphoreType.DMA((20,)), pltpu.SemaphoreType.DMA((S // TC,)),
        ],
        compiler_params=pltpu.CompilerParams(vmem_limit_bytes=120 * 1024 * 1024),
    )(A_x.reshape(S, M).T, A_c_kv.reshape(S, DC), A_w_q.reshape(M * H, D), A_w_uk.reshape(DC * H, D),
      A_w_uv.reshape(DC * H, D), A_w_o.transpose(0, 2, 1), B_Lambda_re, B_Lambda_im,
      B_B_re, B_B_im, B_C_re, B_C_im, B_log_dt, B_Dskip, gate_w)
    return outT.T.reshape(1, S, M)
```

```python
import functools
import math

import jax
import jax.numpy as jnp
from jax import lax
import jax.experimental.pallas as pl
import jax.experimental.pallas.tpu as pltpu

S, M, H, D, DC = 2048, 448, 16, 256, 1024
BQ = 256
TC = 256
CR = 512
CK = 1024
SK = 32
QSCALE = D ** -0.5 * math.log2(math.e)
KV_BEFORE = [2, 3, 4, 5, 6, 7, 8, 8, 8, 8]
OUT_BEFORE = [0, 0, 0, 0, 0, 0, 0, 2, 4, 8]
F32, BF16 = jnp.float32, jnp.bfloat16
V = pltpu.VMEM


def _dot(a, b):
    return jnp.dot(a, b, preferred_element_type=F32)


def _dot_nt(a, b):
    return lax.dot_general(a, b, (((1,), (1,)), ((), ())), preferred_element_type=F32)


def _head_pair(w_ref, j, half, lo, rows):
    return w_ref.at[half].bitcast(jnp.uint32)[pl.ds(lo * 8 + j, rows, stride=8), :]


def _unpair(w):
    return [lax.bitcast_convert_type(x, F32).astype(BF16) for x in (w << 16, w & jnp.uint32(0xFFFF0000))]


def _pacer(zero):
    def after(x, dep):
        bits = lax.bitcast_convert_type(dep, jnp.int32) & zero
        bits = jnp.tile(bits, (x.shape[0] // 8, -(-x.shape[1] // 128)))[:, :x.shape[1]]
        return lax.bitcast_convert_type(lax.bitcast_convert_type(x, jnp.int32) | bits, x.dtype)
    return after


def _pace(work, n, deps, until=0.95):
    for i in range(n):
        work.send(deps[int(until * i / n * len(deps))])


def _start(work):
    next(work)
    return work


def _logged_dot(log, a, b):
    y = _dot(a, b)
    tiles = [(r, c) for c in range(0, y.shape[1], 128) for r in range(0, y.shape[0], 8)]
    n = len(tiles) * -(-a.shape[1] // 128) // 16
    log += [y[r:r + 8, c:c + 128] for r, c in (tiles[i * len(tiles) // n] for i in range(n))]
    return y


def _cmul(ar, ai, br, bi):
    return ar * br - ai * bi, ar * bi + ai * br


def _row(ref):
    return ref[...].astype(F32).reshape(1, M)


def _kernel(xT_hbm, c_hbm, wq_hbm, wk_hbm, wv_hbm, woT_hbm, lre_hbm, lim_hbm,
            bre_hbm, bim_hbm, cre_hbm, cim_hbm, ldt_hbm, dsk_hbm, gw_hbm,
            outT_hbm,
            xT_v, c_v, wq_v, wk_v, wv_v, woT_v, b_v, cre_v, cim_v,
            lre_ref, lim_ref, ldt_ref, dsk_ref, gw_ref,
            qT_v, h_v, cc_v, gT_v, w_v, oT_v, sems, osems):
    halves = lambda src, dst: [(src.at[:, :128], dst.at[0]), (src.at[:, 128:], dst.at[1])]
    x_part = lambda lo, hi: [(xT_hbm.at[:, lo * TC:hi * TC], xT_v.at[:, lo * TC:hi * TC])]
    loads = dict(
        vectors=[(lre_hbm, lre_ref), (lim_hbm, lim_ref), (ldt_hbm, ldt_ref), (dsk_hbm, dsk_ref),
                 (gw_hbm, gw_ref)],
        x0=x_part(0, 1) + [(bre_hbm, b_v.at[:M]), (bim_hbm, b_v.at[M:2 * M])],
        x1=x_part(1, 3), x3=x_part(3, S // TC),
        wq=halves(wq_hbm, wq_v),
        wkv=[(cre_hbm, cre_v), (cim_hbm, cim_v)] + halves(wk_hbm, wk_v) + halves(wv_hbm, wv_v),
        c=[(c_hbm, c_v), (woT_hbm, woT_v)])
    n = 0
    for name, pairs in loads.items():
        loads[name] = [pltpu.make_async_copy(*p, sems.at[n + i]) for i, p in enumerate(pairs)]
        n += len(pairs)
        for cp in loads[name]:
            cp.start()

    def wait(name):
        for cp in loads.get(name, ()):
            cp.wait()

    wait("vectors")
    lre, lim = _row(lre_ref), _row(lim_ref)
    dt = jnp.exp(_row(ldt_ref)).astype(BF16).astype(F32)
    mag = jnp.exp(dt * lre)
    a1r, a1i = mag * jnp.cos(dt * lim), mag * jnp.sin(dt * lim)
    big = jnp.maximum(jnp.abs(lre), jnp.abs(lim))
    nre, nim = lre / big, lim / big
    den = nre * nre + nim * nim
    cfr, cfi = _cmul((a1r - 1.0) / big, a1i / big, 2.0 * nre / den, -2.0 * nim / den)
    a2r, a2i = _cmul(a1r, a1i, a1r, a1i)
    a4r, a4i = _cmul(a2r, a2i, a2r, a2i)
    row = lax.broadcasted_iota(jnp.int32, (8, M), 0)
    powers = (1, a1r, a1i), (2, a2r, a2i), (4, a4r, a4i)
    steps = [(s, jnp.where(row >= s, ar, 0.0), jnp.where(row >= s, ai, 0.0)) for s, ar, ai in powers]
    pwr, pwi = jnp.broadcast_to(a1r, (8, M)), jnp.broadcast_to(a1i, (8, M))
    for s, ar, ai in powers:
        nr, ni = _cmul(pwr, pwi, ar, ai)
        pwr, pwi = jnp.where((row & s) != 0, nr, pwr), jnp.where((row & s) != 0, ni, pwi)
    b_v[2 * M:] = jnp.broadcast_to(_row(gw_ref), (16, M)).astype(BF16)

    @functools.partial(pl.run_scoped, ure_v=V((S, M), F32), uim_v=V((S, M), F32),
                       wqT_v=V((2, 2 * D, M), BF16))
    def _(ure_v, uim_v, wqT_v):
        after = _pacer(lax.bitcast_convert_type(jnp.broadcast_to(mag[:, :128], (8, 128)), jnp.int32) >> 31)
        tiles = [slice(c, min(c + 128, M)) for c in range(0, M, 128)]

        def unpack_wq(j):
            for m in tiles:
                for half in range(2):
                    dep = yield
                    w = after(_head_pair(wq_v, j, half, m.start, m.stop - m.start), dep).T
                    for e, x in enumerate(_unpair(w)):
                        wqT_v[j % 2, pl.ds(e * D + half * 128, 128), m] = x
            yield

        def unpack_wkv():
            for j in range(H // 2):
                for t, w_ref in enumerate((wk_v, wv_v)):
                    for lo in range(0, DC, 32):
                        dep = yield
                        w = jnp.concatenate([_head_pair(w_ref, j, c, lo, 32) for c in range(2)], axis=1)
                        for e, x in enumerate(_unpair(after(w, dep))):
                            w_v[2 * j + e, t, lo:lo + 32, :] = x
            yield

        def scan():
            h = [None] * len(tiles)
            for lo in range(0, S, 16):
                for n, c in enumerate(tiles):
                    ys = []
                    for r in (lo, lo + 8):
                        dep = yield
                        ur, ui = after(ure_v[r:r + 8, c], dep), after(uim_v[r:r + 8, c], dep)
                        for s, ar, ai in steps:
                            dr, di = _cmul(pltpu.roll(ur, s, 0), pltpu.roll(ui, s, 0), ar[:, c], ai[:, c])
                            ur, ui = ur + dr, ui + di
                        if r:
                            dr, di = _cmul(*h[n], pwr[:, c], pwi[:, c])
                            ur, ui = ur + dr, ui + di
                        h[n] = ur[7:8], ui[7:8]
                        ys.append(jnp.concatenate([ur, ui], axis=1))
                    h_v[lo:lo + 16, 2 * c.start:2 * c.stop] = jnp.concatenate(ys, axis=0).astype(BF16)
            yield

        def scale_c():
            for lo in range(0, M, 16):
                dep = yield
                yr, yi = _cmul(after(cre_v[lo:lo + 16].astype(F32), dep), cim_v[lo:lo + 16].astype(F32),
                               cfr, cfi)
                for c in tiles:
                    cc_v[lo:lo + 16, 2 * c.start:2 * c.stop] = jnp.concatenate(
                        [yr[:, c], -yi[:, c]], axis=1).astype(BF16)
            yield

        def clear_out():
            for r in range(0, M, 8):
                dep = yield
                oT_v[r:r + 8, :] = after(jnp.zeros((8, S), F32), dep)
            yield

        def project_q(pairs):
            log = []
            for j in pairs:
                at = len(log)
                for t in range(0, S, CR):
                    q = _logged_dot(log, wqT_v[j % 2], xT_v[:, t:t + CR])
                    for e in range(2):
                        qT_v[2 * j + e, :, t:t + CR] = (q[e * D:(e + 1) * D] * QSCALE).astype(BF16)
                if j + 1 < H // 2:
                    _pace(_start(unpack_wq(j + 1)), 8, log[at:], 0.8)
            return log

        log = []
        for t in range(S // TC):
            wait("wq" if t == S // TC - 2 else f"x{t}")
            ts = pl.ds(t * TC, TC)
            u = _logged_dot(log, b_v[...], xT_v[:, ts])
            ure_v[ts, :] = u[:M].T
            uim_v[ts, :] = u[M:2 * M].T
            gT_v[:, ts] = jax.nn.sigmoid(u[2 * M:2 * M + 8])
        _pace(_start(unpack_wq(0)), 8, log[len(log) * 3 // 4:], 0.8)
        log = project_q(range(H // 4))
        _pace(_start(scan()), S // 2, log)
        _pace(_start(clear_out()), M // 8, log)
        wait("wkv")
        log = project_q(range(H // 4, H // 2))
        _pace(_start(unpack_wkv()), H * DC // 32, log)
        _pace(_start(scale_c()), M // 16, log)

    wait("c")

    def attend(j, k_v, vT_v, s_v, p_v, o_v):
        after = _pacer(jnp.full((8, 128), j >> 4, jnp.int32))
        log = []
        dot = functools.partial(_logged_dot, log)
        causal = (lax.broadcasted_iota(jnp.int32, (128, BQ), 0)
                  <= lax.broadcasted_iota(jnp.int32, (128, BQ), 1))
        blocks = S // BQ
        stats = [dict() for _ in range(blocks)]
        r8 = lambda x: x.reshape(-1, 8, x.shape[1])

        def project_kv(lo, hi):
            for n in range(lo, hi):
                rows = pl.ds(n // 2 * CR, CR)
                y = dot(c_v[rows, :], w_v[j, n % 2])
                if n % 2 == 0:
                    k_v[rows, :] = y.astype(BF16)
                else:
                    vT_v[:, rows] = y.T.astype(BF16)

        def project_out(lo, hi):
            for t in range(lo, hi):
                ts = pl.ds(t * TC, TC)
                oT_v[:, ts] += dot(woT_v[j], o_v[:, ts])

        def keys(t):
            n = t * BQ + 128
            starts = list(range(0, n - 128, CK)) or [0]
            return n, zip(starts, starts[1:] + [n])

        def scores(t):
            n, chunks = keys(t)
            q = qT_v[j, :, t * BQ:(t + 1) * BQ]
            s = jnp.where(causal[:, :128], dot(k_v[n:n + 128, :], q[:, 128:]), -jnp.inf)
            s_v[t % 2, n:n + 128, 128:] = s
            m_tail = jnp.max(r8(s), axis=0)
            for lo, hi in chunks:
                s = dot(k_v[lo:hi, :], q)
                if hi == n:
                    last = jnp.where(causal, s[-128:], -jnp.inf)
                    s = jnp.concatenate([s[:-128], last], axis=0) if hi - lo > 128 else last
                s_v[t % 2, lo:hi, :] = s
                x = jnp.max(r8(s), axis=0)
                m = x if lo == 0 else jnp.maximum(m, x)
            stats[t]["m"] = jnp.concatenate([m[:, :128], jnp.maximum(m[:, 128:], m_tail)], axis=1)

        def softmax(t):
            n = keys(t)[0]
            m = jnp.broadcast_to(jnp.max(stats[t]["m"], axis=0, keepdims=True), (8, BQ))
            l = jnp.zeros((8, BQ), F32)
            for rows, c in ([(pl.ds(n, 64), 128), (pl.ds(n + 64, 64), 128)]
                            + [(pl.ds(lo, SK), 0) for lo in range(0, n, SK)]):
                dep = yield
                p = jnp.exp2(r8(s_v[t % 2, rows, c:]) - after(m[:, c:], dep))
                p_v[t % 2, rows, c:] = p.reshape(-1, BQ - c).astype(BF16)
                p = jnp.sum(p, axis=0)
                l = jnp.concatenate([l[:, :c], l[:, c:] + p], axis=1) if c else l + p
            stats[t]["l"] = l
            yield

        def context(t):
            n, chunks = keys(t)
            tail = dot(vT_v[:, n:n + 128], p_v[t % 2, n:n + 128, 128:])
            for lo, hi in chunks:
                d = dot(vT_v[:, lo:hi], p_v[t % 2, lo:hi, :])
                acc = d if lo == 0 else acc + d
            acc = jnp.concatenate([acc[:, :128], acc[:, 128:] + tail], axis=1)
            l = jnp.sum(stats[t]["l"], axis=0, keepdims=True)
            o_v[:, t * BQ:(t + 1) * BQ] = (acc * (1.0 / l)).astype(BF16)

        project_kv(0, 1)
        scores(0)
        project_kv(1, KV_BEFORE[0])
        for t in range(blocks + 1):
            at = len(log)
            if t == blocks:
                project_out(OUT_BEFORE[t], OUT_BEFORE[t] + 1)
                context(t - 1)
                project_out(OUT_BEFORE[t] + 1, OUT_BEFORE[t + 1])
                break
            if t > 0:
                context(t - 1)
            project_kv(*KV_BEFORE[t:t + 2])
            project_out(*OUT_BEFORE[t:t + 2])
            if t + 1 < blocks:
                scores(t + 1)
            _pace(_start(softmax(t)), keys(t)[0] // SK + 2, log[at:], 0.9)

    @functools.partial(pl.run_scoped, k_v=V((S, D), BF16), vT_v=V((D, S), BF16),
                       s_v=V((2, S, BQ), F32), p_v=V((2, S, BQ), BF16), o_v=V((D, S), BF16))
    def _(**refs):
        lax.fori_loop(0, H, lambda j, _: attend(j, **refs), None)

    dsk = jnp.broadcast_to(_row(dsk_ref), (TC, M)).T
    stores = []
    for t in range(S // TC):
        ts = pl.ds(t * TC, TC)
        b = _dot_nt(cc_v[...], h_v[ts, :]) + xT_v[:, ts].astype(F32) * dsk
        g = gT_v[:1, ts]
        oT_v[:, ts] = g * oT_v[:, ts] + (1.0 - g) * b
        stores.append(pltpu.make_async_copy(oT_v.at[:, ts], outT_hbm.at[:, ts], osems.at[t]))
        stores[-1].start()
    for cp in stores:
        cp.wait()


@jax.jit
def pallas_gated_mix__compressed_kv_cla__ssm_conv_s5__prompt_kernel(
    A_x: jax.Array,
    A_c_kv: jax.Array,
    A_w_q: jax.Array,
    A_w_uk: jax.Array,
    A_w_uv: jax.Array,
    A_w_o: jax.Array,
    B_x: jax.Array,
    B_Lambda_re: jax.Array,
    B_Lambda_im: jax.Array,
    B_B_re: jax.Array,
    B_B_im: jax.Array,
    B_C_re: jax.Array,
    B_C_im: jax.Array,
    B_log_dt: jax.Array,
    B_Dskip: jax.Array,
    gate_w: jax.Array,
):
    del B_x
    hbm = pl.BlockSpec(memory_space=pltpu.MemorySpace.HBM)
    outT = pl.pallas_call(
        _kernel,
        in_specs=[hbm] * 15,
        out_specs=hbm,
        out_shape=jax.ShapeDtypeStruct((M, S), F32),
        scratch_shapes=[
            V((M, S), BF16), V((S, DC), BF16), V((2, M * H, 128), BF16), V((2, DC * H, 128), BF16),
            V((2, DC * H, 128), BF16), V((H, M, D), BF16),
            V((2 * M + 16, M), BF16), V((M, M), BF16), V((M, M), BF16), *[V((M,), BF16)] * 5,
            V((H, D, S), BF16), V((S, 2 * M), BF16), V((M, 2 * M), BF16), V((8, S), F32),
            V((H, 2, DC, D), BF16), V((M, S), F32),
            pltpu.SemaphoreType.DMA((20,)), pltpu.SemaphoreType.DMA((S // TC,)),
        ],
        compiler_params=pltpu.CompilerParams(vmem_limit_bytes=120 * 1024 * 1024),
    )(A_x.reshape(S, M).T, A_c_kv.reshape(S, DC), A_w_q.reshape(M * H, D), A_w_uk.reshape(DC * H, D),
      A_w_uv.reshape(DC * H, D), A_w_o.transpose(0, 2, 1), B_Lambda_re, B_Lambda_im,
      B_B_re, B_B_im, B_C_re, B_C_im, B_log_dt, B_Dskip, gate_w)
    return outT.T.reshape(1, S, M)
```

```python
import functools
import math

import jax
import jax.numpy as jnp
from jax import lax
import jax.experimental.pallas as pl
import jax.experimental.pallas.tpu as pltpu

S, M, H, D, DC = 2048, 448, 16, 256, 1024
BQ = 256
TC = 256
CR = 512
CK = 1024
SK = 32
QSCALE = D ** -0.5 * math.log2(math.e)
KV_BEFORE = [2, 3, 4, 5, 6, 7, 8, 8, 8, 8]
OUT_BEFORE = [0, 0, 0, 0, 0, 0, 0, 2, 4, 8]
F32, BF16 = jnp.float32, jnp.bfloat16
V = pltpu.VMEM


def _dot(a, b):
    return jnp.dot(a, b, preferred_element_type=F32)


def _dot_nt(a, b):
    return lax.dot_general(a, b, (((1,), (1,)), ((), ())), preferred_element_type=F32)


def _head_pair(w_ref, j, half, lo, rows):
    w_ref = w_ref.at[half].bitcast(jnp.uint32).at[pl.ds(lo * 8, rows * 8)]
    return w_ref[pl.ds(j, rows, stride=8), :]


def _unpair(w):
    return [lax.bitcast_convert_type(x, F32).astype(BF16) for x in (w << 16, w & jnp.uint32(0xFFFF0000))]


def _pacer(zero):
    def after(x, dep):
        bits = lax.bitcast_convert_type(dep, jnp.int32) & zero
        bits = jnp.tile(bits, (x.shape[0] // 8, -(-x.shape[1] // 128)))[:, :x.shape[1]]
        return lax.bitcast_convert_type(lax.bitcast_convert_type(x, jnp.int32) | bits, x.dtype)
    return after


def _pace(work, n, deps, until=0.95):
    for i in range(n):
        work.send(deps[int(until * i / n * len(deps))])


def _start(work):
    next(work)
    return work


def _logged_dot(log, a, b):
    y = _dot(a, b)
    tiles = [(r, c) for c in range(0, y.shape[1], 128) for r in range(0, y.shape[0], 8)]
    n = len(tiles) * -(-a.shape[1] // 128) // 16
    log += [y[r:r + 8, c:c + 128] for r, c in (tiles[i * len(tiles) // n] for i in range(n))]
    return y


def _cmul(ar, ai, br, bi):
    return ar * br - ai * bi, ar * bi + ai * br


def _row(ref):
    return ref[...].astype(F32).reshape(1, M)


def _kernel(xT_hbm, c_hbm, wq_hbm, wk_hbm, wv_hbm, woT_hbm, lre_hbm, lim_hbm,
            bre_hbm, bim_hbm, cre_hbm, cim_hbm, ldt_hbm, dsk_hbm, gw_hbm,
            outT_hbm,
            xT_v, c_v, wq_v, wk_v, wv_v, woT_v, b_v, cre_v, cim_v,
            lre_ref, lim_ref, ldt_ref, dsk_ref, gw_ref,
            qT_v, h_v, cc_v, gT_v, w_v, oT_v, sems, osems):
    halves = lambda src, dst: [(src.at[:, :128], dst.at[0]), (src.at[:, 128:], dst.at[1])]
    x_part = lambda lo, hi: [(xT_hbm.at[:, lo * TC:hi * TC], xT_v.at[:, lo * TC:hi * TC])]
    loads = dict(
        vectors=[(lre_hbm, lre_ref), (lim_hbm, lim_ref), (ldt_hbm, ldt_ref), (dsk_hbm, dsk_ref),
                 (gw_hbm, gw_ref)],
        x0=x_part(0, 1) + [(bre_hbm, b_v.at[:M]), (bim_hbm, b_v.at[M:2 * M])],
        x1=x_part(1, 3), x3=x_part(3, S // TC),
        wq=halves(wq_hbm, wq_v),
        wkv=[(cre_hbm, cre_v), (cim_hbm, cim_v)] + halves(wk_hbm, wk_v) + halves(wv_hbm, wv_v),
        c=[(c_hbm, c_v), (woT_hbm, woT_v)])
    n = 0
    for name, pairs in loads.items():
        loads[name] = [pltpu.make_async_copy(*p, sems.at[n + i]) for i, p in enumerate(pairs)]
        n += len(pairs)
        for cp in loads[name]:
            cp.start()

    def wait(name):
        for cp in loads.get(name, ()):
            cp.wait()

    wait("vectors")
    lre, lim = _row(lre_ref), _row(lim_ref)
    dt = jnp.exp(_row(ldt_ref)).astype(BF16).astype(F32)
    mag = jnp.exp(dt * lre)
    a1r, a1i = mag * jnp.cos(dt * lim), mag * jnp.sin(dt * lim)
    big = jnp.maximum(jnp.abs(lre), jnp.abs(lim))
    nre, nim = lre / big, lim / big
    den = nre * nre + nim * nim
    cfr, cfi = _cmul((a1r - 1.0) / big, a1i / big, 2.0 * nre / den, -2.0 * nim / den)
    a2r, a2i = _cmul(a1r, a1i, a1r, a1i)
    a4r, a4i = _cmul(a2r, a2i, a2r, a2i)
    row = lax.broadcasted_iota(jnp.int32, (8, M), 0)
    powers = (1, a1r, a1i), (2, a2r, a2i), (4, a4r, a4i)
    steps = [(s, jnp.where(row >= s, ar, 0.0), jnp.where(row >= s, ai, 0.0)) for s, ar, ai in powers]
    pwr, pwi = jnp.broadcast_to(a1r, (8, M)), jnp.broadcast_to(a1i, (8, M))
    for s, ar, ai in powers:
        nr, ni = _cmul(pwr, pwi, ar, ai)
        pwr, pwi = jnp.where((row & s) != 0, nr, pwr), jnp.where((row & s) != 0, ni, pwi)
    b_v[2 * M:] = jnp.broadcast_to(_row(gw_ref), (16, M)).astype(BF16)

    @functools.partial(pl.run_scoped, ure_v=V((S, M), F32), uim_v=V((S, M), F32),
                       wqT_v=V((H // 2, 2 * D, M), BF16))
    def _(ure_v, uim_v, wqT_v):
        after = _pacer(lax.bitcast_convert_type(jnp.broadcast_to(mag[:, :128], (8, 128)), jnp.int32) >> 31)
        tiles = [slice(c, min(c + 128, M)) for c in range(0, M, 128)]

        def unpack_wq(pairs):
            for j in pairs:
                for m in tiles:
                    for half in range(2):
                        dep = yield
                        w = after(_head_pair(wq_v, j, half, m.start, m.stop - m.start), dep).T
                        for e, x in enumerate(_unpair(w)):
                            wqT_v[j, pl.ds(e * D + half * 128, 128), m] = x
            yield

        def unpack_wkv(quarter):
            for j in range(H // 2):
                for t, w_ref in enumerate((wk_v, wv_v)):
                    for r in range(0, DC // 4, 32):
                        dep = yield
                        lo = pl.multiple_of(quarter * (DC // 4) + r, 32)
                        w = jnp.concatenate([_head_pair(w_ref, j, c, lo, 32) for c in range(2)], axis=1)
                        for e, x in enumerate(_unpair(after(w, dep))):
                            w_v[2 * j + e, t, pl.ds(lo, 32), :] = x
            yield

        def scan():
            h = [None] * len(tiles)
            for lo in range(0, S, 16):
                for n, c in enumerate(tiles):
                    ys = []
                    for r in (lo, lo + 8):
                        dep = yield
                        ur, ui = after(ure_v[r:r + 8, c], dep), after(uim_v[r:r + 8, c], dep)
                        for s, ar, ai in steps:
                            dr, di = _cmul(pltpu.roll(ur, s, 0), pltpu.roll(ui, s, 0), ar[:, c], ai[:, c])
                            ur, ui = ur + dr, ui + di
                        if r:
                            dr, di = _cmul(*h[n], pwr[:, c], pwi[:, c])
                            ur, ui = ur + dr, ui + di
                        h[n] = ur[7:8], ui[7:8]
                        ys.append(jnp.concatenate([ur, ui], axis=1))
                    h_v[lo:lo + 16, 2 * c.start:2 * c.stop] = jnp.concatenate(ys, axis=0).astype(BF16)
            yield

        def scale_c(quarter):
            for r in range(0, M // 4, 16):
                dep = yield
                rows = pl.ds(pl.multiple_of(quarter * (M // 4) + r, 16), 16)
                yr, yi = _cmul(after(cre_v[rows].astype(F32), dep), cim_v[rows].astype(F32), cfr, cfi)
                for c in tiles:
                    cc_v[rows, 2 * c.start:2 * c.stop] = jnp.concatenate(
                        [yr[:, c], -yi[:, c]], axis=1).astype(BF16)
            yield

        def clear_out():
            for r in range(0, M, 8):
                dep = yield
                oT_v[r:r + 8, :] = after(jnp.zeros((8, S), F32), dep)
            yield

        def project_q(j):
            log = []
            for t in range(0, S, CR):
                q = _logged_dot(log, wqT_v[j], xT_v[:, t:t + CR])
                for e in range(2):
                    qT_v[2 * j + e, :, t:t + CR] = (q[e * D:(e + 1) * D] * QSCALE).astype(BF16)
            return log

        log = []
        for t in range(S // TC):
            wait("wq" if t == S // TC - 2 else f"x{t}")
            ts = pl.ds(t * TC, TC)
            u = _logged_dot(log, b_v[...], xT_v[:, ts])
            ure_v[ts, :] = u[:M].T
            uim_v[ts, :] = u[M:2 * M].T
            gT_v[:, ts] = jax.nn.sigmoid(u[2 * M:2 * M + 8])
        _pace(_start(unpack_wq([0])), 8, log[len(log) * 3 // 4:], 0.8)
        log = []
        for j in range(H // 4):
            part = project_q(j)
            pairs = [n for n in (2 * j + 1, 2 * j + 2) if n < H // 2]
            _pace(_start(unpack_wq(pairs)), 8 * len(pairs), part, 0.9)
            log += part
        _pace(_start(scan()), S // 2, log)
        _pace(_start(clear_out()), M // 8, log)
        wait("wkv")

        @pl.loop(0, H // 4)
        def _(i):
            log = project_q(H // 4 + i)
            _pace(_start(unpack_wkv(i)), H * DC // 128, log)
            _pace(_start(scale_c(i)), M // 64, log)

    wait("c")

    def attend(j, k_v, vT_v, s_v, p_v, o_v):
        after = _pacer(jnp.full((8, 128), j >> 4, jnp.int32))
        log = []
        dot = functools.partial(_logged_dot, log)
        causal = (lax.broadcasted_iota(jnp.int32, (128, BQ), 0)
                  <= lax.broadcasted_iota(jnp.int32, (128, BQ), 1))
        blocks = S // BQ
        stats = [dict() for _ in range(blocks)]
        r8 = lambda x: x.reshape(-1, 8, x.shape[1])

        def project_kv(lo, hi):
            for n in range(lo, hi):
                rows = pl.ds(n // 2 * CR, CR)
                y = dot(c_v[rows, :], w_v[j, n % 2])
                if n % 2 == 0:
                    k_v[rows, :] = y.astype(BF16)
                else:
                    vT_v[:, rows] = y.T.astype(BF16)

        def project_out(lo, hi):
            for t in range(lo, hi):
                ts = pl.ds(t * TC, TC)
                oT_v[:, ts] += dot(woT_v[j], o_v[:, ts])

        def keys(t):
            n = t * BQ + 128
            starts = list(range(0, n - 128, CK)) or [0]
            return n, zip(starts, starts[1:] + [n])

        def scores(t):
            n, chunks = keys(t)
            q = qT_v[j, :, t * BQ:(t + 1) * BQ]
            s = jnp.where(causal[:, :128], dot(k_v[n:n + 128, :], q[:, 128:]), -jnp.inf)
            s_v[t % 2, n:n + 128, 128:] = s
            m_tail = jnp.max(r8(s), axis=0)
            for lo, hi in chunks:
                s = dot(k_v[lo:hi, :], q)
                if hi == n:
                    last = jnp.where(causal, s[-128:], -jnp.inf)
                    s = jnp.concatenate([s[:-128], last], axis=0) if hi - lo > 128 else last
                s_v[t % 2, lo:hi, :] = s
                x = jnp.max(r8(s), axis=0)
                m = x if lo == 0 else jnp.maximum(m, x)
            stats[t]["m"] = jnp.concatenate([m[:, :128], jnp.maximum(m[:, 128:], m_tail)], axis=1)

        def softmax(t):
            n = keys(t)[0]
            m = jnp.broadcast_to(jnp.max(stats[t]["m"], axis=0, keepdims=True), (8, BQ))
            l = jnp.zeros((8, BQ), F32)
            for rows, c in ([(pl.ds(n, 64), 128), (pl.ds(n + 64, 64), 128)]
                            + [(pl.ds(lo, SK), 0) for lo in range(0, n, SK)]):
                dep = yield
                p = jnp.exp2(r8(s_v[t % 2, rows, c:]) - after(m[:, c:], dep))
                p_v[t % 2, rows, c:] = p.reshape(-1, BQ - c).astype(BF16)
                p = jnp.sum(p, axis=0)
                l = jnp.concatenate([l[:, :c], l[:, c:] + p], axis=1) if c else l + p
            stats[t]["l"] = l
            yield

        def context(t):
            n, chunks = keys(t)
            tail = dot(vT_v[:, n:n + 128], p_v[t % 2, n:n + 128, 128:])
            for lo, hi in chunks:
                d = dot(vT_v[:, lo:hi], p_v[t % 2, lo:hi, :])
                acc = d if lo == 0 else acc + d
            acc = jnp.concatenate([acc[:, :128], acc[:, 128:] + tail], axis=1)
            l = jnp.sum(stats[t]["l"], axis=0, keepdims=True)
            o_v[:, t * BQ:(t + 1) * BQ] = (acc * (1.0 / l)).astype(BF16)

        project_kv(0, 1)
        scores(0)
        project_kv(1, KV_BEFORE[0])
        for t in range(blocks + 1):
            at = len(log)
            if t == blocks:
                project_out(OUT_BEFORE[t], OUT_BEFORE[t] + 1)
                context(t - 1)
                project_out(OUT_BEFORE[t] + 1, OUT_BEFORE[t + 1])
                break
            if t > 0:
                context(t - 1)
            project_kv(*KV_BEFORE[t:t + 2])
            project_out(*OUT_BEFORE[t:t + 2])
            if t + 1 < blocks:
                scores(t + 1)
            _pace(_start(softmax(t)), keys(t)[0] // SK + 2, log[at:], 0.9)

    @functools.partial(pl.run_scoped, k_v=V((S, D), BF16), vT_v=V((D, S), BF16),
                       s_v=V((2, S, BQ), F32), p_v=V((2, S, BQ), BF16), o_v=V((D, S), BF16))
    def _(**refs):
        lax.fori_loop(0, H, lambda j, _: attend(j, **refs), None)

    dsk = jnp.broadcast_to(_row(dsk_ref), (TC, M)).T
    stores = []
    for t in range(S // TC):
        ts = pl.ds(t * TC, TC)
        b = _dot_nt(cc_v[...], h_v[ts, :]) + xT_v[:, ts].astype(F32) * dsk
        g = gT_v[:1, ts]
        oT_v[:, ts] = g * oT_v[:, ts] + (1.0 - g) * b
        stores.append(pltpu.make_async_copy(oT_v.at[:, ts], outT_hbm.at[:, ts], osems.at[t]))
        stores[-1].start()
    for cp in stores:
        cp.wait()


@jax.jit
def pallas_gated_mix__compressed_kv_cla__ssm_conv_s5__prompt_kernel(
    A_x: jax.Array,
    A_c_kv: jax.Array,
    A_w_q: jax.Array,
    A_w_uk: jax.Array,
    A_w_uv: jax.Array,
    A_w_o: jax.Array,
    B_x: jax.Array,
    B_Lambda_re: jax.Array,
    B_Lambda_im: jax.Array,
    B_B_re: jax.Array,
    B_B_im: jax.Array,
    B_C_re: jax.Array,
    B_C_im: jax.Array,
    B_log_dt: jax.Array,
    B_Dskip: jax.Array,
    gate_w: jax.Array,
):
    del B_x
    hbm = pl.BlockSpec(memory_space=pltpu.MemorySpace.HBM)
    outT = pl.pallas_call(
        _kernel,
        in_specs=[hbm] * 15,
        out_specs=hbm,
        out_shape=jax.ShapeDtypeStruct((M, S), F32),
        scratch_shapes=[
            V((M, S), BF16), V((S, DC), BF16), V((2, M * H, 128), BF16), V((2, DC * H, 128), BF16),
            V((2, DC * H, 128), BF16), V((H, M, D), BF16),
            V((2 * M + 16, M), BF16), V((M, M), BF16), V((M, M), BF16), *[V((M,), BF16)] * 5,
            V((H, D, S), BF16), V((S, 2 * M), BF16), V((M, 2 * M), BF16), V((8, S), F32),
            V((H, 2, DC, D), BF16), V((M, S), F32),
            pltpu.SemaphoreType.DMA((20,)), pltpu.SemaphoreType.DMA((S // TC,)),
        ],
        compiler_params=pltpu.CompilerParams(vmem_limit_bytes=120 * 1024 * 1024),
    )(A_x.reshape(S, M).T, A_c_kv.reshape(S, DC), A_w_q.reshape(M * H, D), A_w_uk.reshape(DC * H, D),
      A_w_uv.reshape(DC * H, D), A_w_o.transpose(0, 2, 1), B_Lambda_re, B_Lambda_im,
      B_B_re, B_B_im, B_C_re, B_C_im, B_log_dt, B_Dskip, gate_w)
    return outT.T.reshape(1, S, M)
```
